```python
import jax
import jax.numpy as jnp

def _softmax(x, axis=-1):
    return jax.nn.softmax(x, axis=axis)
def _gelu(x):
    return jax.nn.gelu(x, approximate=True)
def _silu(x):
    return jax.nn.silu(x)
def _sigmoid(x):
    return jax.nn.sigmoid(x)
def _layernorm(x, axis=-1, eps=1e-5):
    m = jnp.mean(x, axis=axis, keepdims=True)
    v = jnp.var(x, axis=axis, keepdims=True)
    return (x - m) / jnp.sqrt(v + eps)
def _scatter_add(tgt, idx, src, axis=0):
    return tgt.at[idx].add(src)
def _segment_sum(src, seg, n):
    return jax.ops.segment_sum(src, seg, n)
class _Rng:
    def __init__(self, key):
        self._k = key
    def _next(self):
        self._k, sub = jax.random.split(self._k)
        return sub
    def normal(self, shape):
        return jax.random.normal(self._next(), shape, dtype=jnp.bfloat16)
    def randint(self, lo, hi, shape):
        return jax.random.randint(self._next(), shape, lo, hi, dtype=jnp.int32)
    def uniform(self, shape, lo=0.0, hi=1.0):
        return jax.random.uniform(self._next(), shape, jnp.bfloat16, lo, hi)
    def permutation(self, n):
        return jax.random.permutation(self._next(), n)


kernel_name = 'parallel_sum__ssm_conv_h3__dense_activation_gelu__prompt'

def setup_inputs():
    _rng = _Rng(jax.random.key(int.from_bytes(__import__("os").urandom(4), "little")))
    _w = (lambda a: (lambda t: t.astype(jnp.bfloat16) if jnp.issubdtype(t.dtype, jnp.floating) else t)(jnp.asarray(a)))
    def _A_setup():
        B, S, D = 1, 2048, 640
        ks = 4
        return {
            "q": _w((lambda *s: _rng.normal(s) * 0.05)(B, S, D)),
            "k": _w((lambda *s: _rng.normal(s) * 0.05)(B, S, D)),
            "v": _w((lambda *s: _rng.normal(s) * 0.05)(B, S, D)),
            "shift_k": _w((lambda *s: _rng.normal(s) * 0.05)(D, ks) * 0.5),
            "ssm_k": _w((lambda *s: _rng.normal(s) * 0.05)(D, S) * (1.0 / S ** 0.5)),
            "ssm_D": _w((lambda *s: _rng.normal(s) * 0.05)(D)),
        }
    _A_in = _A_setup()

    def _B_setup():
        B, S, D, F = 1, 2048, 640, 1728
        return {
            "x": _w((lambda *s: _rng.normal(s) * 0.05)(B, S, D)),
            "w1": _w((lambda *s: _rng.normal(s) * 0.05)(D, F) * (D ** -0.5)),
            "b1": _w((lambda *s: _rng.normal(s) * 0.05)(F) * 0.01),
            "w2": _w((lambda *s: _rng.normal(s) * 0.05)(F, D) * (F ** -0.5)),
            "b2": _w((lambda *s: _rng.normal(s) * 0.05)(D) * 0.01),
        }
    _B_in = _B_setup()

    return {
        "A_q": _A_in["q"],
        "A_k": _A_in["k"],
        "A_v": _A_in["v"],
        "A_shift_k": _A_in["shift_k"],
        "A_ssm_k": _A_in["ssm_k"],
        "A_ssm_D": _A_in["ssm_D"],
        "B_x": _B_in["x"],
        "B_w1": _B_in["w1"],
        "B_b1": _B_in["b1"],
        "B_w2": _B_in["w2"],
        "B_b2": _B_in["b2"],
    }

def reference(A_q, A_k, A_v, A_shift_k, A_ssm_k, A_ssm_D, B_x, B_w1, B_b1, B_w2, B_b2):
    def _A_ref(q, k, v, shift_k, ssm_k, ssm_D):
        B, S, D = q.shape
        ks = shift_k.shape[-1]
        k_pad = jnp.pad(k, ((0, 0), (ks - 1, 0), (0, 0)))
        k_shift = jnp.zeros_like(k)
        for t in range(ks):
            k_shift = k_shift + k_pad[:, t:t + S, :] * shift_k[:, ks - 1 - t][None, None, :]
        kv = k_shift * v
        L = 2 * S
        kv_pad = jnp.pad(kv, ((0, 0), (0, S), (0, 0)))
        kf_pad = jnp.pad(ssm_k, ((0, 0), (0, S)))
        kv_f = (lambda x, axes=(-2,-1): jnp.fft.rfft2(x.astype(jnp.float32), axes=axes))(kv_pad[:, None, :, :], axes=(1, 2))
        kf_f = (lambda x, axes=(-2,-1): jnp.fft.rfft2(x.astype(jnp.float32), axes=axes))(kf_pad[:, None, :], axes=(1, 2))
        kf_f = (lambda x, *d: x.transpose(*d))(kf_f, 1, 2, 0)
        y_f = kv_f * kf_f[None, :, :, :]
        y = (lambda x, s, axes=(-2,-1): jnp.fft.irfft2(x, s=s, axes=axes).astype(jnp.bfloat16))(y_f, (1, L), axes=(1, 2))[:, 0, :S, :]
        y = y + kv * ssm_D[None, None, :]
        return q * y

    def _B_ref(x, w1, b1, w2, b2):
        h = jnp.einsum("bsd,df->bsf", x, w1) + b1
        h = _gelu(h)
        return jnp.einsum("bsf,fd->bsd", h, w2) + b2

    x = A_q
    xn = _layernorm(x, axis=-1)
    return x + _A_ref(xn, A_k, A_v, A_shift_k, A_ssm_k, A_ssm_D) + _B_ref(xn, B_w1, B_b1, B_w2, B_b2)
```

```python
import functools
import numpy as np
import jax, jax.numpy as jnp
from jax import lax
import jax.experimental.pallas as pl
import jax.experimental.pallas.tpu as pltpu

S, D, F = 2048, 640, 1728
P = 128
NB = S // P
NL = D // 128
f32, bf16 = jnp.float32, jnp.bfloat16

def dft_mats():
    ks = np.concatenate([np.arange(0, 128, 2), np.arange(1, 128, 2)])
    n = np.arange(128)
    fw = np.zeros((256, 128)); inv = np.zeros((128, 256))
    for p in range(16):
        for s in range(8):
            k = ks[8 * p + s]
            w = 2 * np.pi * (k + 0.5) / 256
            fw[16 * p + s] = np.cos(w * n)
            fw[16 * p + 8 + s] = -np.sin(w * n)
            inv[:, 16 * p + s] = np.cos(w * n) / 128
            inv[:, 16 * p + 8 + s] = -np.sin(w * n) / 128
    return fw, inv

def gelu(h):
    c1 = 0.7978845608028654
    c2 = c1 * 0.044715
    u = h * (c1 + c2 * (h * h))
    hh = 0.5 * h
    return hh + hh * jnp.tanh(u)

def make(M0=320, M=288, name="v4", kvn=2, w1c=(0, F), w2c=(0, F), MLA=None):
    ML = S - M0 - NL * M
    assert ML > 0 and ML % 16 == 0 and ML <= M
    R = [0, M0] + [M0 + (i + 1) * M for i in range(NL)] + [S]
    n1, n2 = len(w1c) - 1, len(w2c) - 1
    SEM_Q, SEM_K, SEM_V, SEM_H, SEM_W1, SEM_W2, SEM_O = 0, 7, 12, 17, 22, 22 + n1, 22 + n1 + n2
    NSEM = SEM_O + 4

    def kernel(q_hbm, k_hbm, v_hbm, sk_ref, h_hbm, dd_ref, w1_hbm, b1_ref, w2_hbm, b2_ref, fw_ref, inv_ref,
               out_hbm,
               q_s, k_s, v_s, h_s, w1_s, w2_s, xn_s, p_s, x_s, hf_s, yp_s, o_s, par_s, flag_s, sem):
        def cp(src, dst, i):
            return pltpu.make_async_copy(src, dst, sem.at[i])
        def cq(t, r0, m): return cp(q_hbm.at[pl.ds(r0, m)], q_s.at[pl.ds(r0, m)], SEM_Q + t)
        def cw1(i): return cp(w1_hbm.at[pl.ds(w1c[i], w1c[i + 1] - w1c[i])], w1_s.at[pl.ds(w1c[i], w1c[i + 1] - w1c[i])], SEM_W1 + i)
        def cw2(i): return cp(w2_hbm.at[pl.ds(w2c[i], w2c[i + 1] - w2c[i])], w2_s.at[pl.ds(w2c[i], w2c[i + 1] - w2c[i])], SEM_W2 + i)
        def lane(j): return pl.ds(j * 128, 128) if isinstance(j, int) else pl.ds(pl.multiple_of(j * 128, 128), 128)
        def ck(j): return cp(k_hbm.at[:, lane(j)], k_s.at[j], SEM_K + j)
        def cv(j): return cp(v_hbm.at[:, lane(j)], v_s.at[j], SEM_V + j)
        def ch(j): return cp(h_hbm.at[lane(j), :], h_s.at[j], SEM_H + j)

        cq(0, 0, M0).start()
        for i in range(n1): cw1(i).start()
        for i in range(n2): cw2(i).start()
        cq(1, M0, M).start()
        ck(0).start(); cv(0).start(); ch(0).start()

        skf = sk_ref[...].astype(f32)
        ddf = dd_ref[...].astype(f32).reshape(1, D)
        par = jnp.concatenate([skf, ddf, jnp.zeros((3, D), f32)], axis=0)
        for j in range(NL):
            par_s[j] = par[:, j * 128:(j + 1) * 128]
        flag_s[0] = 100

        row8 = lax.broadcasted_iota(jnp.int32, (8, 128), 0)
        def false_mask():
            return row8 > flag_s[0]

        def ln(r0, m, chain=True):
            fm = lax.broadcasted_iota(jnp.int32, (16, 1), 0) > flag_s[0]
            last = None
            for t in range(m // 16):
                rr = r0 + 16 * t
                if not isinstance(rr, int): rr = pl.multiple_of(rr, 16)
                x = q_s[pl.ds(rr, 16), :].astype(f32)
                sm = jnp.sum(x, axis=-1, keepdims=True)
                if last is not None and chain:
                    sm = jnp.where(fm, last, sm)
                xc = x - sm * (1.0 / D)
                var = jnp.sum(xc * xc, axis=-1, keepdims=True) * (1.0 / D)
                rs = lax.rsqrt(var + 1e-5)
                last = rs
                xn_s[pl.ds(rr, 16), :] = (xc * rs).astype(bf16)

        def mm1(r0, m, f0=0, f1=F):
            xn = xn_s[pl.ds(r0, m), :]
            b1 = b1_ref[...].astype(f32).reshape(1, F)[:, f0:f1]
            h = lax.dot_general(xn, w1_s[f0:f1, :], (((1,), (1,)), ((), ())), preferred_element_type=f32) + b1
            return gelu(h).astype(bf16)

        def mm2_fin(r0, m, o):
            b2 = b2_ref[...].astype(f32).reshape(1, D)
            p_s[pl.ds(r0, m), :] = o + b2 + q_s[pl.ds(r0, m), :].astype(f32)

        def mlp(r0, m):
            h = mm1(r0, m)
            mm2_fin(r0, m, jnp.dot(h, w2_s[...], preferred_element_type=f32))

        def kv_fwd(j):
            sk = par_s[j]
            s = [jnp.broadcast_to(sk[l:l + 1, :], (8, 128)) for l in range(4)]
            dd = sk[4:5, :]
            fm = false_mask()
            masks = [row8 < l for l in range(4)]
            prev = [jnp.zeros((8, 128), f32)] * 4
            lasts = [None] * kvn
            fw = fw_ref[...]
            for a in range(NB):
                outs = []
                for t in range(a * 8, a * 8 + 8):
                    kb = k_s[j, 16 * t:16 * t + 16, :].astype(f32)
                    vb = v_s[j, 16 * t:16 * t + 16, :].astype(f32)
                    for hh in range(2):
                        k8 = kb[8 * hh:8 * hh + 8, :]
                        ci = (2 * t + hh) % kvn
                        if lasts[ci] is not None:
                            k8 = jnp.where(fm, lasts[ci], k8)
                        rl = [None] + [pltpu.roll(k8, l, 0) for l in range(1, 4)]
                        acc = k8 * s[0]
                        for l in range(1, 4):
                            acc = acc + jnp.where(masks[l], prev[l], rl[l]) * s[l]
                        prev = rl
                        o = acc * vb[8 * hh:8 * hh + 8, :]
                        lasts[ci] = o
                        outs.append(o)
                kv = jnp.concatenate(outs, axis=0).astype(bf16)
                hb = lax.dot_general(fw, h_s[j, :, a * P:(a + 1) * P], (((1,), (1,)), ((), ())),
                                     preferred_element_type=f32)
                if a == 0:
                    hb = jnp.concatenate([hb[8 * t:8 * t + 8, :] + dd if t % 2 == 0 else hb[8 * t:8 * t + 8, :] for t in range(32)], axis=0)
                hf_s[a] = hb
                x_s[a] = jnp.dot(fw, kv, preferred_element_type=f32)

        def conv_mac():
            fm = false_mask()
            last = None
            Y = [[None] * 16 for _ in range(NB)]
            for p in range(16):
                r0, i0 = 16 * p, 16 * p + 8
                prev = None
                for c in range(NB):
                    accr = acci = None
                    for a in range(c + 1):
                        b = c - a
                        xr = x_s[a, r0:r0 + 8, :]; xi = x_s[a, i0:i0 + 8, :]
                        hr = hf_s[b, r0:r0 + 8, :]; hi = hf_s[b, i0:i0 + 8, :]
                        if accr is None:
                            t1 = xr * hr; t2 = xr * hi
                            if last is not None:
                                t1 = jnp.where(fm, last[0], t1); t2 = jnp.where(fm, last[1], t2)
                            accr = t1 - xi * hi
                            acci = t2 + xi * hr
                        else:
                            accr = (accr + xr * hr) - xi * hi
                            acci = (acci + xr * hi) + xi * hr
                    last = (accr, acci)
                    if prev is None:
                        yr, yi = accr, acci
                    else:
                        pr, pi = prev
                        yr, yi = (accr - pi, acci + pr) if p < 8 else (accr + pi, acci - pr)
                    prev = (accr, acci)
                    Y[c][p] = jnp.concatenate([yr, yi], axis=0)
            return Y

        def conv_inv(j, Y):
            inv = inv_ref[...]
            for c in range(NB):
                yc = jnp.concatenate(Y[c], axis=0).astype(bf16)
                yp_s[j, c * P:(c + 1) * P, :] = jnp.dot(inv, yc, preferred_element_type=f32)

        def combine(r0, m):
            for j in range(NL):
                xn = xn_s[pl.ds(r0, m), j * 128:(j + 1) * 128].astype(f32)
                o_s[pl.ds(r0, m), j * 128:(j + 1) * 128] = (
                    p_s[pl.ds(r0, m), j * 128:(j + 1) * 128] + xn * yp_s[j, pl.ds(r0, m), :]).astype(bf16)

        cq(0, 0, M0).wait()
        ln(0, M0, False)
        hs = []
        for i in range(n1):
            cw1(i).wait()
            hs.append(mm1(0, M0, w1c[i], w1c[i + 1]))
        h = jnp.concatenate(hs, axis=1) if n1 > 1 else hs[0]
        o = None
        for i in range(n2):
            cw2(i).wait()
            oi = jnp.dot(h[:, w2c[i]:w2c[i + 1]], w2_s[w2c[i]:w2c[i + 1], :], preferred_element_type=f32)
            o = oi if o is None else o + oi
        cq(1, M0, M).wait()
        ck(0).wait(); cv(0).wait(); ch(0).wait()
        cq(2, R[2], M).start()
        ck(1).start(); cv(1).start(); ch(1).start()
        mm2_fin(0, M0, o)
        kv_fwd(0)
        ln(M0, M)

        def body(i, carry):
            r0 = pl.multiple_of(M0 + i * M, 16)
            rn = pl.multiple_of(r0 + M, 16)
            cq(i + 2, rn, M).wait()
            ck(i + 1).wait(); cv(i + 1).wait(); ch(i + 1).wait()
            @pl.when(i < NL - 2)
            def _():
                cq(i + 3, pl.multiple_of(rn + M, 16), M).start()
                ck(i + 2).start(); cv(i + 2).start(); ch(i + 2).start()
            @pl.when(i == NL - 2)
            def _():
                cq(6, R[6], ML).start()
            Y = conv_mac()
            mlp(r0, M)
            conv_inv(i, Y)
            kv_fwd(i + 1)
            ln(rn, M)
            return carry
        lax.fori_loop(0, NL - 1, body, 0)
        cq(6, R[6], ML).wait()
        Y = conv_mac()
        mlp(R[5], M)
        conv_inv(NL - 1, Y)
        ln(R[6], ML)
        rl = R[6]
        combine(0, rl)
        co1 = cp(o_s.at[pl.ds(0, rl)], out_hbm.at[pl.ds(0, rl)], SEM_O); co1.start()
        mlp(rl, ML)
        combine(rl, ML)
        co2 = cp(o_s.at[pl.ds(rl, ML)], out_hbm.at[pl.ds(rl, ML)], SEM_O + 1); co2.start()
        co1.wait(); co2.wait()

    fw, inv = dft_mats()
    @jax.jit
    def f(q, k, v, sk, h, dd, w1, b1, w2, b2):
        any_ = pl.BlockSpec(memory_space=pl.ANY)
        vm = pl.BlockSpec(memory_space=pltpu.VMEM)
        out = pl.pallas_call(
            kernel,
            in_specs=[any_, any_, any_, vm, any_, vm, any_, vm, any_, vm, vm, vm],
            out_specs=any_,
            out_shape=jax.ShapeDtypeStruct((S, D), bf16),
            scratch_shapes=[
                pltpu.VMEM((S, D), bf16),
                pltpu.VMEM((NL, S, 128), bf16),
                pltpu.VMEM((NL, S, 128), bf16),
                pltpu.VMEM((NL, 128, S), bf16),
                pltpu.VMEM((F, D), bf16),
                pltpu.VMEM((F, D), bf16),
                pltpu.VMEM((S, D), bf16),
                pltpu.VMEM((S, D), f32),
                pltpu.VMEM((NB, 256, 128), f32),
                pltpu.VMEM((NB, 256, 128), f32),
                pltpu.VMEM((NL, S, 128), f32),
                pltpu.VMEM((S, D), bf16),
                pltpu.VMEM((NL, 8, 128), f32),
                pltpu.SMEM((8,), jnp.int32),
                pltpu.SemaphoreType.DMA((NSEM,)),
            ],
            compiler_params=pltpu.CompilerParams(vmem_limit_bytes=100 * 2**20),
            name=name,
        )(q.reshape(S, D), k.reshape(S, D), v.reshape(S, D), sk.T, h, dd, w1.T, b1, w2, b2,
          jnp.asarray(fw, bf16), jnp.asarray(inv, bf16))
        return out.reshape(1, S, D)
    return f


_impl = make()


@jax.jit
def pallas_parallel_sum__ssm_conv_h3__dense_activation_gelu__prompt_kernel(
    A_q, A_k, A_v, A_shift_k, A_ssm_k, A_ssm_D, B_x, B_w1, B_b1, B_w2, B_b2,
):
    del B_x
    return _impl(A_q, A_k, A_v, A_shift_k, A_ssm_k, A_ssm_D, B_w1, B_b1, B_w2, B_b2)
```

```python
import functools
import numpy as np
import jax, jax.numpy as jnp
from jax import lax
import jax.experimental.pallas as pl
import jax.experimental.pallas.tpu as pltpu

S, D, F = 2048, 640, 1728
P = 128
NB = S // P
NL = D // 128
f32, bf16, u32 = jnp.float32, jnp.bfloat16, jnp.uint32
KP = 16

def dft_mats():
    ks = np.concatenate([np.arange(0, 128, 2), np.arange(1, 128, 2)])
    n = np.arange(128)
    m = np.arange(64) + 0.5
    fw = np.zeros((2, 256, 128)); inv = np.zeros((2, 64, 128))
    for p in range(16):
        for s in range(8):
            k = ks[8 * p + s]
            w = 2 * np.pi * (k + 0.5) / 256
            fw[0, 16 * p + s] = np.cos(w * (n - 63.5))
            fw[0, 16 * p + 8 + s] = -np.sin(w * (n - 63.5))
            fw[1, 16 * p + s] = np.cos(w * n)
            fw[1, 16 * p + 8 + s] = -np.sin(w * n)
            inv[0, :, 8 * p + s] = np.cos(w * m) / 128
            inv[1, :, 8 * p + s] = np.sin(w * m) / 128
    perm = np.concatenate([16 * t + np.concatenate([np.arange(0, 16, 2), np.arange(1, 16, 2)]) for t in range(8)])
    fw[0] = fw[0][:, perm]
    return fw, inv

def gelu(h):
    c1 = 0.7978845608028654
    c2 = c1 * 0.044715
    u = h * (c1 + c2 * (h * h))
    hh = 0.5 * h
    return hh + hh * jnp.tanh(u)

def make(M0=416, M=288, name="v12", kvn=2, w1c=(0, 256, 768, F), w2c=(0, 1024, F), cn=3, fsplit=1024, osplit=512, kvn0=2, q0a=192, lnn=2, lnlink=False, pins=(3, 6, 9, 12), osp=4, cn5=1, cn6=2, plink=15, plink5=8, static=False, lnlow=False, isplit=0):
    ML = S - M0 - NL * M
    assert ML > 0 and ML % 16 == 0 and ML <= M
    R = [0, M0] + [M0 + (i + 1) * M for i in range(NL)] + [S]
    n1, n2 = len(w1c) - 1, len(w2c) - 1
    SW1 = 2; SW2 = SW1 + n1; SG = SW2 + n2; SO = SG + 5
    NSEM = SO + len(pins) + 2
    HM = max(M0, ML)

    def kernel(q_hbm, k_hbm, v_hbm, sk_hbm, h_hbm, dd_hbm, w1_hbm, b1_hbm, w2_hbm, b2_hbm, fw_hbm, inv_hbm,
               out_hbm,
               q_s, k_s, v_s, h_s, w1_s, w2_s, xn_s, p_s, x_s, hf_s, yp_s, o_s, par_s, hid_s,
               sk_ref, dd_ref, b1_ref, b2_ref, fw_ref, inv_ref, flag_s, sem):
        def cp(src, dst, i):
            return pltpu.make_async_copy(src, dst, sem.at[i])
        def cq(r0, m, si): return cp(q_hbm.at[pl.ds(r0, m)], q_s.at[pl.ds(r0, m)], si)
        def cw(hbm, s_, c, i, si): return cp(hbm.at[pl.ds(c[i], c[i + 1] - c[i])], s_.at[pl.ds(c[i], c[i + 1] - c[i])], si)
        def lane(j): return pl.ds(j * 128, 128) if isinstance(j, int) else pl.ds(pl.multiple_of(j * 128, 128), 128)
        def ckvh(j, si):
            return [cp(h_hbm.at[lane(j), :], h_s.at[j], si), cp(k_hbm.at[:, lane(j)], k_s.at[j, pl.ds(KP, S), :], si),
                    cp(v_hbm.at[:, lane(j)], v_s.at[j], si)]
        g_q0a = [cq(0, q0a, 0)]
        g_q0b = [cq(q0a, M0 - q0a, 1)]
        g_w1 = [[cw(w1_hbm, w1_s, w1c, i, SW1 + i)] for i in range(n1)]
        g_w1[0].append(cp(b1_hbm, b1_ref, SW1))
        g_w2 = [[cw(w2_hbm, w2_s, w2c, i, SW2 + i)] for i in range(n2)]
        g_w2[0] = [cq(M0, M, SW2)] + g_w2[0]
        g_w2[-1] = g_w2[-1] + [cp(b2_hbm, b2_ref, SW2 + n2 - 1), cp(sk_hbm, sk_ref, SW2 + n2 - 1), cp(dd_hbm, dd_ref, SW2 + n2 - 1),
                               cp(fw_hbm, fw_ref, SW2 + n2 - 1), cp(inv_hbm, inv_ref, SW2 + n2 - 1)] + ckvh(0, SW2 + n2 - 1)
        def g_step(i):
            r = R[i + 2] if isinstance(i, int) else pl.multiple_of(M0 + (i + 1) * M, 16)
            return [cq(r, M, SG + i)] + ckvh(i + 1, SG + i)
        g_last = [cq(R[6], ML, SG + 4)]
        for g in [g_q0a, g_q0b] + g_w1 + g_w2 + [g_step(i) for i in range(NL - 1)] + [g_last]:
            for c in g: c.start()
        def wait(g):
            for c in g: c.wait()

        flag_s[0] = 100
        flag_s[1] = 0
        flag_s[2] = 0
        for j in range(NL):
            k_s[j, 0:KP, :] = jnp.zeros((KP, 128), bf16)
        ku_s = k_s.bitcast(u32); vu_s = v_s.bitcast(u32)
        def region(fn):
            pl.when(flag_s[0] == 100)(fn)

        row8 = lax.broadcasted_iota(jnp.int32, (8, 128), 0)
        def false_mask():
            return row8 > flag_s[0]

        def ln(r0, m, n=1):
            fm = lax.broadcasted_iota(jnp.int32, (16, 1), 0) > flag_s[0]
            lasts = [None] * max(n, 1)
            for t in range(m // 16):
                rr = r0 + 16 * t
                if not isinstance(rr, int): rr = pl.multiple_of(rr, 16)
                x = q_s[pl.ds(rr, 16), :].astype(f32)
                low = lnlow and n
                sm = jnp.sum(x, axis=-1, keepdims=True)
                ci = t % max(n, 1)
                if lasts[ci] is not None and n:
                    sm = jnp.where(fm, lasts[ci], sm)
                mu = sm * (1.0 / D)
                if low: x = q_s[pl.ds(pl.multiple_of(rr + flag_s[1], 16), 16), :].astype(f32)
                xc = x - mu
                var = jnp.sum(xc * xc, axis=-1, keepdims=True) * (1.0 / D)
                rs = lax.rsqrt(var + 1e-5)
                lasts[ci] = rs
                if low: xc = q_s[pl.ds(pl.multiple_of(rr + flag_s[2], 16), 16), :].astype(f32) - mu
                xo = xc * rs
                for j in range(NL):
                    xn_s[j, pl.ds(rr, 16), :] = xo[:, j * 128:(j + 1) * 128].astype(bf16)
            return lasts

        def load_xn(r0, m):
            return jnp.concatenate([xn_s[j, pl.ds(r0, m), :] for j in range(NL)], axis=1)

        def mm1(r0, m, f0=0, f1=F, xn=None, pin=None):
            if xn is None:
                xn = load_xn(r0, m)
            b1 = b1_ref[...].astype(f32).reshape(1, F)[:, f0:f1]
            if pin is not None:
                b1 = jnp.where(false_mask()[0:1, :f1 - f0], pin[0:1, :f1 - f0], b1)
            h = lax.dot_general(xn, w1_s[f0:f1, :], (((1,), (1,)), ((), ())), preferred_element_type=f32) + b1
            return gelu(h).astype(bf16)

        def mm2_fin(r0, m, o):
            b2 = b2_ref[...].astype(f32).reshape(1, D)
            p_s[pl.ds(r0, m), :] = o + b2 + q_s[pl.ds(r0, m), :].astype(f32)

        def mlp(r0, m, xn=None):
            h = mm1(r0, m, xn=xn)
            mm2_fin(r0, m, jnp.dot(h, w2_s[...], preferred_element_type=f32))

        def kv_fwd(j, sk, kvn=kvn, hfirst=False):
            s = [jnp.broadcast_to(sk[l:l + 1, :], (8, 128)) for l in range(4)]
            dd = sk[4:5, :]
            fm = false_mask()
            lasts = [None] * kvn
            fwx = fw_ref[0]; fwh = fw_ref[1]
            ev = lambda w: pltpu.bitcast(w << 16, f32)
            od = lambda w: pltpu.bitcast(w & jnp.uint32(0xffff0000), f32)
            kvs = []
            for a in range(NB):
                outs = []
                for t in range(a * 8, a * 8 + 8):
                    bb = KP // 2 + 8 * t
                    w0 = ku_s[j, bb:bb + 8, :]; w1 = ku_s[j, bb - 1:bb + 7, :]; w2 = ku_s[j, bb - 2:bb + 6, :]
                    wv = vu_s[j, 8 * t:8 * t + 8, :]
                    e0, o0, e1, o1, o2 = ev(w0), od(w0), ev(w1), od(w1), od(w2)
                    ci = t % kvn
                    if lasts[ci] is not None:
                        e0 = jnp.where(fm, lasts[ci], e0)
                    oe = (e0 * s[0] + o1 * s[1] + e1 * s[2] + o2 * s[3]) * ev(wv)
                    oo = (e0 * s[1] + o0 * s[0] + o1 * s[2] + e1 * s[3]) * od(wv)
                    lasts[ci] = oo
                    outs += [oe, oo]
                kv = jnp.concatenate(outs, axis=0).astype(bf16)
                hb = lax.dot_general(fwh, h_s[j, :, a * P:(a + 1) * P], (((1,), (1,)), ((), ())),
                                     preferred_element_type=f32)
                if a == 0:
                    hb = jnp.concatenate([hb[8 * t:8 * t + 8, :] + dd if t % 2 == 0 else hb[8 * t:8 * t + 8, :] for t in range(32)], axis=0)
                hf_s[a] = hb
                if hfirst:
                    kvs.append(kv)
                else:
                    x_s[a] = jnp.dot(fwx, kv, preferred_element_type=f32)
            for a, kv in enumerate(kvs):
                x_s[a] = jnp.dot(fwx, kv, preferred_element_type=f32)

        def conv_mac(link=None, plink=plink):
            fm = false_mask()
            last = None
            if link is not None:
                t = link[0]
                for u in link[1:]:
                    t = t + u
                link = jnp.broadcast_to(t[0:8, :], (8, 128))
            Y = [[None] * 16 for _ in range(NB)]
            for p in range(16):
                r0, i0 = 16 * p, 16 * p + 8
                prev = None
                for c in range(NB):
                    accr = acci = None
                    for a in range(c + 1):
                        b = c - a
                        xr = x_s[a, r0:r0 + 8, :]; xi = x_s[a, i0:i0 + 8, :]
                        hr = hf_s[b, r0:r0 + 8, :]; hi = hf_s[b, i0:i0 + 8, :]
                        if link is not None and p == plink and c == 0:
                            xi = jnp.where(fm, link, xi)
                        if accr is None:
                            t1 = xr * hr; t2 = xr * hi
                            if last is not None:
                                t1 = jnp.where(fm, last[0], t1); t2 = jnp.where(fm, last[1], t2)
                            accr = t1 - xi * hi
                            acci = t2 + xi * hr
                        else:
                            accr = (accr + xr * hr) - xi * hi
                            acci = (acci + xr * hi) + xi * hr
                    last = (accr, acci)
                    if prev is None:
                        yr, yi = accr, acci
                    else:
                        pr, pi = prev
                        yr, yi = (accr - pi, acci + pr) if p < 8 else (accr + pi, acci - pr)
                    prev = (accr, acci)
                    Y[c][p] = (yr, yi)
            return Y

        def conv_inv(j, Y, cs=range(NB)):
            ic = inv_ref[0]; isn = inv_ref[1]
            for c in cs:
                yr = jnp.concatenate([y[0] for y in Y[c]], axis=0).astype(bf16)
                yi = jnp.concatenate([y[1] for y in Y[c]], axis=0).astype(bf16)
                e = jnp.dot(ic, yr, preferred_element_type=f32)
                o = jnp.dot(isn, yi, preferred_element_type=f32)
                yp_s[j, c * P + 64:(c + 1) * P, :] = e - o
                lo = e + o
                for i in range(8):
                    yp_s[j, c * P + 8 * (7 - i):c * P + 8 * (8 - i), :] = lo[8 * i:8 * i + 8, :]

        def mlp_conv(r0, m, xn, j, Y):
            if not isplit:
                mlp(r0, m, xn); conv_inv(j, Y); return
            h = mm1(r0, m, xn=xn)
            b2 = b2_ref[...].astype(f32).reshape(1, D)
            c4 = D - 128
            o = jnp.dot(h, w2_s[:, :c4], preferred_element_type=f32)
            p_s[pl.ds(r0, m), :c4] = o + b2[:, :c4] + q_s[pl.ds(r0, m), :c4].astype(f32)
            ks = [0, 256, 768, 1280, F] if isplit == 1 else [0, 768, 1280, F]
            ng = len(ks) - 1
            o = None
            for g in range(ng):
                og = jnp.dot(h[:, ks[g]:ks[g + 1]], w2_s[ks[g]:ks[g + 1], c4:], preferred_element_type=f32)
                o = og if o is None else o + og
                if isplit == 1:
                    conv_inv(j, Y, range(4 * g, 4 * g + 4))
                elif g > 0:
                    conv_inv(j, Y, range(8 * (g - 1), 8 * g))
            p_s[pl.ds(r0, m), c4:] = o + b2[:, c4:] + q_s[pl.ds(r0, m), c4:].astype(f32)

        rev8 = 7 - row8
        def load_y(j, t):
            y = yp_s[j, t:t + 8, :]
            if t % P < 64:
                y = jnp.take_along_axis(y, rev8, axis=0)
            return y

        def combine(items, n, lasts):
            fm = false_mask()
            for i, (t, j) in enumerate(items):
                cs = slice(j * 128, (j + 1) * 128)
                y0 = load_y(j, t); y1 = load_y(j, t + 8)
                ci = i % max(n, 1)
                if n and lasts[ci] is not None:
                    y0 = jnp.where(fm, lasts[ci], y0)
                y = jnp.concatenate([y0, y1], axis=0)
                r = (p_s[t:t + 16, cs] + xn_s[j, t:t + 16, :].astype(f32) * y).astype(bf16)
                lasts[ci] = r.astype(f32)[0:8, :]
                o_s[j, t:t + 16, :] = r

        wait(g_q0a)
        ln(0, q0a, 0)
        wait(g_q0b)
        ln(q0a, M0 - q0a, 0)
        for i in range(n1):
            wait(g_w1[i])
            def r1(i=i):
                hid_s[0:M0, w1c[i]:w1c[i + 1]] = mm1(0, M0, w1c[i], w1c[i + 1])
            region(r1)
        for i in range(n2):
            wait(g_w2[i])
            def r2(i=i):
                o = jnp.dot(hid_s[0:M0, w2c[i]:w2c[i + 1]], w2_s[w2c[i]:w2c[i + 1], :], preferred_element_type=f32)
                if i > 0:
                    o = o + p_s[0:M0, :]
                if i == 0:
                    ln(M0, M, 1)
                if i < n2 - 1:
                    p_s[0:M0, :] = o
                else:
                    mm2_fin(0, M0, o)
                    skf = sk_ref[...].astype(f32)
                    ddf = dd_ref[...].astype(f32).reshape(1, D)
                    par = jnp.concatenate([skf, ddf, jnp.zeros((3, D), f32)], axis=0)
                    for j in range(NL):
                        par_s[j] = par[:, j * 128:(j + 1) * 128]
                    kv_fwd(0, par[:, 0:128], kvn0)
            region(r2)

        def body(i, carry):
            r0 = M0 + i * M if isinstance(i, int) else pl.multiple_of(M0 + i * M, 16)
            rn = r0 + M if isinstance(i, int) else pl.multiple_of(r0 + M, 16)
            if not isinstance(i, int): wait(g_step(i))
            xn = load_xn(r0, M)
            lk = ln(rn, M, lnn)
            Y = conv_mac(lk if lnlink else None)
            mlp_conv(r0, M, xn, i, Y)
            kv_fwd(i + 1, par_s[i + 1])
            return carry
        if static:
            for i in range(NL - 1):
                wait(g_step(i))
                def fb(i=i):
                    body(i, 0)
                region(fb)
        else:
            lax.fori_loop(0, NL - 1, body, 0)
        wait(g_last)
        rl = R[6]
        r5 = R[5]
        def co(i, j, r0, r1):
            return cp(o_s.at[j, pl.ds(r0, r1 - r0), :], out_hbm.at[pl.ds(r0, r1 - r0), pl.ds(j * 128, 128)], SO + i)
        def f5():
            ln(rl, ML, lnn)
            Y = conv_mac()
            mlp_conv(r5, M, None, NL - 1, Y)
        region(f5)
        nco = len(pins)
        rows = [(rl // 16 * i // nco) * 16 for i in range(nco + 1)]
        g_o = [[co(i, j, rows[i], rows[i + 1]) for j in range(NL)] for i in range(nco)]
        g_fa = [co(nco, j, rl, S) for j in range(osp)]
        g_fb = [co(nco + 1, j, rl, S) for j in range(osp, NL)]
        def pin_after(g, i):
            for c in g: c.start()
            z1 = pl.multiple_of(S + flag_s[1], 16); z2 = pl.multiple_of(S + flag_s[2], 16)
            o_s[0, pl.ds(z1, 16), :] = jnp.full((16, 128), i, bf16)
            return o_s[0, pl.ds(z2, 16), :].astype(f32)
        def f6():
            xn = load_xn(rl, ML)
            st = [None] * max(cn6, 1)
            hs = []
            gi = 0
            for f in range(14):
                pin = None
                if gi < nco and pins[gi] == f:
                    combine([(t, j) for t in range(rows[gi], rows[gi + 1], 16) for j in range(NL)], cn6, st)
                    pin = pin_after(g_o[gi], gi)
                    gi += 1
                hs.append(mm1(rl, ML, 128 * f, min(128 * (f + 1), F), xn, pin))
            h = jnp.concatenate(hs, axis=1)
            b2 = b2_ref[...].astype(f32).reshape(1, D)
            for j in range(NL):
                cs = slice(j * 128, (j + 1) * 128)
                bj = b2[:, cs]
                if j == osp:
                    pin = pin_after(g_fa, nco)
                    bj = jnp.where(false_mask()[0:1, :], pin[0:1, :], bj)
                o = jnp.dot(h, w2_s[:, cs], preferred_element_type=f32) + bj + q_s[rl:S, cs].astype(f32)
                y = jnp.concatenate([load_y(j, t) for t in range(rl, S, 8)], axis=0)
                o_s[j, rl:S, :] = (o + xn_s[j, rl:S, :].astype(f32) * y).astype(bf16)
            if osp == NL:
                for c in g_fa: c.start()
        region(f6)
        for c in g_fb: c.start()
        for g in g_o: wait(g)
        wait(g_fa); wait(g_fb)

    fw, inv = dft_mats()
    @jax.jit
    def f(q, k, v, sk, h, dd, w1, b1, w2, b2):
        any_ = pl.BlockSpec(memory_space=pl.ANY)
        out = pl.pallas_call(
            kernel,
            in_specs=[any_] * 12,
            out_specs=any_,
            out_shape=jax.ShapeDtypeStruct((S, D), bf16),
            scratch_shapes=[
                pltpu.VMEM((S, D), bf16),
                pltpu.VMEM((NL, S + KP, 128), bf16),
                pltpu.VMEM((NL, S, 128), bf16),
                pltpu.VMEM((NL, 128, S), bf16),
                pltpu.VMEM((F, D), bf16),
                pltpu.VMEM((F, D), bf16),
                pltpu.VMEM((NL, S, 128), bf16),
                pltpu.VMEM((S, D), f32),
                pltpu.VMEM((NB, 256, 128), f32),
                pltpu.VMEM((NB, 256, 128), f32),
                pltpu.VMEM((NL, S, 128), f32),
                pltpu.VMEM((NL, S + 16, 128), bf16),
                pltpu.VMEM((NL, 8, 128), f32),
                pltpu.VMEM((HM, F), bf16),
                pltpu.VMEM((4, D), bf16), pltpu.VMEM((D,), bf16), pltpu.VMEM((F,), bf16), pltpu.VMEM((D,), bf16),
                pltpu.VMEM((2, 256, 128), bf16), pltpu.VMEM((2, 64, 128), bf16),
                pltpu.SMEM((8,), jnp.int32),
                pltpu.SemaphoreType.DMA((NSEM,)),
            ],
            compiler_params=pltpu.CompilerParams(vmem_limit_bytes=100 * 2**20),
            name=name,
        )(q.reshape(S, D), k.reshape(S, D), v.reshape(S, D), sk.T, h, dd, w1.T, b1, w2, b2,
          jnp.asarray(fw, bf16), jnp.asarray(inv, bf16))
        return out.reshape(1, S, D)
    return f


_impl = make()


@jax.jit
def pallas_parallel_sum__ssm_conv_h3__dense_activation_gelu__prompt_kernel(
    A_q, A_k, A_v, A_shift_k, A_ssm_k, A_ssm_D, B_x, B_w1, B_b1, B_w2, B_b2,
):
    del B_x
    return _impl(A_q, A_k, A_v, A_shift_k, A_ssm_k, A_ssm_D, B_w1, B_b1, B_w2, B_b2)
```

```python
import functools
import numpy as np
import jax, jax.numpy as jnp
from jax import lax
import jax.experimental.pallas as pl
import jax.experimental.pallas.tpu as pltpu

S, D, F = 2048, 640, 1728
P = 128
NB = S // P
NL = D // 128
f32, bf16, u32 = jnp.float32, jnp.bfloat16, jnp.uint32
KP = 16

def dft_mats():
    ks = np.concatenate([np.arange(0, 128, 2), np.arange(1, 128, 2)])
    n = np.arange(128)
    m = np.arange(64) + 0.5
    fw = np.zeros((2, 256, 128)); inv = np.zeros((2, 64, 128))
    for p in range(16):
        for s in range(8):
            k = ks[8 * p + s]
            w = 2 * np.pi * (k + 0.5) / 256
            fw[0, 16 * p + s] = np.cos(w * (n - 63.5))
            fw[0, 16 * p + 8 + s] = -np.sin(w * (n - 63.5))
            fw[1, 16 * p + s] = np.cos(w * n)
            fw[1, 16 * p + 8 + s] = -np.sin(w * n)
            inv[0, :, 8 * p + s] = np.cos(w * m) / 128
            inv[1, :, 8 * p + s] = np.sin(w * m) / 128
    perm = np.concatenate([16 * t + np.concatenate([np.arange(0, 16, 2), np.arange(1, 16, 2)]) for t in range(8)])
    fw[0] = fw[0][:, perm]
    return fw, inv

def gelu(h):
    c1 = 0.7978845608028654
    c2 = c1 * 0.044715
    u = h * (c1 + c2 * (h * h))
    hh = 0.5 * h
    return hh + hh * jnp.tanh(u)

def make(M0=416, M=288, name="v13", kvn=2, w1c=(0, 256, 768, F), w2c=(0, 1024, F), cn=3, fsplit=1024, osplit=512, kvn0=2, q0a=192, lnn=2, lnlink=False, pins=(1, 7, 12, 15), osp=4, prow=(0.03, 0.33, 0.66), elink=(15, 15), cn5=1, cn6=1, plink=15, plink5=8, static=False, lnlow=False, isplit=0):
    ML = S - M0 - NL * M
    assert ML > 0 and ML % 16 == 0 and ML <= M
    R = [0, M0] + [M0 + (i + 1) * M for i in range(NL)] + [S]
    n1, n2 = len(w1c) - 1, len(w2c) - 1
    SW1 = 2; SW2 = SW1 + n1; SG = SW2 + n2; SO = SG + 5
    NSEM = SO + len(pins) + 2
    HM = max(M0, ML)

    def kernel(q_hbm, k_hbm, v_hbm, sk_hbm, h_hbm, dd_hbm, w1_hbm, b1_hbm, w2_hbm, b2_hbm, fw_hbm, inv_hbm,
               out_hbm,
               q_s, k_s, v_s, h_s, w1_s, w2_s, xn_s, p_s, x_s, hf_s, yp_s, o_s, par_s, hid_s,
               sk_ref, dd_ref, b1_ref, b2_ref, fw_ref, inv_ref, flag_s, sem):
        def cp(src, dst, i):
            return pltpu.make_async_copy(src, dst, sem.at[i])
        def cq(r0, m, si): return cp(q_hbm.at[pl.ds(r0, m)], q_s.at[pl.ds(r0, m)], si)
        def cw(hbm, s_, c, i, si): return cp(hbm.at[pl.ds(c[i], c[i + 1] - c[i])], s_.at[pl.ds(c[i], c[i + 1] - c[i])], si)
        def lane(j): return pl.ds(j * 128, 128) if isinstance(j, int) else pl.ds(pl.multiple_of(j * 128, 128), 128)
        def ckvh(j, si):
            return [cp(h_hbm.at[lane(j), :], h_s.at[j], si), cp(k_hbm.at[:, lane(j)], k_s.at[j, pl.ds(KP, S), :], si),
                    cp(v_hbm.at[:, lane(j)], v_s.at[j], si)]
        g_q0a = [cq(0, q0a, 0)]
        g_q0b = [cq(q0a, M0 - q0a, 1)]
        g_w1 = [[cw(w1_hbm, w1_s, w1c, i, SW1 + i)] for i in range(n1)]
        g_w1[0].append(cp(b1_hbm, b1_ref, SW1))
        g_w2 = [[cw(w2_hbm, w2_s, w2c, i, SW2 + i)] for i in range(n2)]
        g_w2[0] = [cq(M0, M, SW2)] + g_w2[0]
        g_w2[-1] = g_w2[-1] + [cp(b2_hbm, b2_ref, SW2 + n2 - 1), cp(sk_hbm, sk_ref, SW2 + n2 - 1), cp(dd_hbm, dd_ref, SW2 + n2 - 1),
                               cp(fw_hbm, fw_ref, SW2 + n2 - 1), cp(inv_hbm, inv_ref, SW2 + n2 - 1)] + ckvh(0, SW2 + n2 - 1)
        def g_step(i):
            r = R[i + 2] if isinstance(i, int) else pl.multiple_of(M0 + (i + 1) * M, 16)
            return [cq(r, M, SG + i)] + ckvh(i + 1, SG + i)
        g_last = [cq(R[6], ML, SG + 4)]
        for g in [g_q0a, g_q0b] + g_w1 + g_w2 + [g_step(i) for i in range(NL - 1)] + [g_last]:
            for c in g: c.start()
        def wait(g):
            for c in g: c.wait()

        flag_s[0] = 100
        flag_s[1] = 0
        flag_s[2] = 0
        for j in range(NL):
            k_s[j, 0:KP, :] = jnp.zeros((KP, 128), bf16)
        ku_s = k_s.bitcast(u32); vu_s = v_s.bitcast(u32)
        def region(fn):
            pl.when(flag_s[0] == 100)(fn)

        row8 = lax.broadcasted_iota(jnp.int32, (8, 128), 0)
        def false_mask():
            return row8 > flag_s[0]

        def ln(r0, m, n=1):
            fm = lax.broadcasted_iota(jnp.int32, (16, 1), 0) > flag_s[0]
            lasts = [None] * max(n, 1)
            for t in range(m // 16):
                rr = r0 + 16 * t
                if not isinstance(rr, int): rr = pl.multiple_of(rr, 16)
                x = q_s[pl.ds(rr, 16), :].astype(f32)
                low = lnlow and n
                sm = jnp.sum(x, axis=-1, keepdims=True)
                ci = t % max(n, 1)
                if lasts[ci] is not None and n:
                    sm = jnp.where(fm, lasts[ci], sm)
                mu = sm * (1.0 / D)
                if low: x = q_s[pl.ds(pl.multiple_of(rr + flag_s[1], 16), 16), :].astype(f32)
                xc = x - mu
                var = jnp.sum(xc * xc, axis=-1, keepdims=True) * (1.0 / D)
                rs = lax.rsqrt(var + 1e-5)
                lasts[ci] = rs
                if low: xc = q_s[pl.ds(pl.multiple_of(rr + flag_s[2], 16), 16), :].astype(f32) - mu
                xo = xc * rs
                for j in range(NL):
                    xn_s[j, pl.ds(rr, 16), :] = xo[:, j * 128:(j + 1) * 128].astype(bf16)
            return lasts

        def load_xn(r0, m):
            return jnp.concatenate([xn_s[j, pl.ds(r0, m), :] for j in range(NL)], axis=1)

        def mm1(r0, m, f0=0, f1=F, xn=None, pin=None):
            if xn is None:
                xn = load_xn(r0, m)
            b1 = b1_ref[...].astype(f32).reshape(1, F)[:, f0:f1]
            if pin is not None:
                b1 = jnp.where(false_mask()[0:1, :f1 - f0], pin[0:1, :f1 - f0], b1)
            h = lax.dot_general(xn, w1_s[f0:f1, :], (((1,), (1,)), ((), ())), preferred_element_type=f32) + b1
            return gelu(h).astype(bf16)

        def mm2_fin(r0, m, o):
            b2 = b2_ref[...].astype(f32).reshape(1, D)
            p_s[pl.ds(r0, m), :] = o + b2 + q_s[pl.ds(r0, m), :].astype(f32)

        def mlp(r0, m, xn=None):
            h = mm1(r0, m, xn=xn)
            mm2_fin(r0, m, jnp.dot(h, w2_s[...], preferred_element_type=f32))

        def kv_fwd(j, sk, kvn=kvn, hfirst=False):
            s = [jnp.broadcast_to(sk[l:l + 1, :], (8, 128)) for l in range(4)]
            dd = sk[4:5, :]
            fm = false_mask()
            lasts = [None] * kvn
            fwx = fw_ref[0]; fwh = fw_ref[1]
            ev = lambda w: pltpu.bitcast(w << 16, f32)
            od = lambda w: pltpu.bitcast(w & jnp.uint32(0xffff0000), f32)
            kvs = []
            for a in range(NB):
                outs = []
                for t in range(a * 8, a * 8 + 8):
                    bb = KP // 2 + 8 * t
                    w0 = ku_s[j, bb:bb + 8, :]; w1 = ku_s[j, bb - 1:bb + 7, :]; w2 = ku_s[j, bb - 2:bb + 6, :]
                    wv = vu_s[j, 8 * t:8 * t + 8, :]
                    e0, o0, e1, o1, o2 = ev(w0), od(w0), ev(w1), od(w1), od(w2)
                    ci = t % kvn
                    if lasts[ci] is not None:
                        e0 = jnp.where(fm, lasts[ci], e0)
                    oe = (e0 * s[0] + o1 * s[1] + e1 * s[2] + o2 * s[3]) * ev(wv)
                    oo = (e0 * s[1] + o0 * s[0] + o1 * s[2] + e1 * s[3]) * od(wv)
                    lasts[ci] = oo
                    outs += [oe, oo]
                kv = jnp.concatenate(outs, axis=0).astype(bf16)
                hb = lax.dot_general(fwh, h_s[j, :, a * P:(a + 1) * P], (((1,), (1,)), ((), ())),
                                     preferred_element_type=f32)
                if a == 0:
                    hb = jnp.concatenate([hb[8 * t:8 * t + 8, :] + dd if t % 2 == 0 else hb[8 * t:8 * t + 8, :] for t in range(32)], axis=0)
                hf_s[a] = hb
                if hfirst:
                    kvs.append(kv)
                else:
                    x_s[a] = jnp.dot(fwx, kv, preferred_element_type=f32)
            for a, kv in enumerate(kvs):
                x_s[a] = jnp.dot(fwx, kv, preferred_element_type=f32)

        def conv_mac(link=None, plink=plink):
            fm = false_mask()
            last = None
            if link is not None:
                t = link[0]
                for u in link[1:]:
                    t = t + u
                link = jnp.broadcast_to(t[0:8, :], (8, 128))
            Y = [[None] * 16 for _ in range(NB)]
            for p in range(16):
                r0, i0 = 16 * p, 16 * p + 8
                prev = None
                for c in range(NB):
                    accr = acci = None
                    for a in range(c + 1):
                        b = c - a
                        xr = x_s[a, r0:r0 + 8, :]; xi = x_s[a, i0:i0 + 8, :]
                        hr = hf_s[b, r0:r0 + 8, :]; hi = hf_s[b, i0:i0 + 8, :]
                        if link is not None and p == plink and c == 0:
                            xi = jnp.where(fm, link, xi)
                        if accr is None:
                            t1 = xr * hr; t2 = xr * hi
                            if last is not None:
                                t1 = jnp.where(fm, last[0], t1); t2 = jnp.where(fm, last[1], t2)
                            accr = t1 - xi * hi
                            acci = t2 + xi * hr
                        else:
                            accr = (accr + xr * hr) - xi * hi
                            acci = (acci + xr * hi) + xi * hr
                    last = (accr, acci)
                    if prev is None:
                        yr, yi = accr, acci
                    else:
                        pr, pi = prev
                        yr, yi = (accr - pi, acci + pr) if p < 8 else (accr + pi, acci - pr)
                    prev = (accr, acci)
                    Y[c][p] = (yr, yi)
                    if elink is not None and (p, c) == tuple(elink):
                        Y.append(accr + acci)
            return Y

        def conv_inv(j, Y, cs=range(NB)):
            ic = inv_ref[0]; isn = inv_ref[1]
            for c in cs:
                yr = jnp.concatenate([y[0] for y in Y[c]], axis=0).astype(bf16)
                yi = jnp.concatenate([y[1] for y in Y[c]], axis=0).astype(bf16)
                e = jnp.dot(ic, yr, preferred_element_type=f32)
                o = jnp.dot(isn, yi, preferred_element_type=f32)
                yp_s[j, c * P + 64:(c + 1) * P, :] = e - o
                lo = e + o
                for i in range(8):
                    yp_s[j, c * P + 8 * (7 - i):c * P + 8 * (8 - i), :] = lo[8 * i:8 * i + 8, :]

        def mlp_conv(r0, m, xn, j, Y):
            if elink is not None:
                h = mm1(r0, m, xn=xn)
                b2 = b2_ref[...].astype(f32).reshape(1, D)
                c4 = D - 128
                o = jnp.dot(h, w2_s[:, :c4], preferred_element_type=f32)
                p_s[pl.ds(r0, m), :c4] = o + b2[:, :c4] + q_s[pl.ds(r0, m), :c4].astype(f32)
                bj = jnp.where(false_mask()[0:1, :], Y[NB][0:1, :], b2[:, c4:])
                o = jnp.dot(h, w2_s[:, c4:], preferred_element_type=f32)
                p_s[pl.ds(r0, m), c4:] = o + bj + q_s[pl.ds(r0, m), c4:].astype(f32)
                conv_inv(j, Y)
                return
            if not isplit:
                mlp(r0, m, xn); conv_inv(j, Y); return
            h = mm1(r0, m, xn=xn)
            b2 = b2_ref[...].astype(f32).reshape(1, D)
            c4 = D - 128
            o = jnp.dot(h, w2_s[:, :c4], preferred_element_type=f32)
            p_s[pl.ds(r0, m), :c4] = o + b2[:, :c4] + q_s[pl.ds(r0, m), :c4].astype(f32)
            ks = [0, 256, 768, 1280, F] if isplit == 1 else [0, 768, 1280, F]
            ng = len(ks) - 1
            o = None
            for g in range(ng):
                og = jnp.dot(h[:, ks[g]:ks[g + 1]], w2_s[ks[g]:ks[g + 1], c4:], preferred_element_type=f32)
                o = og if o is None else o + og
                if isplit == 1:
                    conv_inv(j, Y, range(4 * g, 4 * g + 4))
                elif g > 0:
                    conv_inv(j, Y, range(8 * (g - 1), 8 * g))
            p_s[pl.ds(r0, m), c4:] = o + b2[:, c4:] + q_s[pl.ds(r0, m), c4:].astype(f32)

        rev8 = 7 - row8
        def load_y(j, t):
            y = yp_s[j, t:t + 8, :]
            if t % P < 64:
                y = jnp.take_along_axis(y, rev8, axis=0)
            return y

        def combine(items, n, lasts):
            fm = false_mask()
            for i, (t, j) in enumerate(items):
                cs = slice(j * 128, (j + 1) * 128)
                y = jnp.concatenate([load_y(j, t), load_y(j, t + 8)], axis=0)
                p0 = p_s[t:t + 8, cs]
                ci = i % max(n, 1)
                if n and lasts[ci] is not None:
                    p0 = jnp.where(fm, lasts[ci], p0)
                pp = jnp.concatenate([p0, p_s[t + 8:t + 16, cs]], axis=0)
                r = (pp + xn_s[j, t:t + 16, :].astype(f32) * y).astype(bf16)
                lasts[ci] = r.astype(f32)[0:8, :]
                o_s[j, t:t + 16, :] = r

        wait(g_q0a)
        ln(0, q0a, 0)
        wait(g_q0b)
        ln(q0a, M0 - q0a, 0)
        for i in range(n1):
            wait(g_w1[i])
            def r1(i=i):
                hid_s[0:M0, w1c[i]:w1c[i + 1]] = mm1(0, M0, w1c[i], w1c[i + 1])
            region(r1)
        for i in range(n2):
            wait(g_w2[i])
            def r2(i=i):
                o = jnp.dot(hid_s[0:M0, w2c[i]:w2c[i + 1]], w2_s[w2c[i]:w2c[i + 1], :], preferred_element_type=f32)
                if i > 0:
                    o = o + p_s[0:M0, :]
                if i == 0:
                    ln(M0, M, 1)
                if i < n2 - 1:
                    p_s[0:M0, :] = o
                else:
                    mm2_fin(0, M0, o)
                    skf = sk_ref[...].astype(f32)
                    ddf = dd_ref[...].astype(f32).reshape(1, D)
                    par = jnp.concatenate([skf, ddf, jnp.zeros((3, D), f32)], axis=0)
                    for j in range(NL):
                        par_s[j] = par[:, j * 128:(j + 1) * 128]
                    kv_fwd(0, par[:, 0:128], kvn0)
            region(r2)

        def body(i, carry):
            r0 = M0 + i * M if isinstance(i, int) else pl.multiple_of(M0 + i * M, 16)
            rn = r0 + M if isinstance(i, int) else pl.multiple_of(r0 + M, 16)
            if not isinstance(i, int): wait(g_step(i))
            xn = load_xn(r0, M)
            lk = ln(rn, M, lnn)
            Y = conv_mac(lk if lnlink else None)
            mlp_conv(r0, M, xn, i, Y)
            kv_fwd(i + 1, par_s[i + 1])
            return carry
        if static:
            for i in range(NL - 1):
                wait(g_step(i))
                def fb(i=i):
                    body(i, 0)
                region(fb)
        else:
            lax.fori_loop(0, NL - 1, body, 0)
        wait(g_last)
        rl = R[6]
        r5 = R[5]
        def co(i, j, r0, r1):
            return cp(o_s.at[j, pl.ds(r0, r1 - r0), :], out_hbm.at[pl.ds(r0, r1 - r0), pl.ds(j * 128, 128)], SO + i)
        def f5():
            ln(rl, ML, lnn)
            Y = conv_mac()
            mlp_conv(r5, M, None, NL - 1, Y)
        region(f5)
        nco = len(pins)
        rows = [(rl // 16 * i // nco) * 16 for i in range(nco + 1)] if prow is None else [0] + [int(rl // 16 * x) * 16 for x in prow] + [rl]
        g_o = [[co(i, j, rows[i], rows[i + 1]) for j in range(NL)] for i in range(nco)]
        g_fa = [co(nco, j, rl, S) for j in range(osp)]
        g_fb = [co(nco + 1, j, rl, S) for j in range(osp, NL)]
        def pin_after(g, i):
            for c in g: c.start()
            z1 = pl.multiple_of(S + flag_s[1], 16); z2 = pl.multiple_of(S + flag_s[2], 16)
            o_s[0, pl.ds(z1, 16), :] = jnp.full((16, 128), i, bf16)
            return o_s[0, pl.ds(z2, 16), :].astype(f32)
        def f6():
            xn = load_xn(rl, ML)
            st = [None] * max(cn6, 1)
            hs = []
            gi = 0
            for f in range(14):
                pin = None
                if gi < nco and pins[gi] == f:
                    combine([(t, j) for t in range(rows[gi], rows[gi + 1], 16) for j in range(NL)], cn6, st)
                    pin = pin_after(g_o[gi], gi)
                    gi += 1
                hs.append(mm1(rl, ML, 128 * f, min(128 * (f + 1), F), xn, pin))
            h = jnp.concatenate(hs, axis=1)
            b2 = b2_ref[...].astype(f32).reshape(1, D)
            for j in range(NL):
                cs = slice(j * 128, (j + 1) * 128)
                bj = b2[:, cs]
                if gi < nco and pins[gi] == 14 + j:
                    combine([(t, jj) for t in range(rows[gi], rows[gi + 1], 16) for jj in range(NL)], cn6, st)
                    pin = pin_after(g_o[gi], gi)
                    bj = jnp.where(false_mask()[0:1, :], pin[0:1, :], bj)
                    gi += 1
                if j == osp:
                    pin = pin_after(g_fa, nco)
                    bj = jnp.where(false_mask()[0:1, :], pin[0:1, :], bj)
                o = jnp.dot(h, w2_s[:, cs], preferred_element_type=f32) + bj + q_s[rl:S, cs].astype(f32)
                y = jnp.concatenate([load_y(j, t) for t in range(rl, S, 8)], axis=0)
                o_s[j, rl:S, :] = (o + xn_s[j, rl:S, :].astype(f32) * y).astype(bf16)
            if osp == NL:
                for c in g_fa: c.start()
        region(f6)
        for c in g_fb: c.start()
        for g in g_o: wait(g)
        wait(g_fa); wait(g_fb)

    fw, inv = dft_mats()
    @jax.jit
    def f(q, k, v, sk, h, dd, w1, b1, w2, b2):
        any_ = pl.BlockSpec(memory_space=pl.ANY)
        out = pl.pallas_call(
            kernel,
            in_specs=[any_] * 12,
            out_specs=any_,
            out_shape=jax.ShapeDtypeStruct((S, D), bf16),
            scratch_shapes=[
                pltpu.VMEM((S, D), bf16),
                pltpu.VMEM((NL, S + KP, 128), bf16),
                pltpu.VMEM((NL, S, 128), bf16),
                pltpu.VMEM((NL, 128, S), bf16),
                pltpu.VMEM((F, D), bf16),
                pltpu.VMEM((F, D), bf16),
                pltpu.VMEM((NL, S, 128), bf16),
                pltpu.VMEM((S, D), f32),
                pltpu.VMEM((NB, 256, 128), f32),
                pltpu.VMEM((NB, 256, 128), f32),
                pltpu.VMEM((NL, S, 128), f32),
                pltpu.VMEM((NL, S + 16, 128), bf16),
                pltpu.VMEM((NL, 8, 128), f32),
                pltpu.VMEM((HM, F), bf16),
                pltpu.VMEM((4, D), bf16), pltpu.VMEM((D,), bf16), pltpu.VMEM((F,), bf16), pltpu.VMEM((D,), bf16),
                pltpu.VMEM((2, 256, 128), bf16), pltpu.VMEM((2, 64, 128), bf16),
                pltpu.SMEM((8,), jnp.int32),
                pltpu.SemaphoreType.DMA((NSEM,)),
            ],
            compiler_params=pltpu.CompilerParams(vmem_limit_bytes=100 * 2**20),
            name=name,
        )(q.reshape(S, D), k.reshape(S, D), v.reshape(S, D), sk.T, h, dd, w1.T, b1, w2, b2,
          jnp.asarray(fw, bf16), jnp.asarray(inv, bf16))
        return out.reshape(1, S, D)
    return f


_impl = make(lnn=1, w2c=(0, 1280, F))


@jax.jit
def pallas_parallel_sum__ssm_conv_h3__dense_activation_gelu__prompt_kernel(
    A_q, A_k, A_v, A_shift_k, A_ssm_k, A_ssm_D, B_x, B_w1, B_b1, B_w2, B_b2,
):
    del B_x
    return _impl(A_q, A_k, A_v, A_shift_k, A_ssm_k, A_ssm_D, B_w1, B_b1, B_w2, B_b2)
```

```python
import numpy as np
import jax
import jax.numpy as jnp
from jax import lax
import jax.experimental.pallas as pl
import jax.experimental.pallas.tpu as pltpu

S, D, F = 2048, 640, 1728
P = 128
NB = S // P
NL = D // 128
KP = 64
f32, bf16, u32 = jnp.float32, jnp.bfloat16, jnp.uint32


ALPHA = (0.7978845608028654 * 0.044715) ** (1.0 / 3.0)
C1 = 0.7978845608028654 / ALPHA
OSC = 0.5 / ALPHA


def dft_mats():
    ks = np.concatenate([np.arange(0, 128, 2), np.arange(1, 128, 2)])
    n = np.arange(128)
    m = np.arange(64) + 0.5
    fw = np.zeros((2, 256, 128))
    inv = np.zeros((2, 64, 128))
    for p in range(16):
        for s in range(8):
            w = 2 * np.pi * (ks[8 * p + s] + 0.5) / 256
            fw[0, 16 * p + s] = np.cos(w * (n - 63.5))
            fw[0, 16 * p + 8 + s] = -np.sin(w * (n - 63.5))
            fw[1, 16 * p + s] = np.cos(w * n)
            fw[1, 16 * p + 8 + s] = -np.sin(w * n)
            inv[0, :, 8 * p + s] = np.cos(w * m) / (128 * ALPHA)
            inv[1, :, 8 * p + s] = np.sin(w * m) / (128 * ALPHA)
    perm = np.concatenate(
        [16 * t + np.concatenate([np.arange(0, 16, 2), np.arange(1, 16, 2)]) for t in range(8)])
    fw[0] = fw[0][:, perm]
    return fw, inv


def gelu(g):
    return g * (1.0 + jnp.tanh(g * (C1 + g * g)))


def make(M0=416, M=288, name="v17", kvn=2, kvn0=2, w1c=(0, 256, 768, F), w2c=(0, 1280, F), q0a=192,
         lnn=1, pins=(1, 7, 12, 15), prow=(0.03, 0.33, 0.66), osp=4, lag=2, pitch=None, early=(99, 99, 99), rem=True, lk=0, pf=16, fm_=4, remlast=False, dbg=''):
    ML = S - M0 - NL * M
    assert ML > 0 and ML % 16 == 0
    R = [0, M0] + [M0 + (i + 1) * M for i in range(NL)] + [S]
    PITCH = pitch or -(-max(M0, M, ML) // 64) * 64
    SR = 7 * PITCH

    def srow(r):
        t = max(i for i in range(7) if R[i] <= r)
        return t * PITCH + r - R[t]

    n1, n2, nco = len(w1c) - 1, len(w2c) - 1, len(pins)
    SW1 = 2
    SW2 = SW1 + n1
    SG = SW2 + n2
    SO = SG + 5
    NSEM = SO + 1

    def kernel(q_hbm, k_hbm, v_hbm, sk_hbm, h_hbm, dd_hbm, w1_hbm, b1_hbm, w2_hbm, b2_hbm, fw_hbm, inv_hbm,
               out_hbm,
               q_s, k_s, v_s, h_s, w1_s, w2_s, xn_s, p_s, x_s, hf_s, yp_s, o_s, par_s, hid_s,
               sk_ref, dd_ref, b1_ref, b2_ref, fw_ref, inv_ref, bc_s, flag_s, sem):
        def cp(src, dst, i):
            return pltpu.make_async_copy(src, dst, sem.at[i])

        def cq(r, rs, m, si):
            return cp(q_hbm.at[pl.ds(r, m)], q_s.at[pl.ds(rs, m)], si)

        def cw(hbm, s_, c, i, si):
            rows = pl.ds(c[i], c[i + 1] - c[i])
            return cp(hbm.at[rows], s_.at[rows], si)

        def ckvh(j, si):
            lane = pl.ds(j * 128, 128) if isinstance(j, int) else pl.ds(pl.multiple_of(j * 128, 128), 128)
            return [cp(h_hbm.at[lane, :], h_s.at[j], si),
                    cp(k_hbm.at[:, lane], k_s.at[j, pl.ds(KP, S), :], si),
                    cp(v_hbm.at[:, lane], v_s.at[j], si)]

        g_q0a = [cq(0, 0, q0a, 0)]
        g_q0b = [cq(q0a, q0a, M0 - q0a, 1)]
        g_w1 = [[cw(w1_hbm, w1_s, w1c, i, SW1 + i)] for i in range(n1)]
        g_w1[0].append(cp(b1_hbm, b1_ref, SW1))
        g_w2 = [[cw(w2_hbm, w2_s, w2c, i, SW2 + i)] for i in range(n2)]
        g_w2[0] = [cq(M0, PITCH, M, SW2)] + g_w2[0]
        sl = SW2 + n2 - 1
        g_w2[-1] = g_w2[-1] + [cp(b2_hbm, b2_ref, sl), cp(sk_hbm, sk_ref, sl), cp(dd_hbm, dd_ref, sl),
                               cp(fw_hbm, fw_ref, sl), cp(inv_hbm, inv_ref, sl)] + ckvh(0, sl)

        def g_step(i):
            if isinstance(i, int):
                r, rs = R[i + 2], (i + 2) * PITCH
            else:
                r, rs = pl.multiple_of(M0 + (i + 1) * M, 16), pl.multiple_of((i + 2) * PITCH, 64)
            return [cq(r, rs, M, SG + i)] + ckvh(i + 1, SG + i)

        g_last = [cq(R[6], 6 * PITCH, ML, SG + 4)]
        allg = [g_q0a, g_q0b] + g_w1 + g_w2 + [g_step(i) for i in range(NL - 1)] + [g_last]
        started = [0]

        def start_upto(n):
            while started[0] < min(n, len(allg)):
                for c in allg[started[0]]:
                    c.start()
                started[0] += 1
        start_upto(early[0])

        def wait(g):
            for c in g:
                c.wait()

        flag_s[0] = 100
        flag_s[1] = 0
        flag_s[2] = 0
        for j in range(NL):
            k_s[j, KP - 16:KP, :] = jnp.zeros((16, 128), bf16)
        ku_s = k_s.bitcast(u32)
        vu_s = v_s.bitcast(u32)

        def region(fn):
            pl.when(flag_s[0] == 100)(fn)

        row8 = lax.broadcasted_iota(jnp.int32, (8, 128), 0)

        def false_mask():
            return row8 > flag_s[0]

        def ln(r0, m, n):
            fm = lax.broadcasted_iota(jnp.int32, (16, 1), 0) > flag_s[0]
            lasts = [None] * max(n, 1)
            for t in range(m // 16):
                rr = r0 + 16 * t
                if not isinstance(rr, int):
                    rr = pl.multiple_of(rr, 16)
                x = q_s[pl.ds(rr, 16), :].astype(f32)
                sm = jnp.sum(x, axis=-1, keepdims=True)
                ci = t % max(n, 1)
                if n and lasts[ci] is not None:
                    sm = jnp.where(fm, lasts[ci], sm)
                xc = x - sm * (1.0 / D)
                var = jnp.sum(xc * xc, axis=-1, keepdims=True) * (1.0 / D)
                rs = lax.rsqrt(var + 1e-5) * ALPHA
                lasts[ci] = rs
                xo = xc * rs
                for j in range(NL):
                    xn_s[j, pl.ds(rr, 16), :] = xo[:, j * 128:(j + 1) * 128].astype(bf16)

        def load_xn(r0, m):
            return jnp.concatenate([xn_s[j, pl.ds(r0, m), :] for j in range(NL)], axis=1)

        FR = F - 64

        def mm1_rem(xn):
            m = xn.shape[0]
            ht = lax.dot_general(w1_s[FR:F, :], xn, (((1,), (1,)), ((), ())), preferred_element_type=f32)
            bc = bc_s[...]
            outs = []
            for c0 in range(0, m, 128):
                c1 = min(c0 + 128, m)
                outs.append(gelu(ht[:, c0:c1] + bc[:, :c1 - c0]).T)
            return jnp.concatenate(outs, axis=0).astype(bf16)

        def mm1(xn, f0=0, f1=F, pin=None):
            if rem and f1 == F:
                if f0 == FR:
                    return mm1_rem(xn)
                if remlast:
                    hm = mm1(xn, f0, FR, pin)
                    hr = mm1_rem(xn)
                else:
                    hr = mm1_rem(xn)
                    hm = mm1(xn, f0, FR, pin)
                return jnp.concatenate([hm, hr], axis=1)
            b1 = b1_ref[...].astype(f32).reshape(1, F)[:, f0:f1] * ALPHA
            if pin is not None:
                b1 = jnp.where(false_mask()[0:1, :f1 - f0], pin[0:1, :f1 - f0], b1)
            h = lax.dot_general(xn, w1_s[f0:f1, :], (((1,), (1,)), ((), ())), preferred_element_type=f32) + b1
            return gelu(h).astype(bf16)

        def kv_fwd(j, sk, kvn):
            s = [jnp.broadcast_to(sk[l:l + 1, :], (8, 128)) for l in range(4)]
            dd = sk[4:5, :]
            fm = false_mask()
            lasts = [None] * kvn
            fwx = fw_ref[0]
            fwh = fw_ref[1]
            ev = lambda w: pltpu.bitcast(w << 16, f32)
            od = lambda w: pltpu.bitcast(w & jnp.uint32(0xffff0000), f32)
            kvs = []
            for a in range(NB + lag):
                if a < NB:
                    outs = []
                    for t in range(a * 8, a * 8 + 8):
                        bb = KP // 2 + 8 * t
                        w0 = ku_s[j, bb:bb + 8, :]
                        w1 = ku_s[j, bb - 1:bb + 7, :]
                        w2 = ku_s[j, bb - 2:bb + 6, :]
                        wv = vu_s[j, 8 * t:8 * t + 8, :]
                        e0, o0, e1, o1, o2 = ev(w0), od(w0), ev(w1), od(w1), od(w2)
                        ci = t % kvn
                        if lasts[ci] is not None:
                            e0 = jnp.where(fm, lasts[ci], e0)
                        oe = (e0 * s[0] + o1 * s[1] + e1 * s[2] + o2 * s[3]) * ev(wv)
                        oo = (e0 * s[1] + o0 * s[0] + o1 * s[2] + e1 * s[3]) * od(wv)
                        lasts[ci] = oo
                        outs += [oe, oo]
                    kvs.append(jnp.concatenate(outs, axis=0).astype(bf16) if 'K' not in dbg else v_s[j, a * P:(a + 1) * P, :])
                    hb = lax.dot_general(fwh, h_s[j, :, a * P:(a + 1) * P], (((1,), (1,)), ((), ())),
                                         preferred_element_type=f32)
                    if a == 0:
                        hb = jnp.concatenate(
                            [hb[8 * t:8 * t + 8, :] + dd if t % 2 == 0 else hb[8 * t:8 * t + 8, :]
                             for t in range(32)], axis=0)
                    hf_s[a] = hb
                if a >= lag:
                    x_s[a - lag] = jnp.dot(fwx, kvs[a - lag], preferred_element_type=f32)

        def conv_mac():
            fm = false_mask()
            last = None
            Y = [[None] * 16 for _ in range(NB)]
            for p in range(16):
                r0, i0 = 16 * p, 16 * p + 8
                prev = None
                for c in range(NB):
                    accr = acci = None
                    for a in range(c + 1):
                        b = c - a
                        xr = x_s[a, r0:r0 + 8, :]
                        xi = x_s[a, i0:i0 + 8, :]
                        hr = hf_s[b, r0:r0 + 8, :]
                        hi = hf_s[b, i0:i0 + 8, :]
                        if accr is None:
                            t1 = xr * hr
                            t2 = xr * hi
                            if last is not None:
                                t1 = jnp.where(fm, last[0], t1)
                                t2 = jnp.where(fm, last[1], t2)
                            accr = t1 - xi * hi
                            acci = t2 + xi * hr
                        elif p >= pf and a % fm_ == fm_ - 1:
                            accr = accr + (xr * hr - xi * hi)
                            acci = acci + (xr * hi + xi * hr)
                        else:
                            accr = (accr + xr * hr) - xi * hi
                            acci = (acci + xr * hi) + xi * hr
                    last = (accr, acci)
                    if prev is None:
                        yr, yi = accr, acci
                    else:
                        pr, pi = prev
                        yr, yi = (accr - pi, acci + pr) if p < 8 else (accr + pi, acci - pr)
                    prev = (accr, acci)
                    Y[c][p] = (yr, yi)
            return Y, last[0] + last[1]

        def conv_inv(j, Y):
            ic = inv_ref[0]
            isn = inv_ref[1]
            for c in range(NB):
                yr = jnp.concatenate([y[0] for y in Y[c]], axis=0).astype(bf16)
                yi = jnp.concatenate([y[1] for y in Y[c]], axis=0).astype(bf16)
                e = jnp.dot(ic, yr, preferred_element_type=f32)
                o = jnp.dot(isn, yi, preferred_element_type=f32)
                yp_s[j, c * P + 64:(c + 1) * P, :] = e - o
                lo = e + o
                for i in range(8):
                    yp_s[j, c * P + 8 * (7 - i):c * P + 8 * (8 - i), :] = lo[8 * i:8 * i + 8, :]

        def mlp_conv(r0, m, xn, j):
            Y, link = conv_mac()
            h = mm1(xn)
            b2 = b2_ref[...].astype(f32).reshape(1, D)
            c4 = D - 128
            o = jnp.dot(h, w2_s[:, :c4], preferred_element_type=f32)
            p_s[pl.ds(r0, m), :c4] = o * OSC + (q_s[pl.ds(r0, m), :c4].astype(f32) + b2[:, :c4])
            z = jnp.where(false_mask()[0:1, :], link[0:1, :], b2[:, c4:] * (1.0 / OSC))
            o = z + jnp.dot(h, w2_s[:, c4:], preferred_element_type=f32)
            p_s[pl.ds(r0, m), c4:] = o * OSC + q_s[pl.ds(r0, m), c4:].astype(f32)
            conv_inv(j, Y)

        rev8 = 7 - row8

        def load_y(j, t):
            y = yp_s[j, t:t + 8, :]
            if t % P < 64:
                y = jnp.take_along_axis(y, rev8, axis=0)
            return y

        def combine(r0, r1, st):
            fm = false_mask()
            for t in range(r0, r1, 16):
                ts = srow(t)
                for j in range(NL):
                    cs = slice(j * 128, (j + 1) * 128)
                    y = jnp.concatenate([load_y(j, t), load_y(j, t + 8)], axis=0)
                    p0 = p_s[ts:ts + 8, cs]
                    if st[0] is not None:
                        p0 = jnp.where(fm, st[0], p0)
                    pp = jnp.concatenate([p0, p_s[ts + 8:ts + 16, cs]], axis=0)
                    r = (pp + xn_s[j, ts:ts + 16, :].astype(f32) * y).astype(bf16)
                    st[0] = r.astype(f32)[0:8, :]
                    o_s[j, t:t + 16, :] = r

        wait(g_q0a)
        start_upto(early[1])
        ln(0, q0a, 0)
        wait(g_q0b)
        start_upto(early[2])
        ln(q0a, M0 - q0a, 0)
        for i in range(n1):
            wait(g_w1[i])
            start_upto(99)

            def r1(i=i):
                if i == 0:
                    b1r = b1_ref[...].astype(f32).reshape(1, F)[:, F - 128:F] * ALPHA
                    bc_s[...] = jnp.broadcast_to(b1r, (128, 128)).T[64:128, :]
                hid_s[:, w1c[i]:w1c[i + 1]] = mm1(load_xn(0, M0), w1c[i], w1c[i + 1])
            region(r1)
        for i in range(n2):
            wait(g_w2[i])

            def r2(i=i):
                o = jnp.dot(hid_s[:, w2c[i]:w2c[i + 1]], w2_s[w2c[i]:w2c[i + 1], :], preferred_element_type=f32)
                if i > 0:
                    o = o + p_s[0:M0, :]
                if i == 0:
                    ln(PITCH, M, 1)
                if i < n2 - 1:
                    p_s[0:M0, :] = o
                else:
                    p_s[0:M0, :] = o * OSC + (q_s[0:M0, :].astype(f32) + b2_ref[...].astype(f32).reshape(1, D))
                    skf = sk_ref[...].astype(f32)
                    ddf = dd_ref[...].astype(f32).reshape(1, D)
                    par = jnp.concatenate([skf, ddf, jnp.zeros((3, D), f32)], axis=0)
                    for j in range(NL):
                        par_s[j] = par[:, j * 128:(j + 1) * 128]
                    kv_fwd(0, par[:, 0:128], kvn0)
            region(r2)

        def body(i, carry):
            r0 = pl.multiple_of((i + 1) * PITCH, 64)
            wait(g_step(i))
            xn = load_xn(r0, M)
            if 'L' not in dbg: ln(r0 + PITCH, M, lnn)
            mlp_conv(r0, M, xn, i)
            kv_fwd(i + 1, par_s[i + 1], kvn)
            return carry
        lax.fori_loop(0, NL - 1, body, 0)

        wait(g_last)
        rl, rls = R[6], 6 * PITCH

        def f5():
            ln(rls, ML, lnn)
            mlp_conv(5 * PITCH, M, load_xn(5 * PITCH, M), NL - 1)
        region(f5)

        def co(i, j, r0, r1):
            return cp(o_s.at[j, pl.ds(r0, r1 - r0), :], out_hbm.at[pl.ds(r0, r1 - r0), pl.ds(j * 128, 128)], SO)
        rows = [0] + [int(rl // 16 * x) * 16 for x in prow] + [rl]
        g_o = [[co(i, j, rows[i], rows[i + 1]) for j in range(NL)] for i in range(nco)]
        g_fa = [co(nco, j, rl, S) for j in range(osp)]
        g_fb = [co(nco + 1, j, rl, S) for j in range(osp, NL)]

        def pin_after(g, i):
            for c in g:
                c.start()
            z1 = pl.multiple_of(S + flag_s[1], 16)
            z2 = pl.multiple_of(S + flag_s[2], 16)
            o_s[0, pl.ds(z1, 16), :] = jnp.full((16, 128), i, bf16)
            return o_s[0, pl.ds(z2, 16), :].astype(f32)

        def f6():
            xn = load_xn(rls, ML)
            st = [None]
            hs = []
            gi = 0
            for f in range(14):
                pin = None
                if gi < nco and pins[gi] == f:
                    combine(rows[gi], rows[gi + 1], st)
                    pin = pin_after(g_o[gi], gi)
                    gi += 1
                hs.append(mm1(xn, 128 * f, min(128 * (f + 1), F), pin))
            h = jnp.concatenate(hs, axis=1)
            b2 = b2_ref[...].astype(f32).reshape(1, D)
            for j in range(NL):
                cs = slice(j * 128, (j + 1) * 128)
                bj = b2[:, cs] * (1.0 / OSC)
                if gi < nco and pins[gi] == 14 + j:
                    combine(rows[gi], rows[gi + 1], st)
                    pin = pin_after(g_o[gi], gi)
                    bj = jnp.where(false_mask()[0:1, :], pin[0:1, :], bj)
                    gi += 1
                if j == osp:
                    pin = pin_after(g_fa, nco)
                    bj = jnp.where(false_mask()[0:1, :], pin[0:1, :], bj)
                o = (bj + jnp.dot(h, w2_s[:, cs], preferred_element_type=f32)) * OSC + q_s[rls:rls + ML, cs].astype(f32)
                y = jnp.concatenate([load_y(j, t) for t in range(rl, S, 8)], axis=0)
                o_s[j, rl:S, :] = (o + xn_s[j, rls:rls + ML, :].astype(f32) * y).astype(bf16)
            assert gi == nco
        region(f6)
        for c in g_fb:
            c.start()
        for g in g_o:
            wait(g)
        wait(g_fa)
        wait(g_fb)

    fw, inv = dft_mats()

    @jax.jit
    def f(q, k, v, sk, h, dd, w1, b1, w2, b2):
        any_ = pl.BlockSpec(memory_space=pl.ANY)
        out = pl.pallas_call(
            kernel,
            in_specs=[any_] * 12,
            out_specs=any_,
            out_shape=jax.ShapeDtypeStruct((S, D), bf16),
            scratch_shapes=[
                pltpu.VMEM((SR, D), bf16),
                pltpu.VMEM((NL, S + KP, 128), bf16),
                pltpu.VMEM((NL, S, 128), bf16),
                pltpu.VMEM((NL, 128, S), bf16),
                pltpu.VMEM((F, D), bf16),
                pltpu.VMEM((F, D), bf16),
                pltpu.VMEM((NL, SR, 128), bf16),
                pltpu.VMEM((SR, D), f32),
                pltpu.VMEM((NB, 256, 128), f32),
                pltpu.VMEM((NB, 256, 128), f32),
                pltpu.VMEM((NL, S, 128), f32),
                pltpu.VMEM((NL, S + 16, 128), bf16),
                pltpu.VMEM((NL, 8, 128), f32),
                pltpu.VMEM((M0, F), bf16),
                pltpu.VMEM((4, D), bf16), pltpu.VMEM((D,), bf16), pltpu.VMEM((F,), bf16), pltpu.VMEM((D,), bf16),
                pltpu.VMEM((2, 256, 128), bf16), pltpu.VMEM((2, 64, 128), bf16),
                pltpu.VMEM((64, 128), f32),
                pltpu.SMEM((8,), jnp.int32),
                pltpu.SemaphoreType.DMA((NSEM,)),
            ],
            compiler_params=pltpu.CompilerParams(vmem_limit_bytes=100 * 2**20),
            name=name,
        )(q.reshape(S, D), k.reshape(S, D), v.reshape(S, D), sk.T, h, dd, w1.T, b1, w2, b2,
          jnp.asarray(fw, bf16), jnp.asarray(inv, bf16))
        return out.reshape(1, S, D)
    return f


_impl = make(M0=512, M=256, pins=(1, 6, 10, 14), prow=(0.02, 0.33, 0.66))


@jax.jit
def pallas_parallel_sum__ssm_conv_h3__dense_activation_gelu__prompt_kernel(
    A_q, A_k, A_v, A_shift_k, A_ssm_k, A_ssm_D, B_x, B_w1, B_b1, B_w2, B_b2,
):
    del B_x
    return _impl(A_q, A_k, A_v, A_shift_k, A_ssm_k, A_ssm_D, B_w1, B_b1, B_w2, B_b2)
```

```python
import numpy as np
import jax
import jax.numpy as jnp
from jax import lax
import jax.experimental.pallas as pl
import jax.experimental.pallas.tpu as pltpu

S, D, F = 2048, 640, 1728
P = 128
NB = S // P
NL = D // 128
KP = 64
f32, bf16, u32 = jnp.float32, jnp.bfloat16, jnp.uint32


ALPHA = (0.7978845608028654 * 0.044715) ** (1.0 / 3.0)
C1 = 0.7978845608028654 / ALPHA
OSC = 0.5 / ALPHA


def dft_mats():
    ks = np.concatenate([np.arange(0, 128, 2), np.arange(1, 128, 2)])
    n = np.arange(128)
    m = np.arange(64) + 0.5
    fw = np.zeros((2, 256, 128))
    inv = np.zeros((2, 64, 128))
    for p in range(16):
        for s in range(8):
            w = 2 * np.pi * (ks[8 * p + s] + 0.5) / 256
            fw[0, 16 * p + s] = np.cos(w * (n - 63.5))
            fw[0, 16 * p + 8 + s] = -np.sin(w * (n - 63.5))
            fw[1, 16 * p + s] = np.cos(w * n)
            fw[1, 16 * p + 8 + s] = -np.sin(w * n)
            inv[0, :, 8 * p + s] = np.cos(w * m) / (128 * ALPHA)
            inv[1, :, 8 * p + s] = np.sin(w * m) / (128 * ALPHA)
    perm = np.concatenate(
        [16 * t + np.concatenate([np.arange(0, 16, 2), np.arange(1, 16, 2)]) for t in range(8)])
    fw[0] = fw[0][:, perm]
    return fw, inv


def gelu(g):
    return g * (1.0 + jnp.tanh(g * (C1 + g * g)))


def make(M0=576, M=256, name="v20", kvn=2, kvn0=2, w1c=(0, 256, 768, F), w2c=(0, 640, 1280, F), q0c=(0, 256, 448),
         lnn=1, pins=(2, 7, 12, 15), prow=(0.01, 0.28, 0.6), lnsplit=(512, 512, 448), m56=True, cn6=1, ln0=2, u2=3, mac2=(0, 1, (), 3), mac1=None, lnlow=False, osp=4, lag=2, pitch=None, early=(99, 99, 99), rem=True, lk=0, pf=16, fm_=4, remlast=False, dbg=''):
    ML = S - M0 - NL * M
    assert ML > 0 and ML % 16 == 0
    R = [0, M0] + [M0 + (i + 1) * M for i in range(NL)] + [S]
    assert M0 % 64 == 0 and M % 64 == 0 and sum(lnsplit) == S - M0
    SR = S

    def srow(r):
        return r

    n1, n2, nco = len(w1c) - 1, len(w2c) - 1, len(pins)
    SW1 = len(q0c)
    SW2 = SW1 + n1
    SG = SW2 + n2
    SO = SG + 4
    NSEM = SO + 1

    def kernel(q_hbm, k_hbm, v_hbm, sk_hbm, h_hbm, dd_hbm, w1_hbm, b1_hbm, w2_hbm, b2_hbm, fw_hbm, inv_hbm,
               out_hbm,
               q_s, k_s, v_s, h_s, w1_s, w2_s, xn_s, p_s, x_s, hf_s, yp_s, o_s, par_s, hid_s,
               sk_ref, dd_ref, b1_ref, b2_ref, fw_ref, inv_ref, bc_s, flag_s, sem):
        def cp(src, dst, i):
            return pltpu.make_async_copy(src, dst, sem.at[i])

        def cq(r, rs, m, si):
            return cp(q_hbm.at[pl.ds(r, m)], q_s.at[pl.ds(rs, m)], si)

        def cw(hbm, s_, c, i, si):
            rows = pl.ds(c[i], c[i + 1] - c[i])
            return cp(hbm.at[rows], s_.at[rows], si)

        def ckvh(j, si):
            lane = pl.ds(j * 128, 128) if isinstance(j, int) else pl.ds(pl.multiple_of(j * 128, 128), 128)
            return [cp(h_hbm.at[lane, :], h_s.at[j], si),
                    cp(k_hbm.at[:, lane], k_s.at[j, pl.ds(KP, S), :], si),
                    cp(v_hbm.at[:, lane], v_s.at[j], si)]

        qc = list(q0c) + [M0]
        g_q0 = [[cq(qc[i], qc[i], qc[i + 1] - qc[i], i)] for i in range(len(q0c))]
        g_w1 = [[cw(w1_hbm, w1_s, w1c, i, SW1 + i)] for i in range(n1)]
        g_w1[0].append(cp(b1_hbm, b1_ref, SW1))
        g_w2 = [[cw(w2_hbm, w2_s, w2c, i, SW2 + i)] for i in range(n2)]
        g_w2[0] = [cq(M0, M0, S - M0, SW2)] + g_w2[0]
        sl = SW2 + n2 - 1
        g_w2[-1] = g_w2[-1] + [cp(b2_hbm, b2_ref, sl), cp(sk_hbm, sk_ref, sl), cp(dd_hbm, dd_ref, sl),
                               cp(fw_hbm, fw_ref, sl), cp(inv_hbm, inv_ref, sl)] + ckvh(0, sl)

        def g_step(i):
            return ckvh(i + 1, SG + i)

        allg = g_q0 + g_w1 + g_w2 + [g_step(i) for i in range(NL - 1)]
        started = [0]

        def start_upto(n):
            while started[0] < min(n, len(allg)):
                for c in allg[started[0]]:
                    c.start()
                started[0] += 1
        start_upto(early[0])

        def wait(g):
            for c in g:
                c.wait()

        flag_s[0] = 100
        flag_s[1] = 0
        flag_s[2] = 0
        for j in range(NL):
            k_s[j, KP - 16:KP, :] = jnp.zeros((16, 128), bf16)
        ku_s = k_s.bitcast(u32)
        vu_s = v_s.bitcast(u32)

        def region(fn):
            pl.when(flag_s[0] == 100)(fn)

        row8 = lax.broadcasted_iota(jnp.int32, (8, 128), 0)

        def false_mask():
            return row8 > flag_s[0]

        def ln(r0, m, n):
            fm = lax.broadcasted_iota(jnp.int32, (16, 1), 0) > flag_s[0]
            lasts = [None] * max(n, 1)
            for t in range(m // 16):
                rr = r0 + 16 * t
                if not isinstance(rr, int):
                    rr = pl.multiple_of(rr, 16)
                x = q_s[pl.ds(rr, 16), :].astype(f32)
                sm = jnp.sum(x, axis=-1, keepdims=True)
                ci = t % max(n, 1)
                if n and lasts[ci] is not None:
                    sm = jnp.where(fm, lasts[ci], sm)
                mu = sm * (1.0 / D)
                low = lnlow and n
                if low:
                    x = q_s[pl.ds(pl.multiple_of(rr + flag_s[1], 16), 16), :].astype(f32)
                xc = x - mu
                var = jnp.sum(xc * xc, axis=-1, keepdims=True) * (1.0 / D)
                rs = lax.rsqrt(var + 1e-5) * ALPHA
                lasts[ci] = rs
                if low:
                    xc = q_s[pl.ds(pl.multiple_of(rr + flag_s[2], 16), 16), :].astype(f32) - mu
                xo = xc * rs
                for j in range(NL):
                    xn_s[j, pl.ds(rr, 16), :] = xo[:, j * 128:(j + 1) * 128].astype(bf16)

        def load_xn(r0, m):
            return jnp.concatenate([xn_s[j, pl.ds(r0, m), :] for j in range(NL)], axis=1)

        FR = F - 64

        def mm1_rem(xn):
            m = xn.shape[0]
            ht = lax.dot_general(w1_s[FR:F, :], xn, (((1,), (1,)), ((), ())), preferred_element_type=f32)
            bc = bc_s[...]
            outs = []
            for c0 in range(0, m, 128):
                c1 = min(c0 + 128, m)
                outs.append(gelu(ht[:, c0:c1] + bc[:, :c1 - c0]).T)
            return jnp.concatenate(outs, axis=0).astype(bf16)

        def mm1(xn, f0=0, f1=F, pin=None):
            if rem and f1 == F:
                if f0 == FR:
                    return mm1_rem(xn)
                if remlast:
                    hm = mm1(xn, f0, FR, pin)
                    hr = mm1_rem(xn)
                else:
                    hr = mm1_rem(xn)
                    hm = mm1(xn, f0, FR, pin)
                return jnp.concatenate([hm, hr], axis=1)
            b1 = b1_ref[...].astype(f32).reshape(1, F)[:, f0:f1] * ALPHA
            if pin is not None:
                b1 = jnp.where(false_mask()[0:1, :f1 - f0], pin[0:1, :f1 - f0], b1)
            h = lax.dot_general(xn, w1_s[f0:f1, :], (((1,), (1,)), ((), ())), preferred_element_type=f32) + b1
            return gelu(h).astype(bf16)

        def kv_fwd(j, sk, kvn):
            s = [jnp.broadcast_to(sk[l:l + 1, :], (8, 128)) for l in range(4)]
            dd = sk[4:5, :]
            fm = false_mask()
            lasts = [None] * kvn
            fwx = fw_ref[0]
            fwh = fw_ref[1]
            ev = lambda w: pltpu.bitcast(w << 16, f32)
            od = lambda w: pltpu.bitcast(w & jnp.uint32(0xffff0000), f32)
            kvs = []
            for a in range(NB + lag):
                if a < NB:
                    outs = []
                    for t in range(a * 8, a * 8 + 8):
                        bb = KP // 2 + 8 * t
                        w0 = ku_s[j, bb:bb + 8, :]
                        w1 = ku_s[j, bb - 1:bb + 7, :]
                        w2 = ku_s[j, bb - 2:bb + 6, :]
                        wv = vu_s[j, 8 * t:8 * t + 8, :]
                        e0, o0, e1, o1, o2 = ev(w0), od(w0), ev(w1), od(w1), od(w2)
                        ci = t % kvn
                        if lasts[ci] is not None:
                            e0 = jnp.where(fm, lasts[ci], e0)
                        oe = (e0 * s[0] + o1 * s[1] + e1 * s[2] + o2 * s[3]) * ev(wv)
                        oo = (e0 * s[1] + o0 * s[0] + o1 * s[2] + e1 * s[3]) * od(wv)
                        lasts[ci] = oo
                        outs += [oe, oo]
                    kvs.append(jnp.concatenate(outs, axis=0).astype(bf16) if 'K' not in dbg else v_s[j, a * P:(a + 1) * P, :])
                    hb = lax.dot_general(fwh, h_s[j, :, a * P:(a + 1) * P], (((1,), (1,)), ((), ())),
                                         preferred_element_type=f32)
                    if a == 0:
                        hb = jnp.concatenate(
                            [hb[8 * t:8 * t + 8, :] + dd if t % 2 == 0 else hb[8 * t:8 * t + 8, :]
                             for t in range(32)], axis=0)
                    hf_s[a] = hb
                if a >= lag:
                    x_s[a - lag] = jnp.dot(fwx, kvs[a - lag], preferred_element_type=f32)

        def conv_mac(pf=pf, fm_=fm_, par=(), mg=0):
            fm = false_mask()
            last = None
            Y = [[None] * 16 for _ in range(NB)]
            saved = None
            for p in range(16):
                r0, i0 = 16 * p, 16 * p + 8
                prev = None
                if p in par:
                    other = last
                    last = saved
                else:
                    other = None
                saved = last
                for c in range(NB):
                    accr = acci = None
                    pend = None
                    for a in range(c + 1):
                        b = c - a
                        xr = x_s[a, r0:r0 + 8, :]
                        xi = x_s[a, i0:i0 + 8, :]
                        hr = hf_s[b, r0:r0 + 8, :]
                        hi = hf_s[b, i0:i0 + 8, :]
                        if accr is None:
                            t1 = xr * hr
                            t2 = xr * hi
                            if last is not None:
                                t1 = jnp.where(fm, last[0], t1)
                                t2 = jnp.where(fm, last[1], t2)
                            accr = t1 - xi * hi
                            acci = t2 + xi * hr
                        elif p >= pf and ((a % fm_ == fm_ - 1) if fm_ > 0 else (a % (-fm_) != 0)):
                            tr = xr * hr - xi * hi
                            ti = xr * hi + xi * hr
                            if pend is not None:
                                tr = tr + pend[0]
                                ti = ti + pend[1]
                                pend = None
                            elif mg and a % mg == 1 and a < c:
                                pend = (tr, ti)
                                continue
                            accr = accr + tr
                            acci = acci + ti
                        else:
                            accr = (accr + xr * hr) - xi * hi
                            acci = (acci + xr * hi) + xi * hr
                    last = (accr, acci)
                    if prev is None:
                        yr, yi = accr, acci
                    else:
                        pr, pi = prev
                        yr, yi = (accr - pi, acci + pr) if p < 8 else (accr + pi, acci - pr)
                    prev = (accr, acci)
                    Y[c][p] = (yr, yi)
                if other is not None:
                    last = (last[0] + other[0], last[1] + other[1])
            return Y, last[0] + last[1]

        def conv_inv(j, Y):
            ic = inv_ref[0]
            isn = inv_ref[1]
            for c in range(NB):
                yr = jnp.concatenate([y[0] for y in Y[c]], axis=0).astype(bf16)
                yi = jnp.concatenate([y[1] for y in Y[c]], axis=0).astype(bf16)
                e = jnp.dot(ic, yr, preferred_element_type=f32)
                o = jnp.dot(isn, yi, preferred_element_type=f32)
                yp_s[j, c * P + 64:(c + 1) * P, :] = e - o
                lo = e + o
                for i in range(8):
                    yp_s[j, c * P + 8 * (7 - i):c * P + 8 * (8 - i), :] = lo[8 * i:8 * i + 8, :]

        def mlp_conv(r0, m, xn, j, *mac):
            Y, link = conv_mac(*mac)
            h = mm1(xn)
            b2 = b2_ref[...].astype(f32).reshape(1, D)
            c4 = D - 128
            o = jnp.dot(h, w2_s[:, :c4], preferred_element_type=f32)
            p_s[pl.ds(r0, m), :c4] = o * OSC + (q_s[pl.ds(r0, m), :c4].astype(f32) + b2[:, :c4])
            z = jnp.where(false_mask()[0:1, :], link[0:1, :], b2[:, c4:] * (1.0 / OSC))
            o = z + jnp.dot(h, w2_s[:, c4:], preferred_element_type=f32)
            p_s[pl.ds(r0, m), c4:] = o * OSC + q_s[pl.ds(r0, m), c4:].astype(f32)
            conv_inv(j, Y)

        rev8 = 7 - row8

        def load_y(j, t):
            y = yp_s[j, t:t + 8, :]
            if t % P < 64:
                y = jnp.take_along_axis(y, rev8, axis=0)
            return y

        def combine(r0, r1, st):
            fm = false_mask()
            for t in range(r0, r1, 16):
                ts = srow(t)
                for j in range(NL):
                    cs = slice(j * 128, (j + 1) * 128)
                    y = jnp.concatenate([load_y(j, t), load_y(j, t + 8)], axis=0)
                    p0 = p_s[ts:ts + 8, cs]
                    ci = st[-1] % (len(st) - 1)
                    st[-1] += 1
                    if st[ci] is not None:
                        p0 = jnp.where(fm, st[ci], p0)
                    pp = jnp.concatenate([p0, p_s[ts + 8:ts + 16, cs]], axis=0)
                    r = (pp + xn_s[j, ts:ts + 16, :].astype(f32) * y).astype(bf16)
                    st[ci] = r.astype(f32)[0:8, :]
                    o_s[j, t:t + 16, :] = r

        for i in range(len(q0c)):
            wait(g_q0[i])
            ln(qc[i], qc[i + 1] - qc[i], 0)
        for i in range(n1):
            wait(g_w1[i])
            start_upto(99)

            def r1(i=i):
                if i == 0:
                    b1r = b1_ref[...].astype(f32).reshape(1, F)[:, F - 128:F] * ALPHA
                    bc_s[...] = jnp.broadcast_to(b1r, (128, 128)).T[64:128, :]
                hid_s[:, w1c[i]:w1c[i + 1]] = mm1(load_xn(0, M0), w1c[i], w1c[i + 1])
            region(r1)
        for i in range(n2):
            wait(g_w2[i])

            def r2(i=i):
                o = jnp.dot(hid_s[:, w2c[i]:w2c[i + 1]], w2_s[w2c[i]:w2c[i + 1], :], preferred_element_type=f32)
                if i > 0:
                    o = o + p_s[0:M0, :]
                if i < len(lnsplit):
                    ln(M0 + sum(lnsplit[:i]), lnsplit[i], ln0)
                if i < n2 - 1:
                    p_s[0:M0, :] = o
                else:
                    p_s[0:M0, :] = o * OSC + (q_s[0:M0, :].astype(f32) + b2_ref[...].astype(f32).reshape(1, D))
                    skf = sk_ref[...].astype(f32)
                    ddf = dd_ref[...].astype(f32).reshape(1, D)
                    par = jnp.concatenate([skf, ddf, jnp.zeros((3, D), f32)], axis=0)
                    for j in range(NL):
                        par_s[j] = par[:, j * 128:(j + 1) * 128]
                    kv_fwd(0, par[:, 0:128], kvn0)
            region(r2)

        def body(i, carry):
            r0 = pl.multiple_of(M0 + i * M, 64)
            wait(g_step(i))
            xn = load_xn(r0, M)
            mlp_conv(r0, M, xn, i)
            kv_fwd(i + 1, par_s[i + 1], kvn)
            return carry
        def fence_xh():
            z = NB + flag_s[1]
            x_s[z, 0:8, :] = jnp.zeros((8, 128), f32)
            hf_s[z, 0:8, :] = jnp.zeros((8, 128), f32)

        def step(i, *mac):
            r0 = pl.multiple_of(M0 + i * M, 64)
            mlp_conv(r0, M, load_xn(r0, M), i, *mac)
            kv_fwd(i + 1, par_s[i + 1], kvn)

        if u2 == 3:
            def body3(i, carry):
                wait(g_step(2 * i))
                wait(g_step(2 * i + 1))
                if mac1 is not None:
                    fence_xh()
                    step(2 * i, *mac1)
                else:
                    step(2 * i)
                fence_xh()
                step(2 * i + 1, *mac2)
                return carry
            lax.fori_loop(0, 2, body3, 0)
        elif u2 == 1:
            def body2(i, carry):
                body(2 * i, carry)
                region(lambda: [body(2 * i + 1, carry), None][1])
                return carry
            lax.fori_loop(0, 2, body2, 0)
        elif u2 == 2:
            for i in range(NL - 1):
                region(lambda: [body(jnp.int32(i) + flag_s[1], 0), None][1])
        else:
            lax.fori_loop(0, NL - 1, body, 0)

        rl, rls = R[6], R[6]

        def f5():
            mlp_conv(R[5], M, load_xn(R[5], M), NL - 1)
        if not m56:
            region(f5)

        def co(i, j, r0, r1):
            return cp(o_s.at[j, pl.ds(r0, r1 - r0), :], out_hbm.at[pl.ds(r0, r1 - r0), pl.ds(j * 128, 128)], SO)
        rows = [0] + [int(rl // 16 * x) * 16 for x in prow] + [rl]
        g_o = [[co(i, j, rows[i], rows[i + 1]) for j in range(NL)] for i in range(nco)]
        g_fa = [co(nco, j, rl, S) for j in range(osp)]
        g_fb = [co(nco + 1, j, rl, S) for j in range(osp, NL)]

        def pin_after(g, i):
            for c in g:
                c.start()
            z1 = pl.multiple_of(S + flag_s[1], 16)
            z2 = pl.multiple_of(S + flag_s[2], 16)
            o_s[0, pl.ds(z1, 16), :] = jnp.full((16, 128), i, bf16)
            return o_s[0, pl.ds(z2, 16), :].astype(f32)

        def f6():
            if m56:
                f5()
                yp_s[NL + flag_s[1], 0:8, :] = jnp.zeros((8, 128), f32)
                p_s[pl.ds(pl.multiple_of(SR + flag_s[1], 8), 8), 0:128] = jnp.zeros((8, 128), f32)
            xn = load_xn(rls, ML)
            st = [None] * cn6 + [0]
            hs = []
            gi = 0
            for f in range(14):
                pin = None
                if gi < nco and pins[gi] == f:
                    combine(rows[gi], rows[gi + 1], st)
                    pin = pin_after(g_o[gi], gi)
                    gi += 1
                hs.append(mm1(xn, 128 * f, min(128 * (f + 1), F), pin))
            h = jnp.concatenate(hs, axis=1)
            b2 = b2_ref[...].astype(f32).reshape(1, D)
            for j in range(NL):
                cs = slice(j * 128, (j + 1) * 128)
                bj = b2[:, cs] * (1.0 / OSC)
                if gi < nco and pins[gi] == 14 + j:
                    combine(rows[gi], rows[gi + 1], st)
                    pin = pin_after(g_o[gi], gi)
                    bj = jnp.where(false_mask()[0:1, :], pin[0:1, :], bj)
                    gi += 1
                if j == osp:
                    pin = pin_after(g_fa, nco)
                    bj = jnp.where(false_mask()[0:1, :], pin[0:1, :], bj)
                o = (bj + jnp.dot(h, w2_s[:, cs], preferred_element_type=f32)) * OSC + q_s[rls:rls + ML, cs].astype(f32)
                y = jnp.concatenate([load_y(j, t) for t in range(rl, S, 8)], axis=0)
                o_s[j, rl:S, :] = (o + xn_s[j, rls:rls + ML, :].astype(f32) * y).astype(bf16)
            assert gi == nco
        region(f6)
        for c in g_fb:
            c.start()
        for g in g_o:
            wait(g)
        wait(g_fa)
        wait(g_fb)

    fw, inv = dft_mats()

    @jax.jit
    def f(q, k, v, sk, h, dd, w1, b1, w2, b2):
        any_ = pl.BlockSpec(memory_space=pl.ANY)
        out = pl.pallas_call(
            kernel,
            in_specs=[any_] * 12,
            out_specs=any_,
            out_shape=jax.ShapeDtypeStruct((S, D), bf16),
            scratch_shapes=[
                pltpu.VMEM((SR, D), bf16),
                pltpu.VMEM((NL, S + KP, 128), bf16),
                pltpu.VMEM((NL, S, 128), bf16),
                pltpu.VMEM((NL, 128, S), bf16),
                pltpu.VMEM((F, D), bf16),
                pltpu.VMEM((F, D), bf16),
                pltpu.VMEM((NL, SR, 128), bf16),
                pltpu.VMEM((SR + 8, D), f32),
                pltpu.VMEM((NB + 1, 256, 128), f32),
                pltpu.VMEM((NB + 1, 256, 128), f32),
                pltpu.VMEM((NL + 1, S, 128), f32),
                pltpu.VMEM((NL, S + 16, 128), bf16),
                pltpu.VMEM((NL, 8, 128), f32),
                pltpu.VMEM((M0, F), bf16),
                pltpu.VMEM((4, D), bf16), pltpu.VMEM((D,), bf16), pltpu.VMEM((F,), bf16), pltpu.VMEM((D,), bf16),
                pltpu.VMEM((2, 256, 128), bf16), pltpu.VMEM((2, 64, 128), bf16),
                pltpu.VMEM((64, 128), f32),
                pltpu.SMEM((8,), jnp.int32),
                pltpu.SemaphoreType.DMA((NSEM,)),
            ],
            compiler_params=pltpu.CompilerParams(vmem_limit_bytes=100 * 2**20),
            name=name,
        )(q.reshape(S, D), k.reshape(S, D), v.reshape(S, D), sk.T, h, dd, w1.T, b1, w2, b2,
          jnp.asarray(fw, bf16), jnp.asarray(inv, bf16))
        return out.reshape(1, S, D)
    return f


_impl = make()


@jax.jit
def pallas_parallel_sum__ssm_conv_h3__dense_activation_gelu__prompt_kernel(
    A_q, A_k, A_v, A_shift_k, A_ssm_k, A_ssm_D, B_x, B_w1, B_b1, B_w2, B_b2,
):
    del B_x
    return _impl(A_q, A_k, A_v, A_shift_k, A_ssm_k, A_ssm_D, B_w1, B_b1, B_w2, B_b2)
```

```python
import numpy as np
import jax
import jax.numpy as jnp
from jax import lax
import jax.experimental.pallas as pl
import jax.experimental.pallas.tpu as pltpu

S, D, F = 2048, 640, 1728
P = 128
NB = S // P
NL = D // 128
KP = 64
FR = F - 64
f32, bf16, u32 = jnp.float32, jnp.bfloat16, jnp.uint32
NT = (((1,), (1,)), ((), ()))

ALPHA = (0.7978845608028654 * 0.044715) ** (1.0 / 3.0)
C1 = 0.7978845608028654 / ALPHA
OSC = 0.5 / ALPHA


def dft_mats():
    ks = np.concatenate([np.arange(0, 128, 2), np.arange(1, 128, 2)])
    n = np.arange(128)
    m = np.arange(64) + 0.5
    fw = np.zeros((2, 256, 128))
    inv = np.zeros((2, 64, 128))
    for p in range(16):
        for s in range(8):
            w = 2 * np.pi * (ks[8 * p + s] + 0.5) / 256
            fw[0, 16 * p + s] = np.cos(w * (n - 63.5))
            fw[0, 16 * p + 8 + s] = -np.sin(w * (n - 63.5))
            fw[1, 16 * p + s] = np.cos(w * n)
            fw[1, 16 * p + 8 + s] = -np.sin(w * n)
            inv[0, :, 8 * p + s] = np.cos(w * m) / (128 * ALPHA)
            inv[1, :, 8 * p + s] = np.sin(w * m) / (128 * ALPHA)
    perm = np.concatenate(
        [16 * t + np.concatenate([np.arange(0, 16, 2), np.arange(1, 16, 2)]) for t in range(8)])
    fw[0] = fw[0][:, perm]
    return fw.astype(np.float32).astype(bf16), inv.astype(np.float32).astype(bf16)


def gelu(g):
    return g * (1.0 + jnp.tanh(g * (C1 + g * g)))


def make(M0=576, M=256, name="v24", kvn=2, qa=256, w1c=(0, 256, 768, F), w2k=896, lns=832, ln0=2,
         pins=(2, 7, 12, 15), prow=(0.01, 0.28, 0.6), osp=4, lag=2, mg=3, ring=4):
    ML = S - M0 - NL * M
    assert ML > 0 and ML % 16 == 0 and M0 % 64 == 0 and M % 64 == 0
    n1, nco = len(w1c) - 1, len(pins)

    def kernel(q_hbm, k_hbm, v_hbm, sk_hbm, h_hbm, dd_hbm, w1_hbm, b1_hbm, w2_hbm, b2_hbm, fw_hbm, inv_hbm,
               out_hbm,
               q_s, k_s, v_s, h_s, w1_s, w2_s, xn_s, p_s, x_s, hf_s, yp_s, o_s, par_s, hid_s,
               sk_ref, dd_ref, b1_ref, b2_ref, fw_ref, inv_ref, bc_s, flag_s, sem):
        def rows(src, dst, r0, r1):
            return (src.at[pl.ds(r0, r1 - r0)], dst.at[pl.ds(r0, r1 - r0)])

        def kvh(j):
            lane = pl.ds(j * 128, 128) if isinstance(j, int) else pl.ds(pl.multiple_of(j * 128, 128), 128)
            return [(h_hbm.at[lane, :], h_s.at[j]),
                    (k_hbm.at[:, lane], k_s.at[j, pl.ds(KP, S), :]),
                    (v_hbm.at[:, lane], v_s.at[j])]

        def copies(g, si):
            return [pltpu.make_async_copy(src, dst, sem.at[si]) for src, dst in g]

        groups = [[rows(q_hbm, q_s, 0, qa)],
                  [rows(w1_hbm, w1_s, 0, w1c[1]), (b1_hbm, b1_ref)],
                  [rows(q_hbm, q_s, qa, M0)]]
        groups += [[rows(w1_hbm, w1_s, w1c[i], w1c[i + 1])] for i in range(1, n1)]
        groups += [[rows(q_hbm, q_s, M0, S), rows(w2_hbm, w2_s, 0, w2k)],
                   [rows(w2_hbm, w2_s, w2k, F), (b2_hbm, b2_ref), (sk_hbm, sk_ref), (dd_hbm, dd_ref),
                    (fw_hbm, fw_ref), (inv_hbm, inv_ref)] + kvh(0),
                   kvh(1) + kvh(2), kvh(3) + kvh(4)]
        ng = len(groups)
        sem_out = (ng - 3) % ring if ring < ng else ng

        def start(g):
            if g < ng:
                for c in copies(groups[g], g % ring):
                    c.start()

        def wait(g):
            for c in copies(groups[g], g % ring):
                c.wait()
            start(g + ring)

        for g in range(ring):
            start(g)

        flag_s[0] = 100
        flag_s[1] = 0
        flag_s[2] = 0
        for j in range(NL):
            k_s[j, KP - 16:KP, :] = jnp.zeros((16, 128), bf16)
        ku_s = k_s.bitcast(u32)
        vu_s = v_s.bitcast(u32)

        def region(fn):
            pl.when(flag_s[0] == 100)(fn)

        row8 = lax.broadcasted_iota(jnp.int32, (8, 128), 0)

        def false_mask():
            return row8 > flag_s[0]

        def ln(r0, r1, n):
            fm = lax.broadcasted_iota(jnp.int32, (16, 1), 0) > flag_s[0]
            lasts = [None] * max(n, 1)
            for t, rr in enumerate(range(r0, r1, 16)):
                x = q_s[rr:rr + 16, :].astype(f32)
                sm = jnp.sum(x, axis=-1, keepdims=True)
                ci = t % max(n, 1)
                if n and lasts[ci] is not None:
                    sm = jnp.where(fm, lasts[ci], sm)
                xc = x - sm * (1.0 / D)
                var = jnp.sum(xc * xc, axis=-1, keepdims=True) * (1.0 / D)
                rs = lax.rsqrt(var + 1e-5) * ALPHA
                lasts[ci] = rs
                xo = xc * rs
                for j in range(NL):
                    xn_s[j, rr:rr + 16, :] = xo[:, j * 128:(j + 1) * 128].astype(bf16)

        def load_xn(r0, m):
            return jnp.concatenate([xn_s[j, pl.ds(r0, m), :] for j in range(NL)], axis=1)

        def b1_row():
            return b1_ref[...].astype(f32).reshape(1, F) * ALPHA

        def b2_row():
            return b2_ref[...].astype(f32).reshape(1, D)

        def mm1_rem(xn):
            m = xn.shape[0]
            ht = lax.dot_general(w1_s[FR:F, :], xn, NT, preferred_element_type=f32)
            bc = bc_s[...]
            outs = []
            for c0 in range(0, m, 128):
                c1 = min(c0 + 128, m)
                outs.append(gelu(ht[:, c0:c1] + bc[:, :c1 - c0]).T)
            return jnp.concatenate(outs, axis=0).astype(bf16)

        def mm1(xn, f0=0, f1=F, pin=None):
            if f1 == F:
                hr = mm1_rem(xn)
                if f0 == FR:
                    return hr
                return jnp.concatenate([mm1(xn, f0, FR, pin), hr], axis=1)
            b1 = b1_row()[:, f0:f1]
            if pin is not None:
                b1 = jnp.where(false_mask()[0:1, :f1 - f0], pin[0:1, :f1 - f0], b1)
            h = lax.dot_general(xn, w1_s[f0:f1, :], NT, preferred_element_type=f32) + b1
            return gelu(h).astype(bf16)

        def kv_fwd(j, sk):
            s = [jnp.broadcast_to(sk[l:l + 1, :], (8, 128)) for l in range(4)]
            dd = sk[4:5, :]
            fm = false_mask()
            lasts = [None] * kvn
            fwx = fw_ref[0]
            fwh = fw_ref[1]
            ev = lambda w: pltpu.bitcast(w << 16, f32)
            od = lambda w: pltpu.bitcast(w & jnp.uint32(0xffff0000), f32)
            kvs = []
            for a in range(NB + lag):
                if a < NB:
                    outs = []
                    for t in range(a * 8, a * 8 + 8):
                        bb = KP // 2 + 8 * t
                        w0 = ku_s[j, bb:bb + 8, :]
                        w1 = ku_s[j, bb - 1:bb + 7, :]
                        w2 = ku_s[j, bb - 2:bb + 6, :]
                        wv = vu_s[j, 8 * t:8 * t + 8, :]
                        e0, o0, e1, o1, o2 = ev(w0), od(w0), ev(w1), od(w1), od(w2)
                        ci = t % kvn
                        if lasts[ci] is not None:
                            e0 = jnp.where(fm, lasts[ci], e0)
                        oe = (e0 * s[0] + o1 * s[1] + e1 * s[2] + o2 * s[3]) * ev(wv)
                        oo = (e0 * s[1] + o0 * s[0] + o1 * s[2] + e1 * s[3]) * od(wv)
                        lasts[ci] = oo
                        outs += [oe, oo]
                    kvs.append(jnp.concatenate(outs, axis=0).astype(bf16))
                    hb = lax.dot_general(fwh, h_s[j, :, a * P:(a + 1) * P], NT, preferred_element_type=f32)
                    if a == 0:
                        hb = jnp.concatenate(
                            [hb[8 * t:8 * t + 8, :] + dd if t % 2 == 0 else hb[8 * t:8 * t + 8, :]
                             for t in range(32)], axis=0)
                    hf_s[a] = hb
                if a >= lag:
                    x_s[a - lag] = jnp.dot(fwx, kvs[a - lag], preferred_element_type=f32)

        def conv_mac(short):
            fm = false_mask()
            last = None
            Y = [[None] * 16 for _ in range(NB)]
            for p in range(16):
                r0, i0 = 16 * p, 16 * p + 8
                prev = None
                for c in range(NB):
                    accr = acci = pend = None
                    for a in range(c + 1):
                        b = c - a
                        xr = x_s[a, r0:r0 + 8, :]
                        xi = x_s[a, i0:i0 + 8, :]
                        hr = hf_s[b, r0:r0 + 8, :]
                        hi = hf_s[b, i0:i0 + 8, :]
                        if accr is None:
                            t1 = xr * hr
                            t2 = xr * hi
                            if last is not None:
                                t1 = jnp.where(fm, last[0], t1)
                                t2 = jnp.where(fm, last[1], t2)
                            accr = t1 - xi * hi
                            acci = t2 + xi * hr
                        elif short:
                            tr = xr * hr - xi * hi
                            ti = xr * hi + xi * hr
                            if pend is not None:
                                tr = tr + pend[0]
                                ti = ti + pend[1]
                                pend = None
                            elif a % mg == 1 and a < c:
                                pend = (tr, ti)
                                continue
                            accr = accr + tr
                            acci = acci + ti
                        else:
                            accr = (accr + xr * hr) - xi * hi
                            acci = (acci + xr * hi) + xi * hr
                    last = (accr, acci)
                    if prev is None:
                        yr, yi = accr, acci
                    else:
                        pr, pi = prev
                        yr, yi = (accr - pi, acci + pr) if p < 8 else (accr + pi, acci - pr)
                    prev = (accr, acci)
                    Y[c][p] = (yr, yi)
            return Y, last[0] + last[1]

        def conv_inv(j, Y):
            ic = inv_ref[0]
            isn = inv_ref[1]
            for c in range(NB):
                yr = jnp.concatenate([y[0] for y in Y[c]], axis=0).astype(bf16)
                yi = jnp.concatenate([y[1] for y in Y[c]], axis=0).astype(bf16)
                e = jnp.dot(ic, yr, preferred_element_type=f32)
                o = jnp.dot(isn, yi, preferred_element_type=f32)
                yp_s[j, c * P + 64:(c + 1) * P, :] = e - o
                lo = e + o
                for i in range(8):
                    yp_s[j, c * P + 8 * (7 - i):c * P + 8 * (8 - i), :] = lo[8 * i:8 * i + 8, :]

        def mlp_conv(i, short):
            r0 = M0 + i * M if isinstance(i, int) else pl.multiple_of(M0 + i * M, 64)
            Y, link = conv_mac(short)
            h = mm1(load_xn(r0, M))
            b2 = b2_row()
            c4 = D - 128
            o = jnp.dot(h, w2_s[:, :c4], preferred_element_type=f32)
            p_s[pl.ds(r0, M), :c4] = o * OSC + (q_s[pl.ds(r0, M), :c4].astype(f32) + b2[:, :c4])
            z = jnp.where(false_mask()[0:1, :], link[0:1, :], b2[:, c4:] * (1.0 / OSC))
            o = z + jnp.dot(h, w2_s[:, c4:], preferred_element_type=f32)
            p_s[pl.ds(r0, M), c4:] = o * OSC + q_s[pl.ds(r0, M), c4:].astype(f32)
            conv_inv(i, Y)

        rev8 = 7 - row8

        def load_y(j, t):
            y = yp_s[j, t:t + 8, :]
            if t % P < 64:
                y = jnp.take_along_axis(y, rev8, axis=0)
            return y

        def combine(r0, r1, st):
            fm = false_mask()
            for t in range(r0, r1, 16):
                for j in range(NL):
                    cs = slice(j * 128, (j + 1) * 128)
                    y = jnp.concatenate([load_y(j, t), load_y(j, t + 8)], axis=0)
                    p0 = p_s[t:t + 8, cs]
                    if st[0] is not None:
                        p0 = jnp.where(fm, st[0], p0)
                    pp = jnp.concatenate([p0, p_s[t + 8:t + 16, cs]], axis=0)
                    r = (pp + xn_s[j, t:t + 16, :].astype(f32) * y).astype(bf16)
                    st[0] = r.astype(f32)[0:8, :]
                    o_s[j, t:t + 16, :] = r

        wait(0)
        ln(0, qa, 0)
        wait(1)

        def r0a():
            bc_s[...] = jnp.broadcast_to(b1_row()[:, F - 128:F], (128, 128)).T[64:128, :]
            hid_s[0:qa, 0:w1c[1]] = mm1(load_xn(0, qa), 0, w1c[1])
        region(r0a)
        wait(2)

        def r0b():
            ln(qa, M0, 0)
            hid_s[qa:M0, 0:w1c[1]] = mm1(load_xn(qa, M0 - qa), 0, w1c[1])
        region(r0b)
        for i in range(1, n1):
            wait(2 + i)

            def r1(i=i):
                hid_s[:, w1c[i]:w1c[i + 1]] = mm1(load_xn(0, M0), w1c[i], w1c[i + 1])
            region(r1)
        wait(ng - 4)

        def r2a():
            ln(M0, M0 + lns, ln0)
            p_s[0:M0, :] = jnp.dot(hid_s[:, :w2k], w2_s[:w2k, :], preferred_element_type=f32)
        region(r2a)
        wait(ng - 3)

        def r2b():
            ln(M0 + lns, S, ln0)
            o = jnp.dot(hid_s[:, w2k:], w2_s[w2k:, :], preferred_element_type=f32) + p_s[0:M0, :]
            p_s[0:M0, :] = o * OSC + (q_s[0:M0, :].astype(f32) + b2_row())
            par = jnp.concatenate([sk_ref[...].astype(f32), dd_ref[...].astype(f32).reshape(1, D),
                                   jnp.zeros((3, D), f32)], axis=0)
            for j in range(NL):
                par_s[j] = par[:, j * 128:(j + 1) * 128]
            kv_fwd(0, par[:, 0:128])
        region(r2b)

        def pair(i, carry):
            si = lax.rem(ng - 2 + i, ring)
            for c in copies(kvh(2 * i + 1) + kvh(2 * i + 2), si):
                c.wait()
            mlp_conv(2 * i, False)
            kv_fwd(2 * i + 1, par_s[2 * i + 1])
            z = NB + flag_s[1]
            x_s[z, 0:8, :] = jnp.zeros((8, 128), f32)
            hf_s[z, 0:8, :] = jnp.zeros((8, 128), f32)
            mlp_conv(2 * i + 1, True)
            kv_fwd(2 * i + 2, par_s[2 * i + 2])
            return carry
        lax.fori_loop(0, 2, pair, 0)

        rl = S - ML

        def out_copies(js, r0, r1):
            return copies([(o_s.at[j, pl.ds(r0, r1 - r0), :], out_hbm.at[pl.ds(r0, r1 - r0), pl.ds(j * 128, 128)])
                           for j in js], sem_out)
        cuts = [0] + [int(rl // 16 * x) * 16 for x in prow] + [rl]
        g_o = [out_copies(range(NL), cuts[i], cuts[i + 1]) for i in range(nco)]
        g_fa = out_copies(range(osp), rl, S)
        g_fb = out_copies(range(osp, NL), rl, S)

        def pin_after(g, i):
            for c in g:
                c.start()
            z1 = pl.multiple_of(S + flag_s[1], 16)
            z2 = pl.multiple_of(S + flag_s[2], 16)
            o_s[0, pl.ds(z1, 16), :] = jnp.full((16, 128), i, bf16)
            return o_s[0, pl.ds(z2, 16), :].astype(f32)

        def last():
            mlp_conv(NL - 1, False)
            yp_s[NL + flag_s[1], 0:8, :] = jnp.zeros((8, 128), f32)
            p_s[pl.ds(pl.multiple_of(S + flag_s[1], 8), 8), 0:128] = jnp.zeros((8, 128), f32)
            xn = load_xn(rl, ML)
            st = [None]
            hs = []
            gi = 0
            for f in range(13):
                pin = None
                if gi < nco and pins[gi] == f:
                    combine(cuts[gi], cuts[gi + 1], st)
                    pin = pin_after(g_o[gi], gi)
                    gi += 1
                hs.append(mm1(xn, 128 * f, 128 * (f + 1), pin))
            hs.append(mm1_rem(xn))
            h = jnp.concatenate(hs, axis=1)
            b2 = b2_row() * (1.0 / OSC)
            for j in range(NL):
                cs = slice(j * 128, (j + 1) * 128)
                bj = b2[:, cs]
                if gi < nco and pins[gi] == 14 + j:
                    combine(cuts[gi], cuts[gi + 1], st)
                    bj = jnp.where(false_mask()[0:1, :], pin_after(g_o[gi], gi)[0:1, :], bj)
                    gi += 1
                if j == osp:
                    bj = jnp.where(false_mask()[0:1, :], pin_after(g_fa, nco)[0:1, :], bj)
                o = (bj + jnp.dot(h, w2_s[:, cs], preferred_element_type=f32)) * OSC + q_s[rl:S, cs].astype(f32)
                y = jnp.concatenate([load_y(j, t) for t in range(rl, S, 8)], axis=0)
                o_s[j, rl:S, :] = (o + xn_s[j, rl:S, :].astype(f32) * y).astype(bf16)
            assert gi == nco
        region(last)
        for c in g_fb:
            c.start()
        for g in g_o + [g_fa, g_fb]:
            for c in g:
                c.wait()

    fw, inv = dft_mats()

    @jax.jit
    def f(q, k, v, sk, h, dd, w1, b1, w2, b2):
        any_ = pl.BlockSpec(memory_space=pl.ANY)
        out = pl.pallas_call(
            kernel,
            in_specs=[any_] * 12,
            out_specs=any_,
            out_shape=jax.ShapeDtypeStruct((S, D), bf16),
            scratch_shapes=[
                pltpu.VMEM((S, D), bf16),
                pltpu.VMEM((NL, S + KP, 128), bf16),
                pltpu.VMEM((NL, S, 128), bf16),
                pltpu.VMEM((NL, 128, S), bf16),
                pltpu.VMEM((F, D), bf16),
                pltpu.VMEM((F, D), bf16),
                pltpu.VMEM((NL, S, 128), bf16),
                pltpu.VMEM((S + 8, D), f32),
                pltpu.VMEM((NB + 1, 256, 128), f32),
                pltpu.VMEM((NB + 1, 256, 128), f32),
                pltpu.VMEM((NL + 1, S, 128), f32),
                pltpu.VMEM((NL, S + 16, 128), bf16),
                pltpu.VMEM((NL, 8, 128), f32),
                pltpu.VMEM((M0, F), bf16),
                pltpu.VMEM((4, D), bf16), pltpu.VMEM((D,), bf16), pltpu.VMEM((F,), bf16), pltpu.VMEM((D,), bf16),
                pltpu.VMEM((2, 256, 128), bf16), pltpu.VMEM((2, 64, 128), bf16),
                pltpu.VMEM((64, 128), f32),
                pltpu.SMEM((4,), jnp.int32),
                pltpu.SemaphoreType.DMA((ring if ring < 9 else 10,)),
            ],
            compiler_params=pltpu.CompilerParams(vmem_limit_bytes=100 * 2**20),
            name=name,
        )(q.reshape(S, D), k.reshape(S, D), v.reshape(S, D), sk.T, h, dd, w1.T, b1, w2, b2, fw, inv)
        return out.reshape(1, S, D)
    return f


_impl = make(name="fused_h3_mlp")


@jax.jit
def pallas_parallel_sum__ssm_conv_h3__dense_activation_gelu__prompt_kernel(
    A_q, A_k, A_v, A_shift_k, A_ssm_k, A_ssm_D, B_x, B_w1, B_b1, B_w2, B_b2,
):
    del B_x
    return _impl(A_q, A_k, A_v, A_shift_k, A_ssm_k, A_ssm_D, B_w1, B_b1, B_w2, B_b2)
```

```python
import numpy as np
import jax
import jax.numpy as jnp
from jax import lax
import jax.experimental.pallas as pl
import jax.experimental.pallas.tpu as pltpu

S, D, F = 2048, 640, 1728
P = 128
NB = S // P
NL = D // 128
KP = 64
FR = F - 64
f32, bf16, u32 = jnp.float32, jnp.bfloat16, jnp.uint32
NT = (((1,), (1,)), ((), ()))

ALPHA = (0.7978845608028654 * 0.044715) ** (1.0 / 3.0)
C1 = 0.7978845608028654 / ALPHA
OSC = 0.5 / ALPHA


def dft_mats():
    ks = np.concatenate([np.arange(0, 128, 2), np.arange(1, 128, 2)])
    n = np.arange(128)
    m = np.arange(64) + 0.5
    fw = np.zeros((2, 256, 128))
    inv = np.zeros((2, 64, 128))
    for p in range(16):
        for s in range(8):
            w = 2 * np.pi * (ks[8 * p + s] + 0.5) / 256
            fw[0, 16 * p + s] = np.cos(w * (n - 63.5))
            fw[0, 16 * p + 8 + s] = -np.sin(w * (n - 63.5))
            fw[1, 16 * p + s] = np.cos(w * n)
            fw[1, 16 * p + 8 + s] = -np.sin(w * n)
            inv[0, :, 8 * p + s] = np.cos(w * m) / (128 * ALPHA)
            inv[1, :, 8 * p + s] = np.sin(w * m) / (128 * ALPHA)
    perm = np.concatenate(
        [16 * t + np.concatenate([np.arange(0, 16, 2), np.arange(1, 16, 2)]) for t in range(8)])
    fw[0] = fw[0][:, perm]
    return fw.astype(np.float32).astype(bf16), inv.astype(np.float32).astype(bf16)


def gelu(g):
    return g * (1.0 + jnp.tanh(g * (C1 + g * g)))


def make(M0=576, M=256, name="v27", kvn=2, qa=256, w1c=(0, 256, 768, F), w2k=896, lns=832, ln0=2,
         pins=(2, 7, 12, 15), prow=(0.01, 0.28, 0.6), osp=4, lag=4, mg=3, ring=4, lnk=True, lag0=4, pf=16, pfm=2, rl2=False, rpos=None, lnb=0, bsp=()):
    ML = S - M0 - NL * M
    assert ML > 0 and ML % 16 == 0 and M0 % 64 == 0 and M % 64 == 0
    n1, nco = len(w1c) - 1, len(pins)

    def kernel(q_hbm, k_hbm, v_hbm, sk_hbm, h_hbm, dd_hbm, w1_hbm, b1_hbm, w2_hbm, b2_hbm, fw_hbm, inv_hbm,
               out_hbm,
               q_s, k_s, v_s, h_s, w1_s, w2_s, xn_s, p_s, x_s, hf_s, yp_s, o_s, par_s, hid_s,
               sk_ref, dd_ref, b1_ref, b2_ref, fw_ref, inv_ref, bc_s, flag_s, sem):
        def rows(src, dst, r0, r1):
            return (src.at[pl.ds(r0, r1 - r0)], dst.at[pl.ds(r0, r1 - r0)])

        def kvh(j):
            lane = pl.ds(j * 128, 128) if isinstance(j, int) else pl.ds(pl.multiple_of(j * 128, 128), 128)
            return [(h_hbm.at[lane, :], h_s.at[j]),
                    (k_hbm.at[:, lane], k_s.at[j, pl.ds(KP, S), :]),
                    (v_hbm.at[:, lane], v_s.at[j])]

        def copies(g, si):
            return [pltpu.make_async_copy(src, dst, sem.at[si]) for src, dst in g]

        groups = [[rows(q_hbm, q_s, 0, qa)],
                  [rows(w1_hbm, w1_s, 0, w1c[1]), (b1_hbm, b1_ref)],
                  [rows(q_hbm, q_s, qa, M0)]]
        groups += [[rows(w1_hbm, w1_s, w1c[i], w1c[i + 1])] for i in range(1, n1)]
        groups += [[rows(q_hbm, q_s, M0, S), rows(w2_hbm, w2_s, 0, w2k)],
                   [rows(w2_hbm, w2_s, w2k, F), (b2_hbm, b2_ref), (sk_hbm, sk_ref), (dd_hbm, dd_ref),
                    (fw_hbm, fw_ref), (inv_hbm, inv_ref)] + kvh(0),
                   kvh(1) + kvh(2), kvh(3) + kvh(4)]
        ng = len(groups)
        sem_out = (ng - 3) % ring if ring < ng else ng

        def start(g):
            if g < ng:
                for c in copies(groups[g], g % ring):
                    c.start()

        def wait(g):
            for c in copies(groups[g], g % ring):
                c.wait()
            start(g + ring)

        for g in range(ring):
            start(g)

        flag_s[0] = 100
        flag_s[1] = 0
        flag_s[2] = 0
        for j in range(NL):
            k_s[j, KP - 16:KP, :] = jnp.zeros((16, 128), bf16)
        ku_s = k_s.bitcast(u32)
        vu_s = v_s.bitcast(u32)

        def region(fn):
            pl.when(flag_s[0] == 100)(fn)

        row8 = lax.broadcasted_iota(jnp.int32, (8, 128), 0)

        def false_mask():
            return row8 > flag_s[0]

        def ln(r0, r1, n):
            fm = lax.broadcasted_iota(jnp.int32, (16, 1), 0) > flag_s[0]
            lasts = [None] * max(n, 1)
            for t, rr in enumerate(range(r0, r1, 16)):
                x = q_s[rr:rr + 16, :].astype(f32)
                sm = jnp.sum(x, axis=-1, keepdims=True)
                ci = t % max(n, 1)
                if n and lasts[ci] is not None:
                    sm = jnp.where(fm, lasts[ci], sm)
                xc = x - sm * (1.0 / D)
                var = jnp.sum(xc * xc, axis=-1, keepdims=True) * (1.0 / D)
                rs = lax.rsqrt(var + 1e-5) * ALPHA
                lasts[ci] = rs
                xo = xc * rs
                for j in range(NL):
                    xn_s[j, rr:rr + 16, :] = xo[:, j * 128:(j + 1) * 128].astype(bf16)
            return lasts

        def load_xn(r0, m):
            return jnp.concatenate([xn_s[j, pl.ds(r0, m), :] for j in range(NL)], axis=1)

        def b1_row():
            return b1_ref[...].astype(f32).reshape(1, F) * ALPHA

        def b2_row():
            return b2_ref[...].astype(f32).reshape(1, D)

        def mm1_rem(xn):
            m = xn.shape[0]
            ht = lax.dot_general(w1_s[FR:F, :], xn, NT, preferred_element_type=f32)
            bc = bc_s[...]
            outs = []
            for c0 in range(0, m, 128):
                c1 = min(c0 + 128, m)
                outs.append(gelu(ht[:, c0:c1] + bc[:, :c1 - c0]).T)
            return jnp.concatenate(outs, axis=0)

        def mm1(xn, f0=0, f1=F, pin=None):
            if f1 == F:
                hr = mm1_rem(xn)
                if f0 == FR:
                    return hr
                return jnp.concatenate([mm1(xn, f0, FR, pin), hr], axis=1)
            b1 = b1_row()[:, f0:f1]
            if pin is not None:
                b1 = jnp.where(false_mask()[0:1, :f1 - f0], pin[0:1, :f1 - f0], b1)
            h = lax.dot_general(xn, w1_s[f0:f1, :], NT, preferred_element_type=f32) + b1
            return gelu(h)

        def kv_fwd(j, sk, init=None, lag=lag):
            s = [jnp.broadcast_to(sk[l:l + 1, :], (8, 128)) for l in range(4)]
            dd = sk[4:5, :]
            fm = false_mask()
            lasts = [init] * kvn
            fwx = fw_ref[0]
            fwh = fw_ref[1]
            ev = lambda w: pltpu.bitcast(w << 16, f32)
            od = lambda w: pltpu.bitcast(w & jnp.uint32(0xffff0000), f32)
            kvs = []
            for a in range(NB + lag):
                if a < NB:
                    outs = []
                    for t in range(a * 8, a * 8 + 8):
                        bb = KP // 2 + 8 * t
                        w0 = ku_s[j, bb:bb + 8, :]
                        w1 = ku_s[j, bb - 1:bb + 7, :]
                        w2 = ku_s[j, bb - 2:bb + 6, :]
                        wv = vu_s[j, 8 * t:8 * t + 8, :]
                        e0, o0, e1, o1, o2 = ev(w0), od(w0), ev(w1), od(w1), od(w2)
                        ci = t % kvn
                        if lasts[ci] is not None:
                            e0 = jnp.where(fm, lasts[ci], e0)
                        oe = (e0 * s[0] + o1 * s[1] + e1 * s[2] + o2 * s[3]) * ev(wv)
                        oo = (e0 * s[1] + o0 * s[0] + o1 * s[2] + e1 * s[3]) * od(wv)
                        lasts[ci] = oo
                        outs += [oe, oo]
                    kvs.append(jnp.concatenate(outs, axis=0).astype(bf16))
                    hb = lax.dot_general(fwh, h_s[j, :, a * P:(a + 1) * P], NT, preferred_element_type=f32)
                    if a == 0:
                        hb = jnp.concatenate(
                            [hb[8 * t:8 * t + 8, :] + dd if t % 2 == 0 else hb[8 * t:8 * t + 8, :]
                             for t in range(32)], axis=0)
                    hf_s[a] = hb
                if a >= lag:
                    x_s[a - lag] = jnp.dot(fwx, kvs[a - lag], preferred_element_type=f32)

        def conv_mac(short):
            fm = false_mask()
            last = None
            Y = [[None] * 16 for _ in range(NB)]
            for p in range(16):
                r0, i0 = 16 * p, 16 * p + 8
                prev = None
                for c in range(NB):
                    accr = acci = pend = None
                    for a in range(c + 1):
                        b = c - a
                        xr = x_s[a, r0:r0 + 8, :]
                        xi = x_s[a, i0:i0 + 8, :]
                        hr = hf_s[b, r0:r0 + 8, :]
                        hi = hf_s[b, i0:i0 + 8, :]
                        if accr is None:
                            t1 = xr * hr
                            t2 = xr * hi
                            if last is not None:
                                t1 = jnp.where(fm, last[0], t1)
                                t2 = jnp.where(fm, last[1], t2)
                            accr = t1 - xi * hi
                            acci = t2 + xi * hr
                        elif short:
                            tr = xr * hr - xi * hi
                            ti = xr * hi + xi * hr
                            if pend is not None:
                                tr = tr + pend[0]
                                ti = ti + pend[1]
                                pend = None
                            elif a % mg == 1 and a < c:
                                pend = (tr, ti)
                                continue
                            accr = accr + tr
                            acci = acci + ti
                        elif p >= pf and a % pfm == pfm - 1:
                            accr = accr + (xr * hr - xi * hi)
                            acci = acci + (xr * hi + xi * hr)
                        else:
                            accr = (accr + xr * hr) - xi * hi
                            acci = (acci + xr * hi) + xi * hr
                    last = (accr, acci)
                    if prev is None:
                        yr, yi = accr, acci
                    else:
                        pr, pi = prev
                        yr, yi = (accr - pi, acci + pr) if p < 8 else (accr + pi, acci - pr)
                    prev = (accr, acci)
                    Y[c][p] = (yr, yi)
            return Y, last[0] + last[1]

        def conv_inv(j, Y):
            ic = inv_ref[0]
            isn = inv_ref[1]
            for c in range(NB):
                yr = jnp.concatenate([y[0] for y in Y[c]], axis=0).astype(bf16)
                yi = jnp.concatenate([y[1] for y in Y[c]], axis=0).astype(bf16)
                e = jnp.dot(ic, yr, preferred_element_type=f32)
                o = jnp.dot(isn, yi, preferred_element_type=f32)
                yp_s[j, c * P + 64:(c + 1) * P, :] = e - o
                lo = e + o
                for i in range(8):
                    yp_s[j, c * P + 8 * (7 - i):c * P + 8 * (8 - i), :] = lo[8 * i:8 * i + 8, :]

        def mlp_conv(i, short):
            r0 = M0 + i * M if isinstance(i, int) else pl.multiple_of(M0 + i * M, 64)
            Y, link = conv_mac(short)
            xn = load_xn(r0, M)
            if rpos is not None and (short or rl2):
                ha = mm1(xn, 0, 128 * rpos)
                hr = mm1_rem(xn)
                h = jnp.concatenate([ha, mm1(xn, 128 * rpos, FR), hr] if rpos < 13 else [ha, hr], axis=1)
            else:
                h = mm1(xn)
            h = h.astype(bf16)
            b2 = b2_row()
            c4 = D - 128
            o = jnp.dot(h, w2_s[:, :c4], preferred_element_type=f32)
            p_s[pl.ds(r0, M), :c4] = o * OSC + (q_s[pl.ds(r0, M), :c4].astype(f32) + b2[:, :c4])
            z = jnp.where(false_mask()[0:1, :], link[0:1, :], b2[:, c4:] * (1.0 / OSC))
            o = z + jnp.dot(h, w2_s[:, c4:], preferred_element_type=f32)
            p_s[pl.ds(r0, M), c4:] = o * OSC + q_s[pl.ds(r0, M), c4:].astype(f32)
            conv_inv(i, Y)

        rev8 = 7 - row8

        def load_y(j, t):
            y = yp_s[j, t:t + 8, :]
            if t % P < 64:
                y = jnp.take_along_axis(y, rev8, axis=0)
            return y

        def combine(r0, r1, st):
            fm = false_mask()
            for t in range(r0, r1, 16):
                for j in range(NL):
                    cs = slice(j * 128, (j + 1) * 128)
                    y = jnp.concatenate([load_y(j, t), load_y(j, t + 8)], axis=0)
                    p0 = p_s[t:t + 8, cs]
                    if st[0] is not None:
                        p0 = jnp.where(fm, st[0], p0)
                    pp = jnp.concatenate([p0, p_s[t + 8:t + 16, cs]], axis=0)
                    r = (pp + xn_s[j, t:t + 16, :].astype(f32) * y).astype(bf16)
                    st[0] = r.astype(f32)[0:8, :]
                    o_s[j, t:t + 16, :] = r

        wait(0)
        ln(0, qa, 0)
        wait(1)

        def r0a():
            bc_s[...] = jnp.broadcast_to(b1_row()[:, F - 128:F], (128, 128)).T[64:128, :]
            hid_s[0:qa, 0:w1c[1]] = mm1(load_xn(0, qa), 0, w1c[1]).astype(bf16)
        region(r0a)
        wait(2)

        def r0b():
            ln(qa, M0, lnb)
            cs = [qa] + [qa + x for x in bsp] + [M0]
            for a_, b_ in zip(cs[:-1], cs[1:]):
                hid_s[a_:b_, 0:w1c[1]] = mm1(load_xn(a_, b_ - a_), 0, w1c[1]).astype(bf16)
        region(r0b)
        for i in range(1, n1):
            wait(2 + i)

            def r1(i=i):
                hid_s[:, w1c[i]:w1c[i + 1]] = mm1(load_xn(0, M0), w1c[i], w1c[i + 1]).astype(bf16)
            region(r1)
        wait(ng - 4)

        def r2a():
            ln(M0, M0 + lns, ln0)
            p_s[0:M0, :] = jnp.dot(hid_s[:, :w2k], w2_s[:w2k, :], preferred_element_type=f32)
        region(r2a)
        wait(ng - 3)

        def r2b():
            lk = ln(M0 + lns, S, ln0)
            t = lk[0]
            for u in lk[1:]:
                t = t + u
            lk = jnp.broadcast_to(t[0:8, :], (8, 128)) if lnk else None
            o = jnp.dot(hid_s[:, w2k:], w2_s[w2k:, :], preferred_element_type=f32) + p_s[0:M0, :]
            p_s[0:M0, :] = o * OSC + (q_s[0:M0, :].astype(f32) + b2_row())
            par = jnp.concatenate([sk_ref[...].astype(f32), dd_ref[...].astype(f32).reshape(1, D),
                                   jnp.zeros((3, D), f32)], axis=0)
            for j in range(NL):
                par_s[j] = par[:, j * 128:(j + 1) * 128]
            kv_fwd(0, par[:, 0:128], lk, lag0)
        region(r2b)

        def pair(i, carry):
            si = lax.rem(ng - 2 + i, ring)
            for c in copies(kvh(2 * i + 1) + kvh(2 * i + 2), si):
                c.wait()
            mlp_conv(2 * i, False)
            kv_fwd(2 * i + 1, par_s[2 * i + 1])
            z = NB + flag_s[1]
            x_s[z, 0:8, :] = jnp.zeros((8, 128), f32)
            hf_s[z, 0:8, :] = jnp.zeros((8, 128), f32)
            mlp_conv(2 * i + 1, True)
            kv_fwd(2 * i + 2, par_s[2 * i + 2])
            return carry
        lax.fori_loop(0, 2, pair, 0)

        rl = S - ML

        def out_copies(js, r0, r1):
            return copies([(o_s.at[j, pl.ds(r0, r1 - r0), :], out_hbm.at[pl.ds(r0, r1 - r0), pl.ds(j * 128, 128)])
                           for j in js], sem_out)
        cuts = [0] + [int(rl // 16 * x) * 16 for x in prow] + [rl]
        g_o = [out_copies(range(NL), cuts[i], cuts[i + 1]) for i in range(nco)]
        g_fa = out_copies(range(osp), rl, S)
        g_fb = out_copies(range(osp, NL), rl, S)

        def pin_after(g, i):
            for c in g:
                c.start()
            z1 = pl.multiple_of(S + flag_s[1], 16)
            z2 = pl.multiple_of(S + flag_s[2], 16)
            o_s[0, pl.ds(z1, 16), :] = jnp.full((16, 128), i, bf16)
            return o_s[0, pl.ds(z2, 16), :].astype(f32)

        def last():
            mlp_conv(NL - 1, False)
            yp_s[NL + flag_s[1], 0:8, :] = jnp.zeros((8, 128), f32)
            p_s[pl.ds(pl.multiple_of(S + flag_s[1], 8), 8), 0:128] = jnp.zeros((8, 128), f32)
            xn = load_xn(rl, ML)
            st = [None]
            hs = []
            gi = 0
            for f in range(13):
                pin = None
                if gi < nco and pins[gi] == f:
                    combine(cuts[gi], cuts[gi + 1], st)
                    pin = pin_after(g_o[gi], gi)
                    gi += 1
                hs.append(mm1(xn, 128 * f, 128 * (f + 1), pin))
            hs.append(mm1_rem(xn))
            h = jnp.concatenate(hs, axis=1).astype(bf16)
            b2 = b2_row() * (1.0 / OSC)
            for j in range(NL):
                cs = slice(j * 128, (j + 1) * 128)
                bj = b2[:, cs]
                if gi < nco and pins[gi] == 14 + j:
                    combine(cuts[gi], cuts[gi + 1], st)
                    bj = jnp.where(false_mask()[0:1, :], pin_after(g_o[gi], gi)[0:1, :], bj)
                    gi += 1
                if j == osp:
                    bj = jnp.where(false_mask()[0:1, :], pin_after(g_fa, nco)[0:1, :], bj)
                o = (bj + jnp.dot(h, w2_s[:, cs], preferred_element_type=f32)) * OSC + q_s[rl:S, cs].astype(f32)
                y = jnp.concatenate([load_y(j, t) for t in range(rl, S, 8)], axis=0)
                o_s[j, rl:S, :] = (o + xn_s[j, rl:S, :].astype(f32) * y).astype(bf16)
            assert gi == nco
        region(last)
        for c in g_fb:
            c.start()
        for g in g_o + [g_fa, g_fb]:
            for c in g:
                c.wait()

    fw, inv = dft_mats()

    @jax.jit
    def f(q, k, v, sk, h, dd, w1, b1, w2, b2):
        any_ = pl.BlockSpec(memory_space=pl.ANY)
        out = pl.pallas_call(
            kernel,
            in_specs=[any_] * 12,
            out_specs=any_,
            out_shape=jax.ShapeDtypeStruct((S, D), bf16),
            scratch_shapes=[
                pltpu.VMEM((S, D), bf16),
                pltpu.VMEM((NL, S + KP, 128), bf16),
                pltpu.VMEM((NL, S, 128), bf16),
                pltpu.VMEM((NL, 128, S), bf16),
                pltpu.VMEM((F, D), bf16),
                pltpu.VMEM((F, D), bf16),
                pltpu.VMEM((NL, S, 128), bf16),
                pltpu.VMEM((S + 8, D), f32),
                pltpu.VMEM((NB + 1, 256, 128), f32),
                pltpu.VMEM((NB + 1, 256, 128), f32),
                pltpu.VMEM((NL + 1, S, 128), f32),
                pltpu.VMEM((NL, S + 16, 128), bf16),
                pltpu.VMEM((NL, 8, 128), f32),
                pltpu.VMEM((M0, F), bf16),
                pltpu.VMEM((4, D), bf16), pltpu.VMEM((D,), bf16), pltpu.VMEM((F,), bf16), pltpu.VMEM((D,), bf16),
                pltpu.VMEM((2, 256, 128), bf16), pltpu.VMEM((2, 64, 128), bf16),
                pltpu.VMEM((64, 128), f32),
                pltpu.SMEM((4,), jnp.int32),
                pltpu.SemaphoreType.DMA((ring if ring < 9 else 10,)),
            ],
            compiler_params=pltpu.CompilerParams(vmem_limit_bytes=100 * 2**20),
            name=name,
        )(q.reshape(S, D), k.reshape(S, D), v.reshape(S, D), sk.T, h, dd, w1.T, b1, w2, b2, fw, inv)
        return out.reshape(1, S, D)
    return f


_impl = make(name="fused_h3_mlp", rpos=4, osp=3)


@jax.jit
def pallas_parallel_sum__ssm_conv_h3__dense_activation_gelu__prompt_kernel(
    A_q, A_k, A_v, A_shift_k, A_ssm_k, A_ssm_D, B_x, B_w1, B_b1, B_w2, B_b2,
):
    del B_x
    return _impl(A_q, A_k, A_v, A_shift_k, A_ssm_k, A_ssm_D, B_w1, B_b1, B_w2, B_b2)
```

```python
import numpy as np
import jax
import jax.numpy as jnp
from jax import lax
import jax.experimental.pallas as pl
import jax.experimental.pallas.tpu as pltpu

S, D, F = 2048, 640, 1728
P = 128
NB = S // P
NL = D // 128
KP = 64
FR = F - 64
f32, bf16, u32 = jnp.float32, jnp.bfloat16, jnp.uint32
NT = (((1,), (1,)), ((), ()))

ALPHA = (0.7978845608028654 * 0.044715) ** (1.0 / 3.0)
C1 = 0.7978845608028654 / ALPHA
OSC = 0.5 / ALPHA


def dft_mats():
    ks = np.concatenate([np.arange(0, 128, 2), np.arange(1, 128, 2)])
    n = np.arange(128)
    m = np.arange(64) + 0.5
    fw = np.zeros((2, 256, 128))
    inv = np.zeros((2, 64, 128))
    for p in range(16):
        for s in range(8):
            w = 2 * np.pi * (ks[8 * p + s] + 0.5) / 256
            fw[0, 16 * p + s] = np.cos(w * (n - 63.5))
            fw[0, 16 * p + 8 + s] = -np.sin(w * (n - 63.5))
            fw[1, 16 * p + s] = np.cos(w * n)
            fw[1, 16 * p + 8 + s] = -np.sin(w * n)
            inv[0, :, 8 * p + s] = np.cos(w * m) / (128 * ALPHA)
            inv[1, :, 8 * p + s] = np.sin(w * m) / (128 * ALPHA)
    perm = np.concatenate(
        [16 * t + np.concatenate([np.arange(0, 16, 2), np.arange(1, 16, 2)]) for t in range(8)])
    fw[0] = fw[0][:, perm]
    return fw.astype(np.float32).astype(bf16), inv.astype(np.float32).astype(bf16)


def gelu(g):
    return g * (1.0 + jnp.tanh(g * (C1 + g * g)))


def make(M0=576, M=256, name="v36", kvn=2, qa=256, w1c=(0, 256, 768, F), w2k=1024, lns=960, ln0=2,
         pins=(2, 7, 12, 15), prow=(0.01, 0.28, 0.6), osp=3, lag=4, mg=3, ring=4, lnk=True, lag0=4, pf=16, pfm=2, rl2=False, rpos=4, lnb=0, bsp=()):
    ML = S - M0 - NL * M
    assert ML > 0 and ML % 16 == 0 and M0 % 64 == 0 and M % 64 == 0
    n1, nco = len(w1c) - 1, len(pins)

    def kernel(q_hbm, k_hbm, v_hbm, sk_hbm, h_hbm, dd_hbm, w1_hbm, b1_hbm, w2_hbm, b2_hbm, fw_hbm, inv_hbm,
               out_hbm,
               q_s, k_s, v_s, h_s, w1_s, w2_s, xn_s, p_s, x_s, hf_s, yp_s, o_s, par_s, hid_s,
               sk_ref, dd_ref, b1_ref, b2_ref, fw_ref, inv_ref, bc_s, flag_s, sem):
        def rows(src, dst, r0, r1):
            return (src.at[pl.ds(r0, r1 - r0)], dst.at[pl.ds(r0, r1 - r0)])

        def kvh(j):
            lane = pl.ds(j * 128, 128) if isinstance(j, int) else pl.ds(pl.multiple_of(j * 128, 128), 128)
            return [(h_hbm.at[lane, :], h_s.at[j]),
                    (k_hbm.at[:, lane], k_s.at[j, pl.ds(KP, S), :]),
                    (v_hbm.at[:, lane], v_s.at[j])]

        def copies(g, si):
            return [pltpu.make_async_copy(src, dst, sem.at[si]) for src, dst in g]

        groups = [[rows(q_hbm, q_s, 0, qa)],
                  [rows(w1_hbm, w1_s, 0, w1c[1]), (b1_hbm, b1_ref)],
                  [rows(q_hbm, q_s, qa, M0)]]
        groups += [[rows(w1_hbm, w1_s, w1c[i], w1c[i + 1])] for i in range(1, n1)]
        groups += [[rows(q_hbm, q_s, M0, M0 + lns), rows(w2_hbm, w2_s, 0, w2k)],
                   [rows(q_hbm, q_s, M0 + lns, S), rows(w2_hbm, w2_s, w2k, F), (b2_hbm, b2_ref), (sk_hbm, sk_ref), (dd_hbm, dd_ref),
                    (fw_hbm, fw_ref), (inv_hbm, inv_ref)] + kvh(0),
                   kvh(1) + kvh(2), kvh(3) + kvh(4)]
        ng = len(groups)
        sem_out = (ng - 3) % ring if ring < ng else ng

        def start(g):
            if g < ng:
                for c in copies(groups[g], g % ring):
                    c.start()

        def wait(g):
            for c in copies(groups[g], g % ring):
                c.wait()
            start(g + ring)

        for g in range(ring):
            start(g)

        flag_s[0] = 100
        flag_s[1] = 0
        flag_s[2] = 0
        for j in range(NL):
            k_s[j, KP - 16:KP, :] = jnp.zeros((16, 128), bf16)
        ku_s = k_s.bitcast(u32)
        vu_s = v_s.bitcast(u32)

        def region(fn):
            pl.when(flag_s[0] == 100)(fn)

        row8 = lax.broadcasted_iota(jnp.int32, (8, 128), 0)

        def false_mask():
            return row8 > flag_s[0]

        def ln(r0, r1, n):
            fm = lax.broadcasted_iota(jnp.int32, (16, 1), 0) > flag_s[0]
            lasts = [None] * max(n, 1)
            for t, rr in enumerate(range(r0, r1, 16)):
                x = q_s[rr:rr + 16, :].astype(f32)
                sm = jnp.sum(x, axis=-1, keepdims=True)
                ci = t % max(n, 1)
                if n and lasts[ci] is not None:
                    sm = jnp.where(fm, lasts[ci], sm)
                xc = x - sm * (1.0 / D)
                var = jnp.sum(xc * xc, axis=-1, keepdims=True) * (1.0 / D)
                rs = lax.rsqrt(var + 1e-5) * ALPHA
                lasts[ci] = rs
                xo = xc * rs
                for j in range(NL):
                    xn_s[j, rr:rr + 16, :] = xo[:, j * 128:(j + 1) * 128].astype(bf16)
            return lasts

        def load_xn(r0, m):
            return jnp.concatenate([xn_s[j, pl.ds(r0, m), :] for j in range(NL)], axis=1)

        def b1_row():
            return b1_ref[...].astype(f32).reshape(1, F) * ALPHA

        def b2_row():
            return b2_ref[...].astype(f32).reshape(1, D)

        def mm1_rem(xn):
            m = xn.shape[0]
            ht = lax.dot_general(w1_s[FR:F, :], xn, NT, preferred_element_type=f32)
            bc = bc_s[...]
            outs = []
            for c0 in range(0, m, 128):
                c1 = min(c0 + 128, m)
                outs.append(gelu(ht[:, c0:c1] + bc[:, :c1 - c0]).T)
            return jnp.concatenate(outs, axis=0)

        def mm1(xn, f0=0, f1=F, pin=None):
            if f1 == F:
                hr = mm1_rem(xn)
                if f0 == FR:
                    return hr
                return jnp.concatenate([mm1(xn, f0, FR, pin), hr], axis=1)
            b1 = b1_row()[:, f0:f1]
            if pin is not None:
                b1 = jnp.where(false_mask()[0:1, :f1 - f0], pin[0:1, :f1 - f0], b1)
            h = lax.dot_general(xn, w1_s[f0:f1, :], NT, preferred_element_type=f32) + b1
            return gelu(h)

        def kv_fwd(j, sk, init=None, lag=lag):
            s = [jnp.broadcast_to(sk[l:l + 1, :], (8, 128)) for l in range(4)]
            dd = sk[4:5, :]
            fm = false_mask()
            lasts = [init] * kvn
            fwx = fw_ref[0]
            fwh = fw_ref[1]
            ev = lambda w: pltpu.bitcast(w << 16, f32)
            od = lambda w: pltpu.bitcast(w & jnp.uint32(0xffff0000), f32)
            kvs = []
            for a in range(NB + lag):
                if a < NB:
                    outs = []
                    for t in range(a * 8, a * 8 + 8):
                        bb = KP // 2 + 8 * t
                        w0 = ku_s[j, bb:bb + 8, :]
                        w1 = ku_s[j, bb - 1:bb + 7, :]
                        w2 = ku_s[j, bb - 2:bb + 6, :]
                        wv = vu_s[j, 8 * t:8 * t + 8, :]
                        e0, o0, e1, o1, o2 = ev(w0), od(w0), ev(w1), od(w1), od(w2)
                        ci = t % kvn
                        if lasts[ci] is not None:
                            e0 = jnp.where(fm, lasts[ci], e0)
                        oe = (e0 * s[0] + o1 * s[1] + e1 * s[2] + o2 * s[3]) * ev(wv)
                        oo = (e0 * s[1] + o0 * s[0] + o1 * s[2] + e1 * s[3]) * od(wv)
                        lasts[ci] = oo
                        outs += [oe, oo]
                    kvs.append(jnp.concatenate(outs, axis=0).astype(bf16))
                    hb = lax.dot_general(fwh, h_s[j, :, a * P:(a + 1) * P], NT, preferred_element_type=f32)
                    if a == 0:
                        hb = jnp.concatenate(
                            [hb[8 * t:8 * t + 8, :] + dd if t % 2 == 0 else hb[8 * t:8 * t + 8, :]
                             for t in range(32)], axis=0)
                    hf_s[a] = hb
                if a >= lag:
                    x_s[a - lag] = jnp.dot(fwx, kvs[a - lag], preferred_element_type=f32)

        def conv_mac(short):
            fm = false_mask()
            last = None
            Y = [[None] * 16 for _ in range(NB)]
            for p in range(16):
                r0, i0 = 16 * p, 16 * p + 8
                prev = None
                for c in range(NB):
                    accr = acci = pend = None
                    for a in range(c + 1):
                        b = c - a
                        xr = x_s[a, r0:r0 + 8, :]
                        xi = x_s[a, i0:i0 + 8, :]
                        hr = hf_s[b, r0:r0 + 8, :]
                        hi = hf_s[b, i0:i0 + 8, :]
                        if accr is None:
                            t1 = xr * hr
                            t2 = xr * hi
                            if last is not None:
                                t1 = jnp.where(fm, last[0], t1)
                                t2 = jnp.where(fm, last[1], t2)
                            accr = t1 - xi * hi
                            acci = t2 + xi * hr
                        elif short:
                            tr = xr * hr - xi * hi
                            ti = xr * hi + xi * hr
                            if pend is not None:
                                tr = tr + pend[0]
                                ti = ti + pend[1]
                                pend = None
                            elif a % mg == 1 and a < c:
                                pend = (tr, ti)
                                continue
                            accr = accr + tr
                            acci = acci + ti
                        elif p >= pf and a % pfm == pfm - 1:
                            accr = accr + (xr * hr - xi * hi)
                            acci = acci + (xr * hi + xi * hr)
                        else:
                            accr = (accr + xr * hr) - xi * hi
                            acci = (acci + xr * hi) + xi * hr
                    last = (accr, acci)
                    if prev is None:
                        yr, yi = accr, acci
                    else:
                        pr, pi = prev
                        yr, yi = (accr - pi, acci + pr) if p < 8 else (accr + pi, acci - pr)
                    prev = (accr, acci)
                    Y[c][p] = (yr, yi)
            return Y, last[0] + last[1]

        def conv_inv(j, Y):
            ic = inv_ref[0]
            isn = inv_ref[1]
            for c in range(NB):
                yr = jnp.concatenate([y[0] for y in Y[c]], axis=0).astype(bf16)
                yi = jnp.concatenate([y[1] for y in Y[c]], axis=0).astype(bf16)
                e = jnp.dot(ic, yr, preferred_element_type=f32)
                o = jnp.dot(isn, yi, preferred_element_type=f32)
                yp_s[j, c * P + 64:(c + 1) * P, :] = e - o
                lo = e + o
                for i in range(8):
                    yp_s[j, c * P + 8 * (7 - i):c * P + 8 * (8 - i), :] = lo[8 * i:8 * i + 8, :]

        def mlp_conv(i, short):
            r0 = M0 + i * M if isinstance(i, int) else pl.multiple_of(M0 + i * M, 64)
            Y, link = conv_mac(short)
            xn = load_xn(r0, M)
            if rpos is not None and (short or rl2):
                ha = mm1(xn, 0, 128 * rpos)
                hr = mm1_rem(xn)
                h = jnp.concatenate([ha, mm1(xn, 128 * rpos, FR), hr] if rpos < 13 else [ha, hr], axis=1)
            else:
                h = mm1(xn)
            h = h.astype(bf16)
            b2 = b2_row()
            c4 = D - 128
            o = jnp.dot(h, w2_s[:, :c4], preferred_element_type=f32)
            p_s[pl.ds(r0, M), :c4] = o * OSC + (q_s[pl.ds(r0, M), :c4].astype(f32) + b2[:, :c4])
            z = jnp.where(false_mask()[0:1, :], link[0:1, :], b2[:, c4:] * (1.0 / OSC))
            o = z + jnp.dot(h, w2_s[:, c4:], preferred_element_type=f32)
            p_s[pl.ds(r0, M), c4:] = o * OSC + q_s[pl.ds(r0, M), c4:].astype(f32)
            conv_inv(i, Y)

        rev8 = 7 - row8

        def load_y(j, t):
            y = yp_s[j, t:t + 8, :]
            if t % P < 64:
                y = jnp.take_along_axis(y, rev8, axis=0)
            return y

        def combine(r0, r1, st):
            fm = false_mask()
            for t in range(r0, r1, 16):
                for j in range(NL):
                    cs = slice(j * 128, (j + 1) * 128)
                    y = jnp.concatenate([load_y(j, t), load_y(j, t + 8)], axis=0)
                    p0 = p_s[t:t + 8, cs]
                    if st[0] is not None:
                        p0 = jnp.where(fm, st[0], p0)
                    pp = jnp.concatenate([p0, p_s[t + 8:t + 16, cs]], axis=0)
                    r = (pp + xn_s[j, t:t + 16, :].astype(f32) * y).astype(bf16)
                    st[0] = r.astype(f32)[0:8, :]
                    o_s[j, t:t + 16, :] = r

        def first():
            wait(0)
            ln(0, qa, 0)
            wait(1)

            def r0a():
                bc_s[...] = jnp.broadcast_to(b1_row()[:, F - 128:F], (128, 128)).T[64:128, :]
                hid_s[0:qa, 0:w1c[1]] = mm1(load_xn(0, qa), 0, w1c[1]).astype(bf16)
            region(r0a)
            wait(2)

            def r0b():
                ln(qa, M0, lnb)
                cs = [qa] + [qa + x for x in bsp] + [M0]
                for a_, b_ in zip(cs[:-1], cs[1:]):
                    hid_s[a_:b_, 0:w1c[1]] = mm1(load_xn(a_, b_ - a_), 0, w1c[1]).astype(bf16)
            region(r0b)
            for i in range(1, n1):
                wait(2 + i)

                def r1(i=i):
                    hid_s[:, w1c[i]:w1c[i + 1]] = mm1(load_xn(0, M0), w1c[i], w1c[i + 1]).astype(bf16)
                region(r1)
            wait(ng - 4)

            def r2a():
                ln(M0, M0 + lns, ln0)
                p_s[0:M0, :] = jnp.dot(hid_s[:, :w2k], w2_s[:w2k, :], preferred_element_type=f32)
            region(r2a)
            wait(ng - 3)

            def r2b():
                lk = ln(M0 + lns, S, ln0)
                t = lk[0]
                for u in lk[1:]:
                    t = t + u
                lk = jnp.broadcast_to(t[0:8, :], (8, 128)) if lnk else None
                o = jnp.dot(hid_s[:, w2k:], w2_s[w2k:, :], preferred_element_type=f32) + p_s[0:M0, :]
                p_s[0:M0, :] = o * OSC + (q_s[0:M0, :].astype(f32) + b2_row())
                par = jnp.concatenate([sk_ref[...].astype(f32), dd_ref[...].astype(f32).reshape(1, D),
                                       jnp.zeros((3, D), f32)], axis=0)
                for j in range(NL):
                    par_s[j] = par[:, j * 128:(j + 1) * 128]
                kv_fwd(0, par[:, 0:128], lk, lag0)
            region(r2b)

        def pair(i, carry):
            si = lax.rem(ng - 2 + i, ring)
            for c in copies(kvh(2 * i + 1) + kvh(2 * i + 2), si):
                c.wait()
            mlp_conv(2 * i, False)
            kv_fwd(2 * i + 1, par_s[2 * i + 1])
            z = NB + flag_s[1]
            x_s[z, 0:8, :] = jnp.zeros((8, 128), f32)
            hf_s[z, 0:8, :] = jnp.zeros((8, 128), f32)
            mlp_conv(2 * i + 1, True)
            kv_fwd(2 * i + 2, par_s[2 * i + 2])
            return carry

        rl = S - ML

        def out_copies(js, r0, r1):
            return copies([(o_s.at[j, pl.ds(r0, r1 - r0), :], out_hbm.at[pl.ds(r0, r1 - r0), pl.ds(j * 128, 128)])
                           for j in js], sem_out)
        cuts = [0] + [int(rl // 16 * x) * 16 for x in prow] + [rl]
        g_o = [out_copies(range(NL), cuts[i], cuts[i + 1]) for i in range(nco)]
        g_fa = out_copies(range(osp), rl, S)
        g_fb = out_copies(range(osp, NL), rl, S)

        def pin_after(g, i):
            for c in g:
                c.start()
            z1 = pl.multiple_of(S + flag_s[1], 16)
            z2 = pl.multiple_of(S + flag_s[2], 16)
            o_s[0, pl.ds(z1, 16), :] = jnp.full((16, 128), i, bf16)
            return o_s[0, pl.ds(z2, 16), :].astype(f32)

        def last():
            mlp_conv(NL - 1, False)
            yp_s[NL + flag_s[1], 0:8, :] = jnp.zeros((8, 128), f32)
            p_s[pl.ds(pl.multiple_of(S + flag_s[1], 8), 8), 0:128] = jnp.zeros((8, 128), f32)
            xn = load_xn(rl, ML)
            st = [None]
            hs = []
            gi = 0
            for f in range(13):
                pin = None
                if gi < nco and pins[gi] == f:
                    combine(cuts[gi], cuts[gi + 1], st)
                    pin = pin_after(g_o[gi], gi)
                    gi += 1
                hs.append(mm1(xn, 128 * f, 128 * (f + 1), pin))
            hs.append(mm1_rem(xn))
            h = jnp.concatenate(hs, axis=1).astype(bf16)
            b2 = b2_row() * (1.0 / OSC)
            for j in range(NL):
                cs = slice(j * 128, (j + 1) * 128)
                bj = b2[:, cs]
                if gi < nco and pins[gi] == 14 + j:
                    combine(cuts[gi], cuts[gi + 1], st)
                    bj = jnp.where(false_mask()[0:1, :], pin_after(g_o[gi], gi)[0:1, :], bj)
                    gi += 1
                if j == osp:
                    bj = jnp.where(false_mask()[0:1, :], pin_after(g_fa, nco)[0:1, :], bj)
                o = (bj + jnp.dot(h, w2_s[:, cs], preferred_element_type=f32)) * OSC + q_s[rl:S, cs].astype(f32)
                y = jnp.concatenate([load_y(j, t) for t in range(rl, S, 8)], axis=0)
                o_s[j, rl:S, :] = (o + xn_s[j, rl:S, :].astype(f32) * y).astype(bf16)
            assert gi == nco
        def it(i, carry):
            pl.when(i == 0)(first)
            pair(i, carry)
            pl.when(i == 1)(last)
            return carry
        lax.fori_loop(0, 2, it, 0)
        for c in g_fb:
            c.start()
        for g in g_o + [g_fa, g_fb]:
            for c in g:
                c.wait()

    fw, inv = dft_mats()

    @jax.jit
    def f(q, k, v, sk, h, dd, w1, b1, w2, b2):
        any_ = pl.BlockSpec(memory_space=pl.ANY)
        out = pl.pallas_call(
            kernel,
            in_specs=[any_] * 12,
            out_specs=any_,
            out_shape=jax.ShapeDtypeStruct((S, D), bf16),
            scratch_shapes=[
                pltpu.VMEM((S, D), bf16),
                pltpu.VMEM((NL, S + KP, 128), bf16),
                pltpu.VMEM((NL, S, 128), bf16),
                pltpu.VMEM((NL, 128, S), bf16),
                pltpu.VMEM((F, D), bf16),
                pltpu.VMEM((F, D), bf16),
                pltpu.VMEM((NL, S, 128), bf16),
                pltpu.VMEM((S + 8, D), f32),
                pltpu.VMEM((NB + 1, 256, 128), f32),
                pltpu.VMEM((NB + 1, 256, 128), f32),
                pltpu.VMEM((NL + 1, S, 128), f32),
                pltpu.VMEM((NL, S + 16, 128), bf16),
                pltpu.VMEM((NL, 8, 128), f32),
                pltpu.VMEM((M0, F), bf16),
                pltpu.VMEM((4, D), bf16), pltpu.VMEM((D,), bf16), pltpu.VMEM((F,), bf16), pltpu.VMEM((D,), bf16),
                pltpu.VMEM((2, 256, 128), bf16), pltpu.VMEM((2, 64, 128), bf16),
                pltpu.VMEM((64, 128), f32),
                pltpu.SMEM((4,), jnp.int32),
                pltpu.SemaphoreType.DMA((ring if ring < 9 else 10,)),
            ],
            compiler_params=pltpu.CompilerParams(vmem_limit_bytes=100 * 2**20),
            name=name,
        )(q.reshape(S, D), k.reshape(S, D), v.reshape(S, D), sk.T, h, dd, w1.T, b1, w2, b2, fw, inv)
        return out.reshape(1, S, D)
    return f


_impl = make(name="fused_h3_mlp")


@jax.jit
def pallas_parallel_sum__ssm_conv_h3__dense_activation_gelu__prompt_kernel(
    A_q, A_k, A_v, A_shift_k, A_ssm_k, A_ssm_D, B_x, B_w1, B_b1, B_w2, B_b2,
):
    del B_x
    return _impl(A_q, A_k, A_v, A_shift_k, A_ssm_k, A_ssm_D, B_w1, B_b1, B_w2, B_b2)
```

```python
import numpy as np
import jax
import jax.numpy as jnp
from jax import lax
import jax.experimental.pallas as pl
import jax.experimental.pallas.tpu as pltpu

S, D, F = 2048, 640, 1728
P = 128
NB = S // P
NL = D // 128
KP = 64
FR = F - 64
f32, bf16, u32 = jnp.float32, jnp.bfloat16, jnp.uint32
NT = (((1,), (1,)), ((), ()))

ALPHA = (0.7978845608028654 * 0.044715) ** (1.0 / 3.0)
C1 = 0.7978845608028654 / ALPHA
OSC = 0.5 / ALPHA


def dft_mats():
    ks = np.concatenate([np.arange(0, 128, 2), np.arange(1, 128, 2)])
    n = np.arange(128)
    m = np.arange(64) + 0.5
    fw = np.zeros((2, 256, 128))
    inv = np.zeros((2, 64, 128))
    for p in range(16):
        for s in range(8):
            w = 2 * np.pi * (ks[8 * p + s] + 0.5) / 256
            fw[0, 16 * p + s] = np.cos(w * (n - 63.5))
            fw[0, 16 * p + 8 + s] = -np.sin(w * (n - 63.5))
            fw[1, 16 * p + s] = np.cos(w * n)
            fw[1, 16 * p + 8 + s] = -np.sin(w * n)
            inv[0, :, 8 * p + s] = np.cos(w * m) / (128 * ALPHA)
            inv[1, :, 8 * p + s] = np.sin(w * m) / (128 * ALPHA)
    perm = np.concatenate(
        [16 * t + np.concatenate([np.arange(0, 16, 2), np.arange(1, 16, 2)]) for t in range(8)])
    fw[0] = fw[0][:, perm]
    return fw.astype(np.float32).astype(bf16), inv.astype(np.float32).astype(bf16)


def gelu(g):
    return g * (1.0 + jnp.tanh(g * (C1 + g * g)))


def make(M0=576, M=256, name="v37", kvn=2, qa=256, w1c=(0, 256, 768, F), w2k=1024, lns=960, ln0=2,
         pins=(2, 7, 12, 15), prow=(0.01, 0.28, 0.6), osp=3, lag=4, mg=3, ring=4, rpos=4):
    ML = S - M0 - NL * M
    assert ML > 0 and ML % 16 == 0 and M0 % 64 == 0 and M % 64 == 0
    n1, nco = len(w1c) - 1, len(pins)

    def kernel(q_hbm, k_hbm, v_hbm, sk_hbm, h_hbm, dd_hbm, w1_hbm, b1_hbm, w2_hbm, b2_hbm, fw_hbm, inv_hbm,
               out_hbm,
               q_s, k_s, v_s, h_s, w1_s, w2_s, xn_s, p_s, x_s, hf_s, yp_s, o_s, par_s, hid_s,
               sk_ref, dd_ref, b1_ref, b2_ref, fw_ref, inv_ref, bc_s, flag_s, sem):
        def rows(src, dst, r0, r1):
            return (src.at[pl.ds(r0, r1 - r0)], dst.at[pl.ds(r0, r1 - r0)])

        def kvh(j):
            lane = pl.ds(j * 128, 128) if isinstance(j, int) else pl.ds(pl.multiple_of(j * 128, 128), 128)
            return [(h_hbm.at[lane, :], h_s.at[j]),
                    (k_hbm.at[:, lane], k_s.at[j, pl.ds(KP, S), :]),
                    (v_hbm.at[:, lane], v_s.at[j])]

        def copies(g, si):
            return [pltpu.make_async_copy(src, dst, sem.at[si]) for src, dst in g]

        groups = [[rows(q_hbm, q_s, 0, qa)],
                  [rows(w1_hbm, w1_s, 0, w1c[1]), (b1_hbm, b1_ref)],
                  [rows(q_hbm, q_s, qa, M0)]]
        groups += [[rows(w1_hbm, w1_s, w1c[i], w1c[i + 1])] for i in range(1, n1)]
        groups += [[rows(q_hbm, q_s, M0, M0 + lns), rows(w2_hbm, w2_s, 0, w2k)],
                   [rows(q_hbm, q_s, M0 + lns, S), rows(w2_hbm, w2_s, w2k, F), (b2_hbm, b2_ref), (sk_hbm, sk_ref), (dd_hbm, dd_ref),
                    (fw_hbm, fw_ref), (inv_hbm, inv_ref)] + kvh(0),
                   kvh(1) + kvh(2), kvh(3) + kvh(4)]
        ng = len(groups)
        sem_out = (ng - 3) % ring

        def start(g):
            if g < ng:
                for c in copies(groups[g], g % ring):
                    c.start()

        def wait(g):
            for c in copies(groups[g], g % ring):
                c.wait()
            start(g + ring)

        for g in range(ring):
            start(g)

        flag_s[0] = 100
        flag_s[1] = 0
        flag_s[2] = 0
        for j in range(NL):
            k_s[j, KP - 16:KP, :] = jnp.zeros((16, 128), bf16)
        ku_s = k_s.bitcast(u32)
        vu_s = v_s.bitcast(u32)

        def region(fn):
            pl.when(flag_s[0] == 100)(fn)

        row8 = lax.broadcasted_iota(jnp.int32, (8, 128), 0)

        def false_mask():
            return row8 > flag_s[0]

        def ln(r0, r1, n):
            fm = lax.broadcasted_iota(jnp.int32, (16, 1), 0) > flag_s[0]
            lasts = [None] * max(n, 1)
            for t, rr in enumerate(range(r0, r1, 16)):
                x = q_s[rr:rr + 16, :].astype(f32)
                sm = jnp.sum(x, axis=-1, keepdims=True)
                ci = t % max(n, 1)
                if n and lasts[ci] is not None:
                    sm = jnp.where(fm, lasts[ci], sm)
                xc = x - sm * (1.0 / D)
                var = jnp.sum(xc * xc, axis=-1, keepdims=True) * (1.0 / D)
                rs = lax.rsqrt(var + 1e-5) * ALPHA
                lasts[ci] = rs
                xo = xc * rs
                for j in range(NL):
                    xn_s[j, rr:rr + 16, :] = xo[:, j * 128:(j + 1) * 128].astype(bf16)
            return lasts

        def load_xn(r0, m):
            return jnp.concatenate([xn_s[j, pl.ds(r0, m), :] for j in range(NL)], axis=1)

        def b1_row():
            return b1_ref[...].astype(f32).reshape(1, F) * ALPHA

        def b2_row():
            return b2_ref[...].astype(f32).reshape(1, D)

        def mm1_rem(xn):
            m = xn.shape[0]
            ht = lax.dot_general(w1_s[FR:F, :], xn, NT, preferred_element_type=f32)
            bc = bc_s[...]
            outs = []
            for c0 in range(0, m, 128):
                c1 = min(c0 + 128, m)
                outs.append(gelu(ht[:, c0:c1] + bc[:, :c1 - c0]).T)
            return jnp.concatenate(outs, axis=0)

        def mm1(xn, f0=0, f1=F, pin=None):
            if f1 == F:
                hr = mm1_rem(xn)
                if f0 == FR:
                    return hr
                return jnp.concatenate([mm1(xn, f0, FR, pin), hr], axis=1)
            b1 = b1_row()[:, f0:f1]
            if pin is not None:
                b1 = jnp.where(false_mask()[0:1, :f1 - f0], pin[0:1, :f1 - f0], b1)
            h = lax.dot_general(xn, w1_s[f0:f1, :], NT, preferred_element_type=f32) + b1
            return gelu(h)

        def kv_fwd(j, sk, init=None):
            s = [jnp.broadcast_to(sk[l:l + 1, :], (8, 128)) for l in range(4)]
            dd = sk[4:5, :]
            fm = false_mask()
            lasts = [init] * kvn
            fwx = fw_ref[0]
            fwh = fw_ref[1]
            ev = lambda w: pltpu.bitcast(w << 16, f32)
            od = lambda w: pltpu.bitcast(w & jnp.uint32(0xffff0000), f32)
            kvs = []
            for a in range(NB + lag):
                if a < NB:
                    outs = []
                    for t in range(a * 8, a * 8 + 8):
                        bb = KP // 2 + 8 * t
                        w0 = ku_s[j, bb:bb + 8, :]
                        w1 = ku_s[j, bb - 1:bb + 7, :]
                        w2 = ku_s[j, bb - 2:bb + 6, :]
                        wv = vu_s[j, 8 * t:8 * t + 8, :]
                        e0, o0, e1, o1, o2 = ev(w0), od(w0), ev(w1), od(w1), od(w2)
                        ci = t % kvn
                        if lasts[ci] is not None:
                            e0 = jnp.where(fm, lasts[ci], e0)
                        oe = (e0 * s[0] + o1 * s[1] + e1 * s[2] + o2 * s[3]) * ev(wv)
                        oo = (e0 * s[1] + o0 * s[0] + o1 * s[2] + e1 * s[3]) * od(wv)
                        lasts[ci] = oo
                        outs += [oe, oo]
                    kvs.append(jnp.concatenate(outs, axis=0).astype(bf16))
                    hb = lax.dot_general(fwh, h_s[j, :, a * P:(a + 1) * P], NT, preferred_element_type=f32)
                    if a == 0:
                        hb = jnp.concatenate(
                            [hb[8 * t:8 * t + 8, :] + dd if t % 2 == 0 else hb[8 * t:8 * t + 8, :]
                             for t in range(32)], axis=0)
                    hf_s[a] = hb
                if a >= lag:
                    x_s[a - lag] = jnp.dot(fwx, kvs[a - lag], preferred_element_type=f32)

        def conv_mac(short):
            fm = false_mask()
            last = None
            Y = [[None] * 16 for _ in range(NB)]
            for p in range(16):
                r0, i0 = 16 * p, 16 * p + 8
                prev = None
                for c in range(NB):
                    accr = acci = pend = None
                    for a in range(c + 1):
                        b = c - a
                        xr = x_s[a, r0:r0 + 8, :]
                        xi = x_s[a, i0:i0 + 8, :]
                        hr = hf_s[b, r0:r0 + 8, :]
                        hi = hf_s[b, i0:i0 + 8, :]
                        if accr is None:
                            t1 = xr * hr
                            t2 = xr * hi
                            if last is not None:
                                t1 = jnp.where(fm, last[0], t1)
                                t2 = jnp.where(fm, last[1], t2)
                            accr = t1 - xi * hi
                            acci = t2 + xi * hr
                        elif short:
                            tr = xr * hr - xi * hi
                            ti = xr * hi + xi * hr
                            if pend is not None:
                                tr = tr + pend[0]
                                ti = ti + pend[1]
                                pend = None
                            elif a % mg == 1 and a < c:
                                pend = (tr, ti)
                                continue
                            accr = accr + tr
                            acci = acci + ti
                        else:
                            accr = (accr + xr * hr) - xi * hi
                            acci = (acci + xr * hi) + xi * hr
                    last = (accr, acci)
                    if prev is None:
                        yr, yi = accr, acci
                    else:
                        pr, pi = prev
                        yr, yi = (accr - pi, acci + pr) if p < 8 else (accr + pi, acci - pr)
                    prev = (accr, acci)
                    Y[c][p] = (yr, yi)
            return Y, last[0] + last[1]

        def conv_inv(j, Y):
            ic = inv_ref[0]
            isn = inv_ref[1]
            for c in range(NB):
                yr = jnp.concatenate([y[0] for y in Y[c]], axis=0).astype(bf16)
                yi = jnp.concatenate([y[1] for y in Y[c]], axis=0).astype(bf16)
                e = jnp.dot(ic, yr, preferred_element_type=f32)
                o = jnp.dot(isn, yi, preferred_element_type=f32)
                yp_s[j, c * P + 64:(c + 1) * P, :] = e - o
                lo = e + o
                for i in range(8):
                    yp_s[j, c * P + 8 * (7 - i):c * P + 8 * (8 - i), :] = lo[8 * i:8 * i + 8, :]

        def mlp_conv(i, short):
            r0 = M0 + i * M if isinstance(i, int) else pl.multiple_of(M0 + i * M, 64)
            Y, link = conv_mac(short)
            xn = load_xn(r0, M)
            if short:
                ha = mm1(xn, 0, 128 * rpos)
                hr = mm1_rem(xn)
                h = jnp.concatenate([ha, mm1(xn, 128 * rpos, FR), hr], axis=1)
            else:
                h = mm1(xn)
            h = h.astype(bf16)
            b2 = b2_row()
            c4 = D - 128
            o = jnp.dot(h, w2_s[:, :c4], preferred_element_type=f32)
            p_s[pl.ds(r0, M), :c4] = o * OSC + (q_s[pl.ds(r0, M), :c4].astype(f32) + b2[:, :c4])
            z = jnp.where(false_mask()[0:1, :], link[0:1, :], b2[:, c4:] * (1.0 / OSC))
            o = z + jnp.dot(h, w2_s[:, c4:], preferred_element_type=f32)
            p_s[pl.ds(r0, M), c4:] = o * OSC + q_s[pl.ds(r0, M), c4:].astype(f32)
            conv_inv(i, Y)

        rev8 = 7 - row8

        def load_y(j, t):
            y = yp_s[j, t:t + 8, :]
            if t % P < 64:
                y = jnp.take_along_axis(y, rev8, axis=0)
            return y

        def combine(r0, r1, st):
            fm = false_mask()
            for t in range(r0, r1, 16):
                for j in range(NL):
                    cs = slice(j * 128, (j + 1) * 128)
                    y = jnp.concatenate([load_y(j, t), load_y(j, t + 8)], axis=0)
                    p0 = p_s[t:t + 8, cs]
                    if st[0] is not None:
                        p0 = jnp.where(fm, st[0], p0)
                    pp = jnp.concatenate([p0, p_s[t + 8:t + 16, cs]], axis=0)
                    r = (pp + xn_s[j, t:t + 16, :].astype(f32) * y).astype(bf16)
                    st[0] = r.astype(f32)[0:8, :]
                    o_s[j, t:t + 16, :] = r

        def first():
            wait(0)
            ln(0, qa, 0)
            wait(1)

            def r0a():
                bc_s[...] = jnp.broadcast_to(b1_row()[:, F - 128:F], (128, 128)).T[64:128, :]
                hid_s[0:qa, 0:w1c[1]] = mm1(load_xn(0, qa), 0, w1c[1]).astype(bf16)
            region(r0a)
            wait(2)

            def r0b():
                ln(qa, M0, 0)
                hid_s[qa:M0, 0:w1c[1]] = mm1(load_xn(qa, M0 - qa), 0, w1c[1]).astype(bf16)
            region(r0b)
            for i in range(1, n1):
                wait(2 + i)

                def r1(i=i):
                    hid_s[:, w1c[i]:w1c[i + 1]] = mm1(load_xn(0, M0), w1c[i], w1c[i + 1]).astype(bf16)
                region(r1)
            wait(ng - 4)

            def r2a():
                ln(M0, M0 + lns, ln0)
                p_s[0:M0, :] = jnp.dot(hid_s[:, :w2k], w2_s[:w2k, :], preferred_element_type=f32)
            region(r2a)
            wait(ng - 3)

            def r2b():
                lk = ln(M0 + lns, S, ln0)
                t = lk[0]
                for u in lk[1:]:
                    t = t + u
                lk = jnp.broadcast_to(t[0:8, :], (8, 128))
                o = jnp.dot(hid_s[:, w2k:], w2_s[w2k:, :], preferred_element_type=f32) + p_s[0:M0, :]
                p_s[0:M0, :] = o * OSC + (q_s[0:M0, :].astype(f32) + b2_row())
                par = jnp.concatenate([sk_ref[...].astype(f32), dd_ref[...].astype(f32).reshape(1, D),
                                       jnp.zeros((3, D), f32)], axis=0)
                for j in range(NL):
                    par_s[j] = par[:, j * 128:(j + 1) * 128]
                kv_fwd(0, par[:, 0:128], lk)
            region(r2b)

        def pair(i, carry):
            si = lax.rem(ng - 2 + i, ring)
            for c in copies(kvh(2 * i + 1) + kvh(2 * i + 2), si):
                c.wait()
            mlp_conv(2 * i, False)
            kv_fwd(2 * i + 1, par_s[2 * i + 1])
            z = NB + flag_s[1]
            x_s[z, 0:8, :] = jnp.zeros((8, 128), f32)
            hf_s[z, 0:8, :] = jnp.zeros((8, 128), f32)
            mlp_conv(2 * i + 1, True)
            kv_fwd(2 * i + 2, par_s[2 * i + 2])
            return carry

        rl = S - ML

        def out_copies(js, r0, r1):
            return copies([(o_s.at[j, pl.ds(r0, r1 - r0), :], out_hbm.at[pl.ds(r0, r1 - r0), pl.ds(j * 128, 128)])
                           for j in js], sem_out)
        cuts = [0] + [int(rl // 16 * x) * 16 for x in prow] + [rl]
        g_o = [out_copies(range(NL), cuts[i], cuts[i + 1]) for i in range(nco)]
        g_fa = out_copies(range(osp), rl, S)
        g_fb = out_copies(range(osp, NL), rl, S)

        def pin_after(g, i):
            for c in g:
                c.start()
            z1 = pl.multiple_of(S + flag_s[1], 16)
            z2 = pl.multiple_of(S + flag_s[2], 16)
            o_s[0, pl.ds(z1, 16), :] = jnp.full((16, 128), i, bf16)
            return o_s[0, pl.ds(z2, 16), :].astype(f32)

        def last():
            mlp_conv(NL - 1, False)
            yp_s[NL + flag_s[1], 0:8, :] = jnp.zeros((8, 128), f32)
            p_s[pl.ds(pl.multiple_of(S + flag_s[1], 8), 8), 0:128] = jnp.zeros((8, 128), f32)
            xn = load_xn(rl, ML)
            st = [None]
            hs = []
            gi = 0
            for f in range(13):
                pin = None
                if gi < nco and pins[gi] == f:
                    combine(cuts[gi], cuts[gi + 1], st)
                    pin = pin_after(g_o[gi], gi)
                    gi += 1
                hs.append(mm1(xn, 128 * f, 128 * (f + 1), pin))
            hs.append(mm1_rem(xn))
            h = jnp.concatenate(hs, axis=1).astype(bf16)
            b2 = b2_row() * (1.0 / OSC)
            for j in range(NL):
                cs = slice(j * 128, (j + 1) * 128)
                bj = b2[:, cs]
                if gi < nco and pins[gi] == 14 + j:
                    combine(cuts[gi], cuts[gi + 1], st)
                    bj = jnp.where(false_mask()[0:1, :], pin_after(g_o[gi], gi)[0:1, :], bj)
                    gi += 1
                if j == osp:
                    bj = jnp.where(false_mask()[0:1, :], pin_after(g_fa, nco)[0:1, :], bj)
                o = (bj + jnp.dot(h, w2_s[:, cs], preferred_element_type=f32)) * OSC + q_s[rl:S, cs].astype(f32)
                y = jnp.concatenate([load_y(j, t) for t in range(rl, S, 8)], axis=0)
                o_s[j, rl:S, :] = (o + xn_s[j, rl:S, :].astype(f32) * y).astype(bf16)
            assert gi == nco
        def it(i, carry):
            pl.when(i == 0)(first)
            pair(i, carry)
            pl.when(i == 1)(last)
            return carry
        lax.fori_loop(0, 2, it, 0)
        for c in g_fb:
            c.start()
        for g in g_o + [g_fa, g_fb]:
            for c in g:
                c.wait()

    fw, inv = dft_mats()

    @jax.jit
    def f(q, k, v, sk, h, dd, w1, b1, w2, b2):
        any_ = pl.BlockSpec(memory_space=pl.ANY)
        out = pl.pallas_call(
            kernel,
            in_specs=[any_] * 12,
            out_specs=any_,
            out_shape=jax.ShapeDtypeStruct((S, D), bf16),
            scratch_shapes=[
                pltpu.VMEM((S, D), bf16),
                pltpu.VMEM((NL, S + KP, 128), bf16),
                pltpu.VMEM((NL, S, 128), bf16),
                pltpu.VMEM((NL, 128, S), bf16),
                pltpu.VMEM((F, D), bf16),
                pltpu.VMEM((F, D), bf16),
                pltpu.VMEM((NL, S, 128), bf16),
                pltpu.VMEM((S + 8, D), f32),
                pltpu.VMEM((NB + 1, 256, 128), f32),
                pltpu.VMEM((NB + 1, 256, 128), f32),
                pltpu.VMEM((NL + 1, S, 128), f32),
                pltpu.VMEM((NL, S + 16, 128), bf16),
                pltpu.VMEM((NL, 8, 128), f32),
                pltpu.VMEM((M0, F), bf16),
                pltpu.VMEM((4, D), bf16), pltpu.VMEM((D,), bf16), pltpu.VMEM((F,), bf16), pltpu.VMEM((D,), bf16),
                pltpu.VMEM((2, 256, 128), bf16), pltpu.VMEM((2, 64, 128), bf16),
                pltpu.VMEM((64, 128), f32),
                pltpu.SMEM((4,), jnp.int32),
                pltpu.SemaphoreType.DMA((ring,)),
            ],
            compiler_params=pltpu.CompilerParams(vmem_limit_bytes=100 * 2**20),
            name=name,
        )(q.reshape(S, D), k.reshape(S, D), v.reshape(S, D), sk.T, h, dd, w1.T, b1, w2, b2, fw, inv)
        return out.reshape(1, S, D)
    return f


_impl = make(name="fused_h3_mlp")


@jax.jit
def pallas_parallel_sum__ssm_conv_h3__dense_activation_gelu__prompt_kernel(
    A_q, A_k, A_v, A_shift_k, A_ssm_k, A_ssm_D, B_x, B_w1, B_b1, B_w2, B_b2,
):
    del B_x
    return _impl(A_q, A_k, A_v, A_shift_k, A_ssm_k, A_ssm_D, B_w1, B_b1, B_w2, B_b2)
```

```python
import numpy as np
import jax
import jax.numpy as jnp
from jax import lax
import jax.experimental.pallas as pl
import jax.experimental.pallas.tpu as pltpu

S, D, F = 2048, 640, 1728
P = 128
NB = S // P
NL = D // 128
KP = 64
FR = F - 64
f32, bf16, u32 = jnp.float32, jnp.bfloat16, jnp.uint32
NT = (((1,), (1,)), ((), ()))

ALPHA = (0.7978845608028654 * 0.044715) ** (1.0 / 3.0)
C1 = 0.7978845608028654 / ALPHA
OSC = 0.5 / ALPHA


def dft_mats():
    ks = np.concatenate([np.arange(0, 128, 2), np.arange(1, 128, 2)])
    n = np.arange(128)
    m = np.arange(64) + 0.5
    fw = np.zeros((2, 256, 128))
    inv = np.zeros((2, 64, 128))
    for p in range(16):
        for s in range(8):
            w = 2 * np.pi * (ks[8 * p + s] + 0.5) / 256
            fw[0, 16 * p + s] = np.cos(w * (n - 63.5))
            fw[0, 16 * p + 8 + s] = -np.sin(w * (n - 63.5))
            fw[1, 16 * p + s] = np.cos(w * n)
            fw[1, 16 * p + 8 + s] = -np.sin(w * n)
            inv[0, :, 8 * p + s] = np.cos(w * m) / (128 * ALPHA)
            inv[1, :, 8 * p + s] = np.sin(w * m) / (128 * ALPHA)
    perm = np.concatenate(
        [16 * t + np.concatenate([np.arange(0, 16, 2), np.arange(1, 16, 2)]) for t in range(8)])
    fw[0] = fw[0][:, perm]
    return fw.astype(np.float32).astype(bf16), inv.astype(np.float32).astype(bf16)


def gelu(g):
    return g * (1.0 + jnp.tanh(g * (C1 + g * g)))


def make(M0=576, M=256, name="v40", kvn=2, qa=256, w1c=(0, 256, 768, F), w2k=1024, lns=960, ln0=2,
         pins=(2, 7, 12, 15), prow=(0.01, 0.28, 0.6), osp=3, lag=4, mg=3, ring=4, rpos=4):
    ML = S - M0 - NL * M
    assert ML > 0 and ML % 16 == 0 and M0 % 64 == 0 and M % 64 == 0
    n1, nco = len(w1c) - 1, len(pins)

    def kernel(q_hbm, k_hbm, v_hbm, sk_hbm, h_hbm, dd_hbm, w1_hbm, b1_hbm, w2_hbm, b2_hbm, fw_hbm, inv_hbm,
               out_hbm,
               q_s, k_s, v_s, h_s, w1_s, w2_s, xn_s, p_s, x_s, hf_s, yp_s, o_s, par_s, hid_s,
               sk_ref, dd_ref, b1_ref, b2_ref, fw_ref, inv_ref, bc_s, w1n_s, flag_s, sem):
        def rows(src, dst, r0, r1):
            return (src.at[pl.ds(r0, r1 - r0)], dst.at[pl.ds(r0, r1 - r0)])

        def kvh(j):
            lane = pl.ds(j * 128, 128) if isinstance(j, int) else pl.ds(pl.multiple_of(j * 128, 128), 128)
            return [(h_hbm.at[lane, :], h_s.at[j]),
                    (k_hbm.at[:, lane], k_s.at[j, pl.ds(KP, S), :]),
                    (v_hbm.at[:, lane], v_s.at[j])]

        def copies(g, si):
            return [pltpu.make_async_copy(src, dst, sem.at[si]) for src, dst in g]

        groups = [[rows(q_hbm, q_s, 0, qa)],
                  [rows(w1_hbm, w1_s, 0, w1c[1]), (b1_hbm, b1_ref)],
                  [rows(q_hbm, q_s, qa, M0)]]
        groups += [[rows(w1_hbm, w1_s, w1c[i], w1c[i + 1])] for i in range(1, n1)]
        groups += [[rows(q_hbm, q_s, M0, M0 + lns), rows(w2_hbm, w2_s, 0, w2k)],
                   [rows(q_hbm, q_s, M0 + lns, S), rows(w2_hbm, w2_s, w2k, F), (b2_hbm, b2_ref), (sk_hbm, sk_ref), (dd_hbm, dd_ref),
                    (fw_hbm, fw_ref), (inv_hbm, inv_ref)] + kvh(0),
                   kvh(1) + kvh(2), kvh(3) + kvh(4)]
        ng = len(groups)
        sem_out = (ng - 3) % ring

        def start(g):
            if g < ng:
                for c in copies(groups[g], g % ring):
                    c.start()

        def wait(g):
            for c in copies(groups[g], g % ring):
                c.wait()
            start(g + ring)

        for g in range(ring):
            start(g)

        flag_s[0] = 100
        flag_s[1] = 0
        flag_s[2] = 0
        for j in range(NL):
            k_s[j, KP - 16:KP, :] = jnp.zeros((16, 128), bf16)
        ku_s = k_s.bitcast(u32)
        vu_s = v_s.bitcast(u32)

        def region(fn):
            pl.when(flag_s[0] == 100)(fn)

        row8 = lax.broadcasted_iota(jnp.int32, (8, 128), 0)

        def false_mask():
            return row8 > flag_s[0]

        def ln(r0, r1, n):
            fm = lax.broadcasted_iota(jnp.int32, (16, 1), 0) > flag_s[0]
            lasts = [None] * max(n, 1)
            for t, rr in enumerate(range(r0, r1, 16)):
                x = q_s[rr:rr + 16, :].astype(f32)
                sm = jnp.sum(x, axis=-1, keepdims=True)
                ci = t % max(n, 1)
                if n and lasts[ci] is not None:
                    sm = jnp.where(fm, lasts[ci], sm)
                xc = x - sm * (1.0 / D)
                var = jnp.sum(xc * xc, axis=-1, keepdims=True) * (1.0 / D)
                rs = lax.rsqrt(var + 1e-5) * ALPHA
                lasts[ci] = rs
                xo = xc * rs
                for j in range(NL):
                    xn_s[j, rr:rr + 16, :] = xo[:, j * 128:(j + 1) * 128].astype(bf16)
            return lasts

        def load_xn(r0, m):
            return jnp.concatenate([xn_s[j, pl.ds(r0, m), :] for j in range(NL)], axis=1)

        def b1_row():
            return b1_ref[...].astype(f32).reshape(1, F) * ALPHA

        def b2_row():
            return b2_ref[...].astype(f32).reshape(1, D)

        def mm1_rem(xn):
            m = xn.shape[0]
            ht = lax.dot_general(w1_s[FR:F, :], xn, NT, preferred_element_type=f32)
            bc = bc_s[...]
            outs = []
            for c0 in range(0, m, 128):
                c1 = min(c0 + 128, m)
                outs.append(gelu(ht[:, c0:c1] + bc[:, :c1 - c0]).T)
            return jnp.concatenate(outs, axis=0)

        def mm1(xn, f0=0, f1=F, pin=None):
            if f1 == F:
                hr = mm1_rem(xn)
                if f0 == FR:
                    return hr
                return jnp.concatenate([mm1(xn, f0, FR, pin), hr], axis=1)
            b1 = b1_row()[:, f0:f1]
            if pin is not None:
                b1 = jnp.where(false_mask()[0:1, :f1 - f0], pin[0:1, :f1 - f0], b1)
            h = lax.dot_general(xn, w1_s[f0:f1, :], NT, preferred_element_type=f32) + b1
            return gelu(h)

        def mm1_first(xn):
            return gelu(jnp.dot(xn, w1n_s[...], preferred_element_type=f32) + b1_row()[:, 0:128])

        def kv_fwd(j, sk, init=None):
            s = [jnp.broadcast_to(sk[l:l + 1, :], (8, 128)) for l in range(4)]
            dd = sk[4:5, :]
            fm = false_mask()
            lasts = [init] * kvn
            fwx = fw_ref[0]
            fwh = fw_ref[1]
            ev = lambda w: pltpu.bitcast(w << 16, f32)
            od = lambda w: pltpu.bitcast(w & jnp.uint32(0xffff0000), f32)
            kvs = []
            for a in range(NB + lag):
                if a < NB:
                    outs = []
                    for t in range(a * 8, a * 8 + 8):
                        bb = KP // 2 + 8 * t
                        w0 = ku_s[j, bb:bb + 8, :]
                        w1 = ku_s[j, bb - 1:bb + 7, :]
                        w2 = ku_s[j, bb - 2:bb + 6, :]
                        wv = vu_s[j, 8 * t:8 * t + 8, :]
                        e0, o0, e1, o1, o2 = ev(w0), od(w0), ev(w1), od(w1), od(w2)
                        ci = t % kvn
                        if lasts[ci] is not None:
                            e0 = jnp.where(fm, lasts[ci], e0)
                        oe = (e0 * s[0] + o1 * s[1] + e1 * s[2] + o2 * s[3]) * ev(wv)
                        oo = (e0 * s[1] + o0 * s[0] + o1 * s[2] + e1 * s[3]) * od(wv)
                        lasts[ci] = oo
                        outs += [oe, oo]
                    kvs.append(jnp.concatenate(outs, axis=0).astype(bf16))
                    hb = lax.dot_general(fwh, h_s[j, :, a * P:(a + 1) * P], NT, preferred_element_type=f32)
                    if a == 0:
                        hb = jnp.concatenate(
                            [hb[8 * t:8 * t + 8, :] + dd if t % 2 == 0 else hb[8 * t:8 * t + 8, :]
                             for t in range(32)], axis=0)
                    hf_s[a] = hb
                if a >= lag:
                    x_s[a - lag] = jnp.dot(fwx, kvs[a - lag], preferred_element_type=f32)

        def conv_mac(short):
            fm = false_mask()
            last = None
            Y = [[None] * 16 for _ in range(NB)]
            for p in range(16):
                r0, i0 = 16 * p, 16 * p + 8
                prev = None
                for c in range(NB):
                    accr = acci = pend = None
                    for a in range(c + 1):
                        b = c - a
                        xr = x_s[a, r0:r0 + 8, :]
                        xi = x_s[a, i0:i0 + 8, :]
                        hr = hf_s[b, r0:r0 + 8, :]
                        hi = hf_s[b, i0:i0 + 8, :]
                        if accr is None:
                            t1 = xr * hr
                            t2 = xr * hi
                            if last is not None:
                                t1 = jnp.where(fm, last[0], t1)
                                t2 = jnp.where(fm, last[1], t2)
                            accr = t1 - xi * hi
                            acci = t2 + xi * hr
                        elif short:
                            tr = xr * hr - xi * hi
                            ti = xr * hi + xi * hr
                            if pend is not None:
                                tr = tr + pend[0]
                                ti = ti + pend[1]
                                pend = None
                            elif a % mg == 1 and a < c:
                                pend = (tr, ti)
                                continue
                            accr = accr + tr
                            acci = acci + ti
                        else:
                            accr = (accr + xr * hr) - xi * hi
                            acci = (acci + xr * hi) + xi * hr
                    last = (accr, acci)
                    if prev is None:
                        yr, yi = accr, acci
                    else:
                        pr, pi = prev
                        yr, yi = (accr - pi, acci + pr) if p < 8 else (accr + pi, acci - pr)
                    prev = (accr, acci)
                    Y[c][p] = (yr, yi)
            return Y, last[0] + last[1]

        def conv_inv(j, Y):
            ic = inv_ref[0]
            isn = inv_ref[1]
            for c in range(NB):
                yr = jnp.concatenate([y[0] for y in Y[c]], axis=0).astype(bf16)
                yi = jnp.concatenate([y[1] for y in Y[c]], axis=0).astype(bf16)
                e = jnp.dot(ic, yr, preferred_element_type=f32)
                o = jnp.dot(isn, yi, preferred_element_type=f32)
                yp_s[j, c * P + 64:(c + 1) * P, :] = e - o
                lo = e + o
                for i in range(8):
                    yp_s[j, c * P + 8 * (7 - i):c * P + 8 * (8 - i), :] = lo[8 * i:8 * i + 8, :]

        def mlp_conv(i, short):
            r0 = M0 + i * M if isinstance(i, int) else pl.multiple_of(M0 + i * M, 64)
            Y, link = conv_mac(short)
            xn = load_xn(r0, M)
            h0 = mm1_first(xn)
            if short:
                ha = mm1(xn, 128, 128 * rpos)
                hr = mm1_rem(xn)
                h = jnp.concatenate([h0, ha, mm1(xn, 128 * rpos, FR), hr], axis=1)
            else:
                hr = mm1_rem(xn)
                h = jnp.concatenate([h0, mm1(xn, 128, FR), hr], axis=1)
            h = h.astype(bf16)
            b2 = b2_row()
            c4 = D - 128
            o = jnp.dot(h, w2_s[:, :c4], preferred_element_type=f32)
            p_s[pl.ds(r0, M), :c4] = o * OSC + (q_s[pl.ds(r0, M), :c4].astype(f32) + b2[:, :c4])
            z = jnp.where(false_mask()[0:1, :], link[0:1, :], b2[:, c4:] * (1.0 / OSC))
            o = z + jnp.dot(h, w2_s[:, c4:], preferred_element_type=f32)
            p_s[pl.ds(r0, M), c4:] = o * OSC + q_s[pl.ds(r0, M), c4:].astype(f32)
            conv_inv(i, Y)

        rev8 = 7 - row8

        def load_y(j, t):
            y = yp_s[j, t:t + 8, :]
            if t % P < 64:
                y = jnp.take_along_axis(y, rev8, axis=0)
            return y

        def combine(r0, r1, st):
            fm = false_mask()
            for t in range(r0, r1, 16):
                for j in range(NL):
                    cs = slice(j * 128, (j + 1) * 128)
                    y = jnp.concatenate([load_y(j, t), load_y(j, t + 8)], axis=0)
                    p0 = p_s[t:t + 8, cs]
                    if st[0] is not None:
                        p0 = jnp.where(fm, st[0], p0)
                    pp = jnp.concatenate([p0, p_s[t + 8:t + 16, cs]], axis=0)
                    r = (pp + xn_s[j, t:t + 16, :].astype(f32) * y).astype(bf16)
                    st[0] = r.astype(f32)[0:8, :]
                    o_s[j, t:t + 16, :] = r

        def first():
            wait(0)
            ln(0, qa, 0)
            wait(1)

            def r0a():
                bc_s[...] = jnp.broadcast_to(b1_row()[:, F - 128:F], (128, 128)).T[64:128, :]
                hid_s[0:qa, 0:w1c[1]] = mm1(load_xn(0, qa), 0, w1c[1]).astype(bf16)
            region(r0a)
            wait(2)

            def r0b():
                ln(qa, M0, 0)
                hid_s[qa:M0, 0:w1c[1]] = mm1(load_xn(qa, M0 - qa), 0, w1c[1]).astype(bf16)
            region(r0b)
            for i in range(1, n1):
                wait(2 + i)

                def r1(i=i):
                    if i == 1:
                        for j in range(NL):
                            w1n_s[j * 128:(j + 1) * 128, :] = (
                                w1_s[0:128, j * 128:(j + 1) * 128].astype(f32).T.astype(bf16))
                    hid_s[:, w1c[i]:w1c[i + 1]] = mm1(load_xn(0, M0), w1c[i], w1c[i + 1]).astype(bf16)
                region(r1)
            wait(ng - 4)

            def r2a():
                ln(M0, M0 + lns, ln0)
                p_s[0:M0, :] = jnp.dot(hid_s[:, :w2k], w2_s[:w2k, :], preferred_element_type=f32)
            region(r2a)
            wait(ng - 3)

            def r2b():
                lk = ln(M0 + lns, S, ln0)
                t = lk[0]
                for u in lk[1:]:
                    t = t + u
                lk = jnp.broadcast_to(t[0:8, :], (8, 128))
                o = jnp.dot(hid_s[:, w2k:], w2_s[w2k:, :], preferred_element_type=f32) + p_s[0:M0, :]
                p_s[0:M0, :] = o * OSC + (q_s[0:M0, :].astype(f32) + b2_row())
                par = jnp.concatenate([sk_ref[...].astype(f32), dd_ref[...].astype(f32).reshape(1, D),
                                       jnp.zeros((3, D), f32)], axis=0)
                for j in range(NL):
                    par_s[j] = par[:, j * 128:(j + 1) * 128]
                kv_fwd(0, par[:, 0:128], lk)
            region(r2b)

        def pair(i, carry):
            si = lax.rem(ng - 2 + i, ring)
            for c in copies(kvh(2 * i + 1) + kvh(2 * i + 2), si):
                c.wait()
            mlp_conv(2 * i, False)
            kv_fwd(2 * i + 1, par_s[2 * i + 1])
            z = NB + flag_s[1]
            x_s[z, 0:8, :] = jnp.zeros((8, 128), f32)
            hf_s[z, 0:8, :] = jnp.zeros((8, 128), f32)
            mlp_conv(2 * i + 1, True)
            kv_fwd(2 * i + 2, par_s[2 * i + 2])
            return carry

        rl = S - ML

        def out_copies(js, r0, r1):
            return copies([(o_s.at[j, pl.ds(r0, r1 - r0), :], out_hbm.at[pl.ds(r0, r1 - r0), pl.ds(j * 128, 128)])
                           for j in js], sem_out)
        cuts = [0] + [int(rl // 16 * x) * 16 for x in prow] + [rl]
        g_o = [out_copies(range(NL), cuts[i], cuts[i + 1]) for i in range(nco)]
        g_fa = out_copies(range(osp), rl, S)
        g_fb = out_copies(range(osp, NL), rl, S)

        def pin_after(g, i):
            for c in g:
                c.start()
            z1 = pl.multiple_of(S + flag_s[1], 16)
            z2 = pl.multiple_of(S + flag_s[2], 16)
            o_s[0, pl.ds(z1, 16), :] = jnp.full((16, 128), i, bf16)
            return o_s[0, pl.ds(z2, 16), :].astype(f32)

        def last():
            mlp_conv(NL - 1, False)
            yp_s[NL + flag_s[1], 0:8, :] = jnp.zeros((8, 128), f32)
            p_s[pl.ds(pl.multiple_of(S + flag_s[1], 8), 8), 0:128] = jnp.zeros((8, 128), f32)
            xn = load_xn(rl, ML)
            st = [None]
            hs = []
            gi = 0
            for f in range(13):
                pin = None
                if gi < nco and pins[gi] == f:
                    combine(cuts[gi], cuts[gi + 1], st)
                    pin = pin_after(g_o[gi], gi)
                    gi += 1
                hs.append(mm1(xn, 128 * f, 128 * (f + 1), pin) if f else mm1_first(xn))
            hs.append(mm1_rem(xn))
            h = jnp.concatenate(hs, axis=1).astype(bf16)
            b2 = b2_row() * (1.0 / OSC)
            for j in range(NL):
                cs = slice(j * 128, (j + 1) * 128)
                bj = b2[:, cs]
                if gi < nco and pins[gi] == 14 + j:
                    combine(cuts[gi], cuts[gi + 1], st)
                    bj = jnp.where(false_mask()[0:1, :], pin_after(g_o[gi], gi)[0:1, :], bj)
                    gi += 1
                if j == osp:
                    bj = jnp.where(false_mask()[0:1, :], pin_after(g_fa, nco)[0:1, :], bj)
                o = (bj + jnp.dot(h, w2_s[:, cs], preferred_element_type=f32)) * OSC + q_s[rl:S, cs].astype(f32)
                y = jnp.concatenate([load_y(j, t) for t in range(rl, S, 8)], axis=0)
                o_s[j, rl:S, :] = (o + xn_s[j, rl:S, :].astype(f32) * y).astype(bf16)
            assert gi == nco
        def it(i, carry):
            pl.when(i == 0)(first)
            pair(i, carry)
            pl.when(i == 1)(last)
            return carry
        lax.fori_loop(0, 2, it, 0)
        for c in g_fb:
            c.start()
        for g in g_o + [g_fa, g_fb]:
            for c in g:
                c.wait()

    fw, inv = dft_mats()

    @jax.jit
    def f(q, k, v, sk, h, dd, w1, b1, w2, b2):
        any_ = pl.BlockSpec(memory_space=pl.ANY)
        out = pl.pallas_call(
            kernel,
            in_specs=[any_] * 12,
            out_specs=any_,
            out_shape=jax.ShapeDtypeStruct((S, D), bf16),
            scratch_shapes=[
                pltpu.VMEM((S, D), bf16),
                pltpu.VMEM((NL, S + KP, 128), bf16),
                pltpu.VMEM((NL, S, 128), bf16),
                pltpu.VMEM((NL, 128, S), bf16),
                pltpu.VMEM((F, D), bf16),
                pltpu.VMEM((F, D), bf16),
                pltpu.VMEM((NL, S, 128), bf16),
                pltpu.VMEM((S + 8, D), f32),
                pltpu.VMEM((NB + 1, 256, 128), f32),
                pltpu.VMEM((NB + 1, 256, 128), f32),
                pltpu.VMEM((NL + 1, S, 128), f32),
                pltpu.VMEM((NL, S + 16, 128), bf16),
                pltpu.VMEM((NL, 8, 128), f32),
                pltpu.VMEM((M0, F), bf16),
                pltpu.VMEM((4, D), bf16), pltpu.VMEM((D,), bf16), pltpu.VMEM((F,), bf16), pltpu.VMEM((D,), bf16),
                pltpu.VMEM((2, 256, 128), bf16), pltpu.VMEM((2, 64, 128), bf16),
                pltpu.VMEM((64, 128), f32),
                pltpu.VMEM((D, 128), bf16),
                pltpu.SMEM((4,), jnp.int32),
                pltpu.SemaphoreType.DMA((ring,)),
            ],
            compiler_params=pltpu.CompilerParams(vmem_limit_bytes=100 * 2**20),
            name=name,
        )(q.reshape(S, D), k.reshape(S, D), v.reshape(S, D), sk.T, h, dd, w1.T, b1, w2, b2, fw, inv)
        return out.reshape(1, S, D)
    return f


_impl = make(name="fused_h3_mlp")


@jax.jit
def pallas_parallel_sum__ssm_conv_h3__dense_activation_gelu__prompt_kernel(
    A_q, A_k, A_v, A_shift_k, A_ssm_k, A_ssm_D, B_x, B_w1, B_b1, B_w2, B_b2,
):
    del B_x
    return _impl(A_q, A_k, A_v, A_shift_k, A_ssm_k, A_ssm_D, B_w1, B_b1, B_w2, B_b2)
```

```python
import numpy as np
import jax
import jax.numpy as jnp
from jax import lax
import jax.experimental.pallas as pl
import jax.experimental.pallas.tpu as pltpu

S, D, F = 2048, 640, 1728
P = 128
NB = S // P
NL = D // 128
KP = 64
FR = F - 64
f32, bf16, u32 = jnp.float32, jnp.bfloat16, jnp.uint32
NT = (((1,), (1,)), ((), ()))

ALPHA = (0.7978845608028654 * 0.044715) ** (1.0 / 3.0)
C1 = 0.7978845608028654 / ALPHA
OSC = 0.5 / ALPHA


def dft_mats():
    ks = np.concatenate([np.arange(0, 128, 2), np.arange(1, 128, 2)])
    n = np.arange(128)
    m = np.arange(64) + 0.5
    fw = np.zeros((2, 256, 128))
    inv = np.zeros((2, 64, 128))
    for p in range(16):
        for s in range(8):
            w = 2 * np.pi * (ks[8 * p + s] + 0.5) / 256
            fw[0, 16 * p + s] = np.cos(w * (n - 63.5))
            fw[0, 16 * p + 8 + s] = -np.sin(w * (n - 63.5))
            fw[1, 16 * p + s] = np.cos(w * n)
            fw[1, 16 * p + 8 + s] = -np.sin(w * n)
            inv[0, :, 8 * p + s] = np.cos(w * m) / (128 * ALPHA)
            inv[1, :, 8 * p + s] = np.sin(w * m) / (128 * ALPHA)
    perm = np.concatenate(
        [16 * t + np.concatenate([np.arange(0, 16, 2), np.arange(1, 16, 2)]) for t in range(8)])
    fw[0] = fw[0][:, perm]
    return fw.astype(np.float32).astype(bf16), inv.astype(np.float32).astype(bf16)


def gelu(g):
    return g * (1.0 + jnp.tanh(g * (C1 + g * g)))


def make(M0=576, M=256, name="v42", kvn=2, qa=256, w1c=(0, 256, 768, F), w2k=1024, lns=960,
         pins=(2, 7, 12, 15), prow=(0.01, 0.28, 0.6), osp=3, lag=4, mg=3, ring=4, rpos=4):
    ML = S - M0 - NL * M
    assert ML > 0 and ML % 16 == 0 and M0 % 64 == 0 and M % 64 == 0
    n1, nco = len(w1c) - 1, len(pins)

    def kernel(q_hbm, k_hbm, v_hbm, sk_hbm, h_hbm, dd_hbm, w1_hbm, b1_hbm, w2_hbm, b2_hbm, fw_hbm, inv_hbm,
               out_hbm,
               q_s, k_s, v_s, h_s, w1_s, w2_s, xn_s, p_s, x_s, hf_s, yp_s, o_s, par_s, hid_s,
               sk_ref, dd_ref, b1_ref, b2_ref, fw_ref, inv_ref, bc_s, w1n_s, flag_s, sem):
        def rows(src, dst, r0, r1):
            return (src.at[pl.ds(r0, r1 - r0)], dst.at[pl.ds(r0, r1 - r0)])

        def kvh(j):
            lane = pl.ds(j * 128, 128) if isinstance(j, int) else pl.ds(pl.multiple_of(j * 128, 128), 128)
            return [(h_hbm.at[lane, :], h_s.at[j]),
                    (k_hbm.at[:, lane], k_s.at[j, pl.ds(KP, S), :]),
                    (v_hbm.at[:, lane], v_s.at[j])]

        def copies(g, si):
            return [pltpu.make_async_copy(src, dst, sem.at[si]) for src, dst in g]

        groups = [[rows(q_hbm, q_s, 0, qa)],
                  [rows(w1_hbm, w1_s, 0, w1c[1]), (b1_hbm, b1_ref)],
                  [rows(q_hbm, q_s, qa, M0)]]
        groups += [[rows(w1_hbm, w1_s, w1c[i], w1c[i + 1])] for i in range(1, n1)]
        groups += [[rows(q_hbm, q_s, M0, M0 + lns), rows(w2_hbm, w2_s, 0, w2k)],
                   [rows(q_hbm, q_s, M0 + lns, S), rows(w2_hbm, w2_s, w2k, F), (b2_hbm, b2_ref), (sk_hbm, sk_ref), (dd_hbm, dd_ref),
                    (fw_hbm, fw_ref), (inv_hbm, inv_ref)] + kvh(0),
                   kvh(1) + kvh(2), kvh(3) + kvh(4)]
        ng = len(groups)
        sem_out = (ng - 3) % ring

        def start(g):
            if g < ng:
                for c in copies(groups[g], g % ring):
                    c.start()

        def wait(g):
            for c in copies(groups[g], g % ring):
                c.wait()
            start(g + ring)

        for g in range(ring):
            start(g)

        flag_s[0] = 100
        flag_s[1] = 0
        flag_s[2] = 0
        for j in range(NL):
            k_s[j, KP - 16:KP, :] = jnp.zeros((16, 128), bf16)
        ku_s = k_s.bitcast(u32)
        vu_s = v_s.bitcast(u32)

        def region(fn):
            pl.when(flag_s[0] == 100)(fn)

        row8 = lax.broadcasted_iota(jnp.int32, (8, 128), 0)

        def false_mask():
            return row8 > flag_s[0]

        def ln(r0, r1, chain):
            fm = lax.broadcasted_iota(jnp.int32, (16, 1), 0) > flag_s[0]
            rs = None
            for rr in range(r0, r1, 16):
                x = q_s[rr:rr + 16, :].astype(f32)
                xc = x - jnp.sum(x, axis=-1, keepdims=True) * (1.0 / D)
                var = jnp.sum(xc * xc, axis=-1, keepdims=True) * (1.0 / D)
                if chain and rs is not None:
                    var = jnp.where(fm, rs, var)
                rs = lax.rsqrt(var + 1e-5) * ALPHA
                xo = xc * rs
                for j in range(NL):
                    xn_s[j, rr:rr + 16, :] = xo[:, j * 128:(j + 1) * 128].astype(bf16)
            return rs

        def load_xn(r0, m):
            return jnp.concatenate([xn_s[j, pl.ds(r0, m), :] for j in range(NL)], axis=1)

        def b1_row():
            return b1_ref[...].astype(f32).reshape(1, F) * ALPHA

        def b2_row():
            return b2_ref[...].astype(f32).reshape(1, D)

        def mm1_rem(xn):
            m = xn.shape[0]
            ht = lax.dot_general(w1_s[FR:F, :], xn, NT, preferred_element_type=f32)
            bc = bc_s[...]
            outs = []
            for c0 in range(0, m, 128):
                c1 = min(c0 + 128, m)
                outs.append(gelu(ht[:, c0:c1] + bc[:, :c1 - c0]).T)
            return jnp.concatenate(outs, axis=0)

        def mm1(xn, f0=0, f1=F, pin=None):
            if f1 == F:
                hr = mm1_rem(xn)
                if f0 == FR:
                    return hr
                return jnp.concatenate([mm1(xn, f0, FR, pin), hr], axis=1)
            b1 = b1_row()[:, f0:f1]
            if pin is not None:
                b1 = jnp.where(false_mask()[0:1, :f1 - f0], pin[0:1, :f1 - f0], b1)
            h = lax.dot_general(xn, w1_s[f0:f1, :], NT, preferred_element_type=f32) + b1
            return gelu(h)

        def mm1_first(xn):
            return gelu(jnp.dot(xn, w1n_s[...], preferred_element_type=f32) + b1_row()[:, 0:128])

        def kv_fwd(j, sk, init=None):
            s = [jnp.broadcast_to(sk[l:l + 1, :], (8, 128)) for l in range(4)]
            dd = sk[4:5, :]
            fm = false_mask()
            lasts = [init] * kvn
            fwx = fw_ref[0]
            fwh = fw_ref[1]
            ev = lambda w: pltpu.bitcast(w << 16, f32)
            od = lambda w: pltpu.bitcast(w & jnp.uint32(0xffff0000), f32)
            kvs = []
            for a in range(NB + lag):
                if a < NB:
                    outs = []
                    for t in range(a * 8, a * 8 + 8):
                        bb = KP // 2 + 8 * t
                        w0 = ku_s[j, bb:bb + 8, :]
                        w1 = ku_s[j, bb - 1:bb + 7, :]
                        w2 = ku_s[j, bb - 2:bb + 6, :]
                        wv = vu_s[j, 8 * t:8 * t + 8, :]
                        e0, o0, e1, o1, o2 = ev(w0), od(w0), ev(w1), od(w1), od(w2)
                        ci = t % kvn
                        if lasts[ci] is not None:
                            e0 = jnp.where(fm, lasts[ci], e0)
                        oe = (e0 * s[0] + o1 * s[1] + e1 * s[2] + o2 * s[3]) * ev(wv)
                        oo = (e0 * s[1] + o0 * s[0] + o1 * s[2] + e1 * s[3]) * od(wv)
                        lasts[ci] = oo
                        outs += [oe, oo]
                    kvs.append(jnp.concatenate(outs, axis=0).astype(bf16))
                    hb = lax.dot_general(fwh, h_s[j, :, a * P:(a + 1) * P], NT, preferred_element_type=f32)
                    if a == 0:
                        hb = jnp.concatenate(
                            [hb[8 * t:8 * t + 8, :] + dd if t % 2 == 0 else hb[8 * t:8 * t + 8, :]
                             for t in range(32)], axis=0)
                    hf_s[a] = hb
                if a >= lag:
                    x_s[a - lag] = jnp.dot(fwx, kvs[a - lag], preferred_element_type=f32)

        def conv_mac(short):
            fm = false_mask()
            last = None
            Y = [[None] * 16 for _ in range(NB)]
            for p in range(16):
                r0, i0 = 16 * p, 16 * p + 8
                prev = None
                for c in range(NB):
                    accr = acci = pend = None
                    for a in range(c + 1):
                        b = c - a
                        xr = x_s[a, r0:r0 + 8, :]
                        xi = x_s[a, i0:i0 + 8, :]
                        hr = hf_s[b, r0:r0 + 8, :]
                        hi = hf_s[b, i0:i0 + 8, :]
                        if accr is None:
                            t1 = xr * hr
                            t2 = xr * hi
                            if last is not None:
                                t1 = jnp.where(fm, last[0], t1)
                                t2 = jnp.where(fm, last[1], t2)
                            accr = t1 - xi * hi
                            acci = t2 + xi * hr
                        elif short:
                            tr = xr * hr - xi * hi
                            ti = xr * hi + xi * hr
                            if pend is not None:
                                tr = tr + pend[0]
                                ti = ti + pend[1]
                                pend = None
                            elif a % mg == 1 and a < c:
                                pend = (tr, ti)
                                continue
                            accr = accr + tr
                            acci = acci + ti
                        else:
                            accr = (accr + xr * hr) - xi * hi
                            acci = (acci + xr * hi) + xi * hr
                    last = (accr, acci)
                    if prev is None:
                        yr, yi = accr, acci
                    else:
                        pr, pi = prev
                        yr, yi = (accr - pi, acci + pr) if p < 8 else (accr + pi, acci - pr)
                    prev = (accr, acci)
                    Y[c][p] = (yr, yi)
            return Y, last[0] + last[1]

        def conv_inv(j, Y):
            ic = inv_ref[0]
            isn = inv_ref[1]
            for c in range(NB):
                yr = jnp.concatenate([y[0] for y in Y[c]], axis=0).astype(bf16)
                yi = jnp.concatenate([y[1] for y in Y[c]], axis=0).astype(bf16)
                e = jnp.dot(ic, yr, preferred_element_type=f32)
                o = jnp.dot(isn, yi, preferred_element_type=f32)
                yp_s[j, c * P + 64:(c + 1) * P, :] = e - o
                lo = e + o
                for i in range(8):
                    yp_s[j, c * P + 8 * (7 - i):c * P + 8 * (8 - i), :] = lo[8 * i:8 * i + 8, :]

        def mlp_conv(i, short):
            r0 = M0 + i * M if isinstance(i, int) else pl.multiple_of(M0 + i * M, 64)
            Y, link = conv_mac(short)
            xn = load_xn(r0, M)
            h0 = mm1_first(xn)
            if short:
                ha = mm1(xn, 128, 128 * rpos)
                hr = mm1_rem(xn)
                h = jnp.concatenate([h0, ha, mm1(xn, 128 * rpos, FR), hr], axis=1)
            else:
                hr = mm1_rem(xn)
                h = jnp.concatenate([h0, mm1(xn, 128, FR), hr], axis=1)
            h = h.astype(bf16)
            b2 = b2_row()
            c4 = D - 128
            o = jnp.dot(h, w2_s[:, :c4], preferred_element_type=f32)
            p_s[pl.ds(r0, M), :c4] = o * OSC + (q_s[pl.ds(r0, M), :c4].astype(f32) + b2[:, :c4])
            z = jnp.where(false_mask()[0:1, :], link[0:1, :], b2[:, c4:] * (1.0 / OSC))
            o = z + jnp.dot(h, w2_s[:, c4:], preferred_element_type=f32)
            p_s[pl.ds(r0, M), c4:] = o * OSC + q_s[pl.ds(r0, M), c4:].astype(f32)
            conv_inv(i, Y)

        rev8 = 7 - row8

        def load_y(j, t):
            y = yp_s[j, t:t + 8, :]
            if t % P < 64:
                y = jnp.take_along_axis(y, rev8, axis=0)
            return y

        def combine(r0, r1, st):
            fm = false_mask()
            for t in range(r0, r1, 16):
                for j in range(NL):
                    cs = slice(j * 128, (j + 1) * 128)
                    y = jnp.concatenate([load_y(j, t), load_y(j, t + 8)], axis=0)
                    p0 = p_s[t:t + 8, cs]
                    if st[0] is not None:
                        p0 = jnp.where(fm, st[0], p0)
                    pp = jnp.concatenate([p0, p_s[t + 8:t + 16, cs]], axis=0)
                    r = (pp + xn_s[j, t:t + 16, :].astype(f32) * y).astype(bf16)
                    st[0] = r.astype(f32)[0:8, :]
                    o_s[j, t:t + 16, :] = r

        def first():
            wait(0)
            ln(0, qa, False)
            wait(1)

            def r0a():
                bc_s[...] = jnp.broadcast_to(b1_row()[:, F - 128:F], (128, 128)).T[64:128, :]
                hid_s[0:qa, 0:w1c[1]] = mm1(load_xn(0, qa), 0, w1c[1]).astype(bf16)
            region(r0a)
            wait(2)

            def r0b():
                ln(qa, M0, False)
                hid_s[qa:M0, 0:w1c[1]] = mm1(load_xn(qa, M0 - qa), 0, w1c[1]).astype(bf16)
            region(r0b)
            for i in range(1, n1):
                wait(2 + i)

                def r1(i=i):
                    if i == 1:
                        for j in range(NL):
                            w1n_s[j * 128:(j + 1) * 128, :] = (
                                w1_s[0:128, j * 128:(j + 1) * 128].astype(f32).T.astype(bf16))
                    hid_s[:, w1c[i]:w1c[i + 1]] = mm1(load_xn(0, M0), w1c[i], w1c[i + 1]).astype(bf16)
                region(r1)
            wait(ng - 4)

            def r2a():
                ln(M0, M0 + lns, True)
                p_s[0:M0, :] = jnp.dot(hid_s[:, :w2k], w2_s[:w2k, :], preferred_element_type=f32)
            region(r2a)
            wait(ng - 3)

            def r2b():
                lk = jnp.broadcast_to(ln(M0 + lns, S, True)[0:8, :], (8, 128))
                o = jnp.dot(hid_s[:, w2k:], w2_s[w2k:, :], preferred_element_type=f32) + p_s[0:M0, :]
                p_s[0:M0, :] = o * OSC + (q_s[0:M0, :].astype(f32) + b2_row())
                par = jnp.concatenate([sk_ref[...].astype(f32), dd_ref[...].astype(f32).reshape(1, D),
                                       jnp.zeros((3, D), f32)], axis=0)
                for j in range(NL):
                    par_s[j] = par[:, j * 128:(j + 1) * 128]
                kv_fwd(0, par[:, 0:128], lk)
            region(r2b)

        def pair(i, carry):
            si = lax.rem(ng - 2 + i, ring)
            for c in copies(kvh(2 * i + 1) + kvh(2 * i + 2), si):
                c.wait()
            mlp_conv(2 * i, False)
            kv_fwd(2 * i + 1, par_s[2 * i + 1])
            z = NB + flag_s[1]
            x_s[z, 0:8, :] = jnp.zeros((8, 128), f32)
            hf_s[z, 0:8, :] = jnp.zeros((8, 128), f32)
            mlp_conv(2 * i + 1, True)
            kv_fwd(2 * i + 2, par_s[2 * i + 2])
            return carry

        rl = S - ML

        def out_copies(js, r0, r1):
            return copies([(o_s.at[j, pl.ds(r0, r1 - r0), :], out_hbm.at[pl.ds(r0, r1 - r0), pl.ds(j * 128, 128)])
                           for j in js], sem_out)
        cuts = [0] + [int(rl // 16 * x) * 16 for x in prow] + [rl]
        g_o = [out_copies(range(NL), cuts[i], cuts[i + 1]) for i in range(nco)]
        g_fa = out_copies(range(osp), rl, S)
        g_fb = out_copies(range(osp, NL), rl, S)

        def pin_after(g, i):
            for c in g:
                c.start()
            z1 = pl.multiple_of(S + flag_s[1], 16)
            z2 = pl.multiple_of(S + flag_s[2], 16)
            o_s[0, pl.ds(z1, 16), :] = jnp.full((16, 128), i, bf16)
            return o_s[0, pl.ds(z2, 16), :].astype(f32)

        def last():
            mlp_conv(NL - 1, False)
            yp_s[NL + flag_s[1], 0:8, :] = jnp.zeros((8, 128), f32)
            p_s[pl.ds(pl.multiple_of(S + flag_s[1], 8), 8), 0:128] = jnp.zeros((8, 128), f32)
            xn = load_xn(rl, ML)
            st = [None]
            hs = []
            gi = 0
            for f in range(13):
                pin = None
                if gi < nco and pins[gi] == f:
                    combine(cuts[gi], cuts[gi + 1], st)
                    pin = pin_after(g_o[gi], gi)
                    gi += 1
                hs.append(mm1(xn, 128 * f, 128 * (f + 1), pin) if f else mm1_first(xn))
            hs.append(mm1_rem(xn))
            h = jnp.concatenate(hs, axis=1).astype(bf16)
            b2 = b2_row() * (1.0 / OSC)
            for j in range(NL):
                cs = slice(j * 128, (j + 1) * 128)
                bj = b2[:, cs]
                if gi < nco and pins[gi] == 14 + j:
                    combine(cuts[gi], cuts[gi + 1], st)
                    bj = jnp.where(false_mask()[0:1, :], pin_after(g_o[gi], gi)[0:1, :], bj)
                    gi += 1
                if j == osp:
                    bj = jnp.where(false_mask()[0:1, :], pin_after(g_fa, nco)[0:1, :], bj)
                o = (bj + jnp.dot(h, w2_s[:, cs], preferred_element_type=f32)) * OSC + q_s[rl:S, cs].astype(f32)
                y = jnp.concatenate([load_y(j, t) for t in range(rl, S, 8)], axis=0)
                o_s[j, rl:S, :] = (o + xn_s[j, rl:S, :].astype(f32) * y).astype(bf16)
            assert gi == nco
        def it(i, carry):
            pl.when(i == 0)(first)
            pair(i, carry)
            pl.when(i == 1)(last)
            return carry
        lax.fori_loop(0, 2, it, 0)
        for c in g_fb:
            c.start()
        for g in g_o + [g_fa, g_fb]:
            for c in g:
                c.wait()

    fw, inv = dft_mats()

    @jax.jit
    def f(q, k, v, sk, h, dd, w1, b1, w2, b2):
        any_ = pl.BlockSpec(memory_space=pl.ANY)
        out = pl.pallas_call(
            kernel,
            in_specs=[any_] * 12,
            out_specs=any_,
            out_shape=jax.ShapeDtypeStruct((S, D), bf16),
            scratch_shapes=[
                pltpu.VMEM((S, D), bf16),
                pltpu.VMEM((NL, S + KP, 128), bf16),
                pltpu.VMEM((NL, S, 128), bf16),
                pltpu.VMEM((NL, 128, S), bf16),
                pltpu.VMEM((F, D), bf16),
                pltpu.VMEM((F, D), bf16),
                pltpu.VMEM((NL, S, 128), bf16),
                pltpu.VMEM((S + 8, D), f32),
                pltpu.VMEM((NB + 1, 256, 128), f32),
                pltpu.VMEM((NB + 1, 256, 128), f32),
                pltpu.VMEM((NL + 1, S, 128), f32),
                pltpu.VMEM((NL, S + 16, 128), bf16),
                pltpu.VMEM((NL, 8, 128), f32),
                pltpu.VMEM((M0, F), bf16),
                pltpu.VMEM((4, D), bf16), pltpu.VMEM((D,), bf16), pltpu.VMEM((F,), bf16), pltpu.VMEM((D,), bf16),
                pltpu.VMEM((2, 256, 128), bf16), pltpu.VMEM((2, 64, 128), bf16),
                pltpu.VMEM((64, 128), f32),
                pltpu.VMEM((D, 128), bf16),
                pltpu.SMEM((4,), jnp.int32),
                pltpu.SemaphoreType.DMA((ring,)),
            ],
            compiler_params=pltpu.CompilerParams(vmem_limit_bytes=100 * 2**20),
            name=name,
        )(q.reshape(S, D), k.reshape(S, D), v.reshape(S, D), sk.T, h, dd, w1.T, b1, w2, b2, fw, inv)
        return out.reshape(1, S, D)
    return f


_impl = make(name="fused_h3_mlp")


@jax.jit
def pallas_parallel_sum__ssm_conv_h3__dense_activation_gelu__prompt_kernel(
    A_q, A_k, A_v, A_shift_k, A_ssm_k, A_ssm_D, B_x, B_w1, B_b1, B_w2, B_b2,
):
    del B_x
    return _impl(A_q, A_k, A_v, A_shift_k, A_ssm_k, A_ssm_D, B_w1, B_b1, B_w2, B_b2)
```

```python
import numpy as np
import jax
import jax.numpy as jnp
from jax import lax
import jax.experimental.pallas as pl
import jax.experimental.pallas.tpu as pltpu

S, D, F = 2048, 640, 1728
P = 128
NB = S // P
NL = D // 128
KP = 64
FR = F - 64
f32, bf16, u32 = jnp.float32, jnp.bfloat16, jnp.uint32
NT = (((1,), (1,)), ((), ()))

ALPHA = (0.7978845608028654 * 0.044715) ** (1.0 / 3.0)
C1 = 0.7978845608028654 / ALPHA
OSC = 0.5 / ALPHA


def dft_mats():
    ks = np.concatenate([np.arange(0, 128, 2), np.arange(1, 128, 2)])
    n = np.arange(128)
    m = np.arange(64) + 0.5
    fw = np.zeros((2, 256, 128))
    inv = np.zeros((2, 64, 128))
    for p in range(16):
        for s in range(8):
            w = 2 * np.pi * (ks[8 * p + s] + 0.5) / 256
            fw[0, 16 * p + s] = np.cos(w * (n - 63.5))
            fw[0, 16 * p + 8 + s] = -np.sin(w * (n - 63.5))
            fw[1, 16 * p + s] = np.cos(w * n)
            fw[1, 16 * p + 8 + s] = -np.sin(w * n)
            inv[0, :, 8 * p + s] = np.cos(w * m) / (128 * ALPHA)
            inv[1, :, 8 * p + s] = np.sin(w * m) / (128 * ALPHA)
    perm = np.concatenate(
        [16 * t + np.concatenate([np.arange(0, 16, 2), np.arange(1, 16, 2)]) for t in range(8)])
    fw[0] = fw[0][:, perm]
    return fw.astype(np.float32).astype(bf16), inv.astype(np.float32).astype(bf16)


def gelu(g):
    return g * (1.0 + jnp.tanh(g * (C1 + g * g)))


def make(M0=576, M=256, name="v47", kvn=2, qa=256, w1c=(0, 256, 768, F), w2k=1024, lns=960,
         pins=(2, 7, 12, 15), prow=(0.01, 0.28, 0.6), osp=3, lag=4, mg=3, ring=4, rpos=4):
    ML = S - M0 - NL * M
    assert ML > 0 and ML % 16 == 0 and M0 % 64 == 0 and M % 64 == 0
    n1, nco = len(w1c) - 1, len(pins)

    def kernel(q_hbm, k_hbm, v_hbm, sk_hbm, h_hbm, dd_hbm, w1_hbm, b1_hbm, w2_hbm, b2_hbm, fw_hbm, inv_hbm,
               out_hbm,
               q_s, ql_s, k_s, v_s, h_s, w1_s, w2_s, xn_s, p_s, x_s, hf_s, yp_s, o_s, par_s, hid_s,
               sk_ref, dd_ref, b1_ref, b2_ref, fw_ref, inv_ref, bc_s, w1n_s, flag_s, sem):
        def rows(src, dst, r0, r1):
            return (src.at[pl.ds(r0, r1 - r0)], dst.at[pl.ds(r0, r1 - r0)])

        def qrows(r0, r1):
            return [(q_hbm.at[pl.ds(r0, r1 - r0), pl.ds(j * 128, 128)], ql_s.at[j, pl.ds(r0, r1 - r0), :])
                    for j in range(NL)]

        def load_q(r0, m, j0=0, j1=NL):
            if isinstance(r0, int) and r0 < M0:
                return q_s[r0:r0 + m, j0 * 128:j1 * 128].astype(f32)
            return jnp.concatenate([ql_s[j, pl.ds(r0, m), :].astype(f32) for j in range(j0, j1)], axis=1)

        def kvh(j):
            lane = pl.ds(j * 128, 128) if isinstance(j, int) else pl.ds(pl.multiple_of(j * 128, 128), 128)
            return [(h_hbm.at[lane, :], h_s.at[j]),
                    (k_hbm.at[:, lane], k_s.at[j, pl.ds(KP, S), :]),
                    (v_hbm.at[:, lane], v_s.at[j])]

        def copies(g, si):
            return [pltpu.make_async_copy(src, dst, sem.at[si]) for src, dst in g]

        groups = [[rows(q_hbm, q_s, 0, qa)],
                  [rows(w1_hbm, w1_s, 0, w1c[1]), (b1_hbm, b1_ref)],
                  [rows(q_hbm, q_s, qa, M0)]]
        groups += [[rows(w1_hbm, w1_s, w1c[i], w1c[i + 1])] for i in range(1, n1)]
        groups += [qrows(M0, M0 + lns) + [rows(w2_hbm, w2_s, 0, w2k)],
                   qrows(M0 + lns, S) + [rows(w2_hbm, w2_s, w2k, F), (b2_hbm, b2_ref), (sk_hbm, sk_ref),
                                         (dd_hbm, dd_ref), (fw_hbm, fw_ref), (inv_hbm, inv_ref)] + kvh(0),
                   kvh(1) + kvh(2), kvh(3) + kvh(4)]
        ng = len(groups)
        assert ng == 2 + n1 + ring
        sem_out = (ng - 3) % ring

        def start(g):
            if g < ng:
                for c in copies(groups[g], g % ring):
                    c.start()

        def wait(g):
            for c in copies(groups[g], g % ring):
                c.wait()

        for g in range(ring):
            start(g)

        flag_s[0] = 100
        flag_s[1] = 0
        flag_s[2] = 0
        for j in range(NL):
            k_s[j, KP - 16:KP, :] = jnp.zeros((16, 128), bf16)
        ku_s = k_s.bitcast(u32)
        vu_s = v_s.bitcast(u32)

        def region(fn):
            pl.when(flag_s[0] == 100)(fn)

        row8 = lax.broadcasted_iota(jnp.int32, (8, 128), 0)

        def false_mask():
            return row8 > flag_s[0]

        def ln(r0, r1, chain):
            fm = lax.broadcasted_iota(jnp.int32, (16, 1), 0) > flag_s[0]
            rs = None
            for rr in range(r0, r1, 16):
                x = load_q(rr, 16)
                xc = x - jnp.sum(x, axis=-1, keepdims=True) * (1.0 / D)
                var = jnp.sum(xc * xc, axis=-1, keepdims=True) * (1.0 / D)
                if chain and rs is not None:
                    var = jnp.where(fm, rs, var)
                rs = lax.rsqrt(var + 1e-5) * ALPHA
                xo = xc * rs
                for j in range(NL):
                    xn_s[j, rr:rr + 16, :] = xo[:, j * 128:(j + 1) * 128].astype(bf16)
            return rs

        def load_xn(r0, m):
            return jnp.concatenate([xn_s[j, pl.ds(r0, m), :] for j in range(NL)], axis=1)

        def b1_row():
            return b1_ref[...].astype(f32).reshape(1, F) * ALPHA

        def b2_row():
            return b2_ref[...].astype(f32).reshape(1, D)

        def mm1_rem(xn):
            m = xn.shape[0]
            ht = lax.dot_general(w1_s[FR:F, :], xn, NT, preferred_element_type=f32)
            bc = bc_s[...]
            outs = []
            for c0 in range(0, m, 128):
                c1 = min(c0 + 128, m)
                outs.append(gelu(ht[:, c0:c1] + bc[:, :c1 - c0]).T)
            return jnp.concatenate(outs, axis=0)

        def mm1(xn, f0=0, f1=F, pin=None):
            if f1 == F:
                hr = mm1_rem(xn)
                if f0 == FR:
                    return hr
                return jnp.concatenate([mm1(xn, f0, FR, pin), hr], axis=1)
            b1 = b1_row()[:, f0:f1]
            if pin is not None:
                b1 = jnp.where(false_mask()[0:1, :f1 - f0], pin[0:1, :f1 - f0], b1)
            h = lax.dot_general(xn, w1_s[f0:f1, :], NT, preferred_element_type=f32) + b1
            return gelu(h)

        def mm1_first(xn):
            return gelu(jnp.dot(xn, w1n_s[...], preferred_element_type=f32) + b1_row()[:, 0:128])

        def kv_fwd(j, sk, init=None):
            s = [jnp.broadcast_to(sk[l:l + 1, :], (8, 128)) for l in range(4)]
            dd = sk[4:5, :]
            fm = false_mask()
            lasts = [init] * kvn
            fwx = fw_ref[0]
            fwh = fw_ref[1]
            ev = lambda w: pltpu.bitcast(w << 16, f32)
            od = lambda w: pltpu.bitcast(w & jnp.uint32(0xffff0000), f32)
            kvs = []
            for a in range(NB + lag):
                if a < NB:
                    outs = []
                    for t in range(a * 8, a * 8 + 8):
                        bb = KP // 2 + 8 * t
                        w0 = ku_s[j, bb:bb + 8, :]
                        w1 = ku_s[j, bb - 1:bb + 7, :]
                        w2 = ku_s[j, bb - 2:bb + 6, :]
                        wv = vu_s[j, 8 * t:8 * t + 8, :]
                        e0, o0, e1, o1, o2 = ev(w0), od(w0), ev(w1), od(w1), od(w2)
                        ci = t % kvn
                        if lasts[ci] is not None:
                            e0 = jnp.where(fm, lasts[ci], e0)
                        oe = (e0 * s[0] + o1 * s[1] + e1 * s[2] + o2 * s[3]) * ev(wv)
                        oo = (e0 * s[1] + o0 * s[0] + o1 * s[2] + e1 * s[3]) * od(wv)
                        lasts[ci] = oo
                        outs += [oe, oo]
                    kvs.append(jnp.concatenate(outs, axis=0).astype(bf16))
                    hb = lax.dot_general(fwh, h_s[j, :, a * P:(a + 1) * P], NT, preferred_element_type=f32)
                    if a == 0:
                        hb = jnp.concatenate(
                            [hb[8 * t:8 * t + 8, :] + dd if t % 2 == 0 else hb[8 * t:8 * t + 8, :]
                             for t in range(32)], axis=0)
                    hf_s[a] = hb
                if a >= lag:
                    x_s[a - lag] = jnp.dot(fwx, kvs[a - lag], preferred_element_type=f32)

        def conv_mac(short):
            fm = false_mask()
            last = None
            Y = [[None] * 16 for _ in range(NB)]
            for p in range(16):
                r0, i0 = 16 * p, 16 * p + 8
                prev = None
                for c in range(NB):
                    accr = acci = pend = None
                    for a in range(c + 1):
                        b = c - a
                        xr = x_s[a, r0:r0 + 8, :]
                        xi = x_s[a, i0:i0 + 8, :]
                        hr = hf_s[b, r0:r0 + 8, :]
                        hi = hf_s[b, i0:i0 + 8, :]
                        if accr is None:
                            t1 = xr * hr
                            t2 = xr * hi
                            if last is not None:
                                t1 = jnp.where(fm, last[0], t1)
                                t2 = jnp.where(fm, last[1], t2)
                            accr = t1 - xi * hi
                            acci = t2 + xi * hr
                        elif short:
                            tr = xr * hr - xi * hi
                            ti = xr * hi + xi * hr
                            if pend is not None:
                                tr = tr + pend[0]
                                ti = ti + pend[1]
                                pend = None
                            elif a % mg == 1 and a < c:
                                pend = (tr, ti)
                                continue
                            accr = accr + tr
                            acci = acci + ti
                        else:
                            accr = (accr + xr * hr) - xi * hi
                            acci = (acci + xr * hi) + xi * hr
                    last = (accr, acci)
                    if prev is None:
                        yr, yi = accr, acci
                    else:
                        pr, pi = prev
                        yr, yi = (accr - pi, acci + pr) if p < 8 else (accr + pi, acci - pr)
                    prev = (accr, acci)
                    Y[c][p] = (yr, yi)
            return Y, last[0] + last[1]

        def conv_inv(j, Y):
            ic = inv_ref[0]
            isn = inv_ref[1]
            for c in range(NB):
                yr = jnp.concatenate([y[0] for y in Y[c]], axis=0).astype(bf16)
                yi = jnp.concatenate([y[1] for y in Y[c]], axis=0).astype(bf16)
                e = jnp.dot(ic, yr, preferred_element_type=f32)
                o = jnp.dot(isn, yi, preferred_element_type=f32)
                yp_s[j, c * P + 64:(c + 1) * P, :] = e - o
                lo = e + o
                for i in range(8):
                    yp_s[j, c * P + 8 * (7 - i):c * P + 8 * (8 - i), :] = lo[8 * i:8 * i + 8, :]

        def mlp_conv(i, short):
            r0 = M0 + i * M if isinstance(i, int) else pl.multiple_of(M0 + i * M, 64)
            Y, link = conv_mac(short)
            xn = load_xn(r0, M)
            h0 = mm1_first(xn)
            if short:
                ha = mm1(xn, 128, 128 * rpos)
                hr = mm1_rem(xn)
                h = jnp.concatenate([h0, ha, mm1(xn, 128 * rpos, FR), hr], axis=1)
            else:
                hr = mm1_rem(xn)
                h = jnp.concatenate([h0, mm1(xn, 128, FR), hr], axis=1)
            h = h.astype(bf16)
            b2 = b2_row()
            c4 = D - 128
            o = jnp.dot(h, w2_s[:, :c4], preferred_element_type=f32)
            p_s[pl.ds(r0, M), :c4] = o * OSC + (load_q(r0, M, 0, NL - 1) + b2[:, :c4])
            z = jnp.where(false_mask()[0:1, :], link[0:1, :], b2[:, c4:] * (1.0 / OSC))
            o = z + jnp.dot(h, w2_s[:, c4:], preferred_element_type=f32)
            p_s[pl.ds(r0, M), c4:] = o * OSC + load_q(r0, M, NL - 1, NL)
            conv_inv(i, Y)

        rev8 = 7 - row8

        def load_y(j, t):
            y = yp_s[j, t:t + 8, :]
            if t % P < 64:
                y = jnp.take_along_axis(y, rev8, axis=0)
            return y

        def combine(r0, r1, st):
            fm = false_mask()
            for t in range(r0, r1, 16):
                for j in range(NL):
                    cs = slice(j * 128, (j + 1) * 128)
                    y = jnp.concatenate([load_y(j, t), load_y(j, t + 8)], axis=0)
                    p0 = p_s[t:t + 8, cs]
                    if st[0] is not None:
                        p0 = jnp.where(fm, st[0], p0)
                    pp = jnp.concatenate([p0, p_s[t + 8:t + 16, cs]], axis=0)
                    r = (pp + xn_s[j, t:t + 16, :].astype(f32) * y).astype(bf16)
                    st[0] = r.astype(f32)[0:8, :]
                    o_s[j, t:t + 16, :] = r

        def first():
            wait(0)
            start(ring)
            ln(0, qa, False)
            wait(1)

            def r0a():
                start(1 + ring)
                bc_s[...] = jnp.broadcast_to(b1_row()[:, F - 128:F], (128, 128)).T[64:128, :]
                hid_s[0:qa, 0:w1c[1]] = mm1(load_xn(0, qa), 0, w1c[1]).astype(bf16)
            region(r0a)
            wait(2)

            def r0b():
                start(2 + ring)
                ln(qa, M0, False)
                hid_s[qa:M0, 0:w1c[1]] = mm1(load_xn(qa, M0 - qa), 0, w1c[1]).astype(bf16)
            region(r0b)
            for i in range(1, n1):
                wait(2 + i)

                def r1(i=i):
                    start(2 + i + ring)
                    if i == 1:
                        for j in range(NL):
                            w1n_s[j * 128:(j + 1) * 128, :] = (
                                w1_s[0:128, j * 128:(j + 1) * 128].astype(f32).T.astype(bf16))
                    hid_s[:, w1c[i]:w1c[i + 1]] = mm1(load_xn(0, M0), w1c[i], w1c[i + 1]).astype(bf16)
                region(r1)
            wait(ng - 4)

            def r2a():
                ln(M0, M0 + lns, True)
                p_s[0:M0, :] = jnp.dot(hid_s[:, :w2k], w2_s[:w2k, :], preferred_element_type=f32)
            region(r2a)
            wait(ng - 3)

            def r2b():
                lk = jnp.broadcast_to(ln(M0 + lns, S, True)[0:8, :], (8, 128))
                o = jnp.dot(hid_s[:, w2k:], w2_s[w2k:, :], preferred_element_type=f32) + p_s[0:M0, :]
                p_s[0:M0, :] = o * OSC + (load_q(0, M0) + b2_row())
                par = jnp.concatenate([sk_ref[...].astype(f32), dd_ref[...].astype(f32).reshape(1, D),
                                       jnp.zeros((3, D), f32)], axis=0)
                for j in range(NL):
                    par_s[j] = par[:, j * 128:(j + 1) * 128]
                kv_fwd(0, par[:, 0:128], lk)
            region(r2b)

        def pair(i, carry):
            si = lax.rem(ng - 2 + i, ring)
            for c in copies(kvh(2 * i + 1) + kvh(2 * i + 2), si):
                c.wait()
            mlp_conv(2 * i, False)
            kv_fwd(2 * i + 1, par_s[2 * i + 1])
            z = NB + flag_s[1]
            x_s[z, 0:8, :] = jnp.zeros((8, 128), f32)
            hf_s[z, 0:8, :] = jnp.zeros((8, 128), f32)
            mlp_conv(2 * i + 1, True)
            kv_fwd(2 * i + 2, par_s[2 * i + 2])
            return carry

        rl = S - ML

        def out_copies(js, r0, r1):
            return copies([(o_s.at[j, pl.ds(r0, r1 - r0), :], out_hbm.at[pl.ds(r0, r1 - r0), pl.ds(j * 128, 128)])
                           for j in js], sem_out)
        cuts = [0] + [int(rl // 16 * x) * 16 for x in prow] + [rl]
        g_o = [out_copies(range(NL), cuts[i], cuts[i + 1]) for i in range(nco)]
        g_fa = out_copies(range(osp), rl, S)
        g_fb = out_copies(range(osp, NL), rl, S)

        def pin_after(g, i):
            for c in g:
                c.start()
            z1 = pl.multiple_of(S + flag_s[1], 16)
            z2 = pl.multiple_of(S + flag_s[2], 16)
            o_s[0, pl.ds(z1, 16), :] = jnp.full((16, 128), i, bf16)
            return o_s[0, pl.ds(z2, 16), :].astype(f32)

        def last():
            mlp_conv(NL - 1, False)
            yp_s[NL + flag_s[1], 0:8, :] = jnp.zeros((8, 128), f32)
            p_s[pl.ds(pl.multiple_of(S + flag_s[1], 8), 8), 0:128] = jnp.zeros((8, 128), f32)
            xn = load_xn(rl, ML)
            st = [None]
            hs = []
            gi = 0
            for f in range(13):
                pin = None
                if gi < nco and pins[gi] == f:
                    combine(cuts[gi], cuts[gi + 1], st)
                    pin = pin_after(g_o[gi], gi)
                    gi += 1
                hs.append(mm1(xn, 128 * f, 128 * (f + 1), pin) if f else mm1_first(xn))
            hs.append(mm1_rem(xn))
            h = jnp.concatenate(hs, axis=1).astype(bf16)
            b2 = b2_row() * (1.0 / OSC)
            for j in range(NL):
                cs = slice(j * 128, (j + 1) * 128)
                bj = b2[:, cs]
                if gi < nco and pins[gi] == 14 + j:
                    combine(cuts[gi], cuts[gi + 1], st)
                    bj = jnp.where(false_mask()[0:1, :], pin_after(g_o[gi], gi)[0:1, :], bj)
                    gi += 1
                if j == osp:
                    bj = jnp.where(false_mask()[0:1, :], pin_after(g_fa, nco)[0:1, :], bj)
                o = (bj + jnp.dot(h, w2_s[:, cs], preferred_element_type=f32)) * OSC + load_q(rl, ML, j, j + 1)
                y = jnp.concatenate([load_y(j, t) for t in range(rl, S, 8)], axis=0)
                o_s[j, rl:S, :] = (o + xn_s[j, rl:S, :].astype(f32) * y).astype(bf16)
            assert gi == nco
        def it(i, carry):
            pl.when(i == 0)(first)
            pair(i, carry)
            pl.when(i == 1)(last)
            return carry
        lax.fori_loop(0, 2, it, 0)
        for c in g_fb:
            c.start()
        for g in g_o + [g_fa, g_fb]:
            for c in g:
                c.wait()

    fw, inv = dft_mats()

    @jax.jit
    def f(q, k, v, sk, h, dd, w1, b1, w2, b2):
        any_ = pl.BlockSpec(memory_space=pl.ANY)
        out = pl.pallas_call(
            kernel,
            in_specs=[any_] * 12,
            out_specs=any_,
            out_shape=jax.ShapeDtypeStruct((S, D), bf16),
            scratch_shapes=[
                pltpu.VMEM((M0, D), bf16),
                pltpu.VMEM((NL, S, 128), bf16),
                pltpu.VMEM((NL, S + KP, 128), bf16),
                pltpu.VMEM((NL, S, 128), bf16),
                pltpu.VMEM((NL, 128, S), bf16),
                pltpu.VMEM((F, D), bf16),
                pltpu.VMEM((F, D), bf16),
                pltpu.VMEM((NL, S, 128), bf16),
                pltpu.VMEM((S + 8, D), f32),
                pltpu.VMEM((NB + 1, 256, 128), f32),
                pltpu.VMEM((NB + 1, 256, 128), f32),
                pltpu.VMEM((NL + 1, S, 128), f32),
                pltpu.VMEM((NL, S + 16, 128), bf16),
                pltpu.VMEM((NL, 8, 128), f32),
                pltpu.VMEM((M0, F), bf16),
                pltpu.VMEM((4, D), bf16), pltpu.VMEM((D,), bf16), pltpu.VMEM((F,), bf16), pltpu.VMEM((D,), bf16),
                pltpu.VMEM((2, 256, 128), bf16), pltpu.VMEM((2, 64, 128), bf16),
                pltpu.VMEM((64, 128), f32),
                pltpu.VMEM((D, 128), bf16),
                pltpu.SMEM((4,), jnp.int32),
                pltpu.SemaphoreType.DMA((ring,)),
            ],
            compiler_params=pltpu.CompilerParams(vmem_limit_bytes=100 * 2**20),
            name=name,
        )(q.reshape(S, D), k.reshape(S, D), v.reshape(S, D), sk.T, h, dd, w1.T, b1, w2, b2, fw, inv)
        return out.reshape(1, S, D)
    return f


_impl = make(name="fused_h3_mlp")


@jax.jit
def pallas_parallel_sum__ssm_conv_h3__dense_activation_gelu__prompt_kernel(
    A_q, A_k, A_v, A_shift_k, A_ssm_k, A_ssm_D, B_x, B_w1, B_b1, B_w2, B_b2,
):
    del B_x
    return _impl(A_q, A_k, A_v, A_shift_k, A_ssm_k, A_ssm_D, B_w1, B_b1, B_w2, B_b2)
```

```python
import numpy as np
import jax
import jax.numpy as jnp
from jax import lax
import jax.experimental.pallas as pl
import jax.experimental.pallas.tpu as pltpu

S, D, F = 2048, 640, 1728
P = 128
NB = S // P
NL = D // 128
KP = 64
FR = F - 64
f32, bf16, u32 = jnp.float32, jnp.bfloat16, jnp.uint32
NT = (((1,), (1,)), ((), ()))

ALPHA = (0.7978845608028654 * 0.044715) ** (1.0 / 3.0)
C1 = 0.7978845608028654 / ALPHA
OSC = 0.5 / ALPHA


def dft_mats():
    ks = np.concatenate([np.arange(0, 128, 2), np.arange(1, 128, 2)])
    n = np.arange(128)
    m = np.arange(64) + 0.5
    fw = np.zeros((2, 256, 128))
    inv = np.zeros((2, 64, 128))
    for p in range(16):
        for s in range(8):
            w = 2 * np.pi * (ks[8 * p + s] + 0.5) / 256
            fw[0, 16 * p + s] = np.cos(w * (n - 63.5))
            fw[0, 16 * p + 8 + s] = -np.sin(w * (n - 63.5))
            fw[1, 16 * p + s] = np.cos(w * n)
            fw[1, 16 * p + 8 + s] = -np.sin(w * n)
            inv[0, :, 8 * p + s] = np.cos(w * m) / (128 * ALPHA)
            inv[1, :, 8 * p + s] = np.sin(w * m) / (128 * ALPHA)
    perm = np.concatenate(
        [16 * t + np.concatenate([np.arange(0, 16, 2), np.arange(1, 16, 2)]) for t in range(8)])
    fw[0] = fw[0][:, perm]
    return fw.astype(np.float32).astype(bf16), inv.astype(np.float32).astype(bf16)


def gelu(g):
    return g * (1.0 + jnp.tanh(g * (C1 + g * g)))


def make(M0=576, M=256, name="v50", kvn=2, qa=256, w1c=(0, 256, 768, F), w2k=1024, lns=960,
         pins=(2, 7, 12, 15), prow=(0.01, 0.28, 0.6), osp=4, lag=4, mg=3, ring=4, rpos=4, rsp=96):
    ML = S - M0 - NL * M
    assert ML > 0 and ML % 16 == 0 and M0 % 64 == 0 and M % 64 == 0
    n1, nco = len(w1c) - 1, len(pins)

    def kernel(q_hbm, k_hbm, v_hbm, sk_hbm, h_hbm, dd_hbm, w1_hbm, b1_hbm, w2_hbm, b2_hbm, fw_hbm, inv_hbm,
               out_hbm,
               q_s, ql_s, k_s, v_s, h_s, w1_s, w2_s, xn_s, p_s, x_s, hf_s, yp_s, o_s, par_s, hid_s,
               sk_ref, dd_ref, b1_ref, b2_ref, fw_ref, inv_ref, bc_s, w1n_s, flag_s, sem):
        def rows(src, dst, r0, r1):
            return (src.at[pl.ds(r0, r1 - r0)], dst.at[pl.ds(r0, r1 - r0)])

        def qrows(r0, r1):
            return [(q_hbm.at[pl.ds(r0, r1 - r0), pl.ds(j * 128, 128)], ql_s.at[j, pl.ds(r0, r1 - r0), :])
                    for j in range(NL)]

        def load_q(r0, m, j0=0, j1=NL):
            if isinstance(r0, int) and r0 < M0:
                return q_s[r0:r0 + m, j0 * 128:j1 * 128].astype(f32)
            return jnp.concatenate([ql_s[j, pl.ds(r0, m), :].astype(f32) for j in range(j0, j1)], axis=1)

        def kvh(j):
            lane = pl.ds(j * 128, 128) if isinstance(j, int) else pl.ds(pl.multiple_of(j * 128, 128), 128)
            return [(h_hbm.at[lane, :], h_s.at[j]),
                    (k_hbm.at[:, lane], k_s.at[j, pl.ds(KP, S), :]),
                    (v_hbm.at[:, lane], v_s.at[j])]

        def copies(g, si):
            return [pltpu.make_async_copy(src, dst, sem.at[si]) for src, dst in g]

        groups = [[rows(q_hbm, q_s, 0, qa)],
                  [rows(w1_hbm, w1_s, 0, w1c[1]), (b1_hbm, b1_ref)],
                  [rows(q_hbm, q_s, qa, M0)]]
        groups += [[rows(w1_hbm, w1_s, w1c[i], w1c[i + 1])] for i in range(1, n1)]
        groups += [qrows(M0, M0 + lns) + [rows(w2_hbm, w2_s, 0, w2k)],
                   qrows(M0 + lns, S) + [rows(w2_hbm, w2_s, w2k, F), (b2_hbm, b2_ref), (sk_hbm, sk_ref),
                                         (dd_hbm, dd_ref), (fw_hbm, fw_ref), (inv_hbm, inv_ref)] + kvh(0),
                   kvh(1) + kvh(2), kvh(3) + kvh(4)]
        ng = len(groups)
        assert ng == 2 + n1 + ring
        sem_out = (ng - 3) % ring

        def start(g):
            if g < ng:
                for c in copies(groups[g], g % ring):
                    c.start()

        def wait(g):
            for c in copies(groups[g], g % ring):
                c.wait()

        for g in range(ring):
            start(g)

        flag_s[0] = 100
        flag_s[1] = 0
        flag_s[2] = 0
        for j in range(NL):
            k_s[j, KP - 16:KP, :] = jnp.zeros((16, 128), bf16)
        ku_s = k_s.bitcast(u32)
        vu_s = v_s.bitcast(u32)

        def region(fn):
            pl.when(flag_s[0] == 100)(fn)

        row8 = lax.broadcasted_iota(jnp.int32, (8, 128), 0)

        def false_mask():
            return row8 > flag_s[0]

        def ln(r0, r1, chain):
            fm = lax.broadcasted_iota(jnp.int32, (16, 1), 0) > flag_s[0]
            rs = None
            for rr in range(r0, r1, 16):
                x = load_q(rr, 16)
                xc = x - jnp.sum(x, axis=-1, keepdims=True) * (1.0 / D)
                var = jnp.sum(xc * xc, axis=-1, keepdims=True) * (1.0 / D)
                if chain and rs is not None:
                    var = jnp.where(fm, rs, var)
                rs = lax.rsqrt(var + 1e-5) * ALPHA
                xo = xc * rs
                for j in range(NL):
                    xn_s[j, rr:rr + 16, :] = xo[:, j * 128:(j + 1) * 128].astype(bf16)
            return rs

        def load_xn(r0, m):
            return jnp.concatenate([xn_s[j, pl.ds(r0, m), :] for j in range(NL)], axis=1)

        def b1_row():
            return b1_ref[...].astype(f32).reshape(1, F) * ALPHA

        def b2_row():
            return b2_ref[...].astype(f32).reshape(1, D)

        def mm1_rem(xn):
            m = xn.shape[0]
            ht = lax.dot_general(w1_s[FR:F, :], xn, NT, preferred_element_type=f32)
            bc = bc_s[...]
            outs = []
            for c0 in range(0, m, 128):
                c1 = min(c0 + 128, m)
                outs.append(gelu(ht[:, c0:c1] + bc[:, :c1 - c0]).T)
            return jnp.concatenate(outs, axis=0)

        def mm1(xn, f0=0, f1=F, pin=None):
            if f1 == F:
                hr = mm1_rem(xn)
                if f0 == FR:
                    return hr
                return jnp.concatenate([mm1(xn, f0, FR, pin), hr], axis=1)
            b1 = b1_row()[:, f0:f1]
            if pin is not None:
                b1 = jnp.where(false_mask()[0:1, :f1 - f0], pin[0:1, :f1 - f0], b1)
            h = lax.dot_general(xn, w1_s[f0:f1, :], NT, preferred_element_type=f32) + b1
            return gelu(h)

        def mm1_first(xn):
            return gelu(jnp.dot(xn, w1n_s[...], preferred_element_type=f32) + b1_row()[:, 0:128])

        def kv_fwd(j, sk, init=None):
            s = [jnp.broadcast_to(sk[l:l + 1, :], (8, 128)) for l in range(4)]
            dd = sk[4:5, :]
            fm = false_mask()
            lasts = [init] * kvn
            fwx = fw_ref[0]
            fwh = fw_ref[1]
            ev = lambda w: pltpu.bitcast(w << 16, f32)
            od = lambda w: pltpu.bitcast(w & jnp.uint32(0xffff0000), f32)
            kvs = []
            for a in range(NB + lag):
                if a < NB:
                    outs = []
                    for t in range(a * 8, a * 8 + 8):
                        bb = KP // 2 + 8 * t
                        w0 = ku_s[j, bb:bb + 8, :]
                        w1 = ku_s[j, bb - 1:bb + 7, :]
                        w2 = ku_s[j, bb - 2:bb + 6, :]
                        wv = vu_s[j, 8 * t:8 * t + 8, :]
                        e0, o0, e1, o1, o2 = ev(w0), od(w0), ev(w1), od(w1), od(w2)
                        ci = t % kvn
                        if lasts[ci] is not None:
                            e0 = jnp.where(fm, lasts[ci], e0)
                        oe = (e0 * s[0] + o1 * s[1] + e1 * s[2] + o2 * s[3]) * ev(wv)
                        oo = (e0 * s[1] + o0 * s[0] + o1 * s[2] + e1 * s[3]) * od(wv)
                        lasts[ci] = oo
                        outs += [oe, oo]
                    kvs.append(jnp.concatenate(outs, axis=0).astype(bf16))
                    hb = lax.dot_general(fwh, h_s[j, :, a * P:(a + 1) * P], NT, preferred_element_type=f32)
                    if a == 0:
                        hb = jnp.concatenate(
                            [hb[8 * t:8 * t + 8, :] + dd if t % 2 == 0 else hb[8 * t:8 * t + 8, :]
                             for t in range(32)], axis=0)
                    hf_s[a] = hb
                if a >= lag:
                    x_s[a - lag] = jnp.dot(fwx, kvs[a - lag], preferred_element_type=f32)

        def conv_mac(short):
            fm = false_mask()
            last = None
            Y = [[None] * 16 for _ in range(NB)]
            for p in range(16):
                r0, i0 = 16 * p, 16 * p + 8
                prev = None
                for c in range(NB):
                    accr = acci = pend = None
                    for a in range(c + 1):
                        b = c - a
                        xr = x_s[a, r0:r0 + 8, :]
                        xi = x_s[a, i0:i0 + 8, :]
                        hr = hf_s[b, r0:r0 + 8, :]
                        hi = hf_s[b, i0:i0 + 8, :]
                        if accr is None:
                            t1 = xr * hr
                            t2 = xr * hi
                            if last is not None:
                                t1 = jnp.where(fm, last[0], t1)
                                t2 = jnp.where(fm, last[1], t2)
                            accr = t1 - xi * hi
                            acci = t2 + xi * hr
                        elif short:
                            tr = xr * hr - xi * hi
                            ti = xr * hi + xi * hr
                            if pend is not None:
                                tr = tr + pend[0]
                                ti = ti + pend[1]
                                pend = None
                            elif a % mg == 1 and a < c:
                                pend = (tr, ti)
                                continue
                            accr = accr + tr
                            acci = acci + ti
                        else:
                            accr = (accr + xr * hr) - xi * hi
                            acci = (acci + xr * hi) + xi * hr
                    last = (accr, acci)
                    if prev is None:
                        yr, yi = accr, acci
                    else:
                        pr, pi = prev
                        yr, yi = (accr - pi, acci + pr) if p < 8 else (accr + pi, acci - pr)
                    prev = (accr, acci)
                    Y[c][p] = (yr, yi)
            return Y, last[0] + last[1]

        def conv_inv(j, Y):
            ic = inv_ref[0]
            isn = inv_ref[1]
            for c in range(NB):
                yr = jnp.concatenate([y[0] for y in Y[c]], axis=0).astype(bf16)
                yi = jnp.concatenate([y[1] for y in Y[c]], axis=0).astype(bf16)
                e = jnp.dot(ic, yr, preferred_element_type=f32)
                o = jnp.dot(isn, yi, preferred_element_type=f32)
                yp_s[j, c * P + 64:(c + 1) * P, :] = e - o
                lo = e + o
                for i in range(8):
                    yp_s[j, c * P + 8 * (7 - i):c * P + 8 * (8 - i), :] = lo[8 * i:8 * i + 8, :]

        def mlp_conv(i, short):
            r0 = M0 + i * M if isinstance(i, int) else pl.multiple_of(M0 + i * M, 64)
            Y, link = conv_mac(short)
            xn = load_xn(r0, M)
            h0 = mm1_first(xn)
            if short:
                ha = mm1(xn, 128, 128 * rpos)
                hr = mm1_rem(xn)
                h = jnp.concatenate([h0, ha, mm1(xn, 128 * rpos, FR), hr], axis=1)
            else:
                hr = mm1_rem(xn)
                h = jnp.concatenate([h0, mm1(xn, 128, FR), hr], axis=1)
            h = h.astype(bf16)
            b2 = b2_row()
            c4 = D - 128
            o = jnp.dot(h, w2_s[:, :c4], preferred_element_type=f32)
            p_s[pl.ds(r0, M), :c4] = o * OSC + (load_q(r0, M, 0, NL - 1) + b2[:, :c4])
            z = jnp.where(false_mask()[0:1, :], link[0:1, :], b2[:, c4:] * (1.0 / OSC))
            o = z + jnp.dot(h, w2_s[:, c4:], preferred_element_type=f32)
            p_s[pl.ds(r0, M), c4:] = o * OSC + load_q(r0, M, NL - 1, NL)
            conv_inv(i, Y)

        rev8 = 7 - row8

        def load_y(j, t):
            y = yp_s[j, t:t + 8, :]
            if t % P < 64:
                y = jnp.take_along_axis(y, rev8, axis=0)
            return y

        def combine(r0, r1, st):
            fm = false_mask()
            for t in range(r0, r1, 16):
                for j in range(NL):
                    cs = slice(j * 128, (j + 1) * 128)
                    y = jnp.concatenate([load_y(j, t), load_y(j, t + 8)], axis=0)
                    p0 = p_s[t:t + 8, cs]
                    if st[0] is not None:
                        p0 = jnp.where(fm, st[0], p0)
                    pp = jnp.concatenate([p0, p_s[t + 8:t + 16, cs]], axis=0)
                    r = (pp + xn_s[j, t:t + 16, :].astype(f32) * y).astype(bf16)
                    st[0] = r.astype(f32)[0:8, :]
                    o_s[j, t:t + 16, :] = r

        def first():
            wait(0)
            start(ring)
            ln(0, qa, False)
            wait(1)

            def r0a():
                start(1 + ring)
                bc_s[...] = jnp.broadcast_to(b1_row()[:, F - 128:F], (128, 128)).T[64:128, :]
                hid_s[0:qa, 0:w1c[1]] = mm1(load_xn(0, qa), 0, w1c[1]).astype(bf16)
            region(r0a)
            wait(2)

            def r0b():
                start(2 + ring)
                ln(qa, M0, False)
                hid_s[qa:M0, 0:w1c[1]] = mm1(load_xn(qa, M0 - qa), 0, w1c[1]).astype(bf16)
            region(r0b)
            for i in range(1, n1):
                wait(2 + i)

                def r1(i=i):
                    start(2 + i + ring)
                    if i == 1:
                        for j in range(NL):
                            w1n_s[j * 128:(j + 1) * 128, :] = (
                                w1_s[0:128, j * 128:(j + 1) * 128].astype(f32).T.astype(bf16))
                    hid_s[:, w1c[i]:w1c[i + 1]] = mm1(load_xn(0, M0), w1c[i], w1c[i + 1]).astype(bf16)
                region(r1)
            wait(ng - 4)

            def r2a():
                ln(M0, M0 + lns, True)
                p_s[0:M0, :] = jnp.dot(hid_s[:, :w2k], w2_s[:w2k, :], preferred_element_type=f32)
            region(r2a)
            wait(ng - 3)

            def r2b():
                lk = jnp.broadcast_to(ln(M0 + lns, S, True)[0:8, :], (8, 128))
                o = jnp.dot(hid_s[:, w2k:], w2_s[w2k:, :], preferred_element_type=f32) + p_s[0:M0, :]
                p_s[0:M0, :] = o * OSC + (load_q(0, M0) + b2_row())
                par = jnp.concatenate([sk_ref[...].astype(f32), dd_ref[...].astype(f32).reshape(1, D),
                                       jnp.zeros((3, D), f32)], axis=0)
                for j in range(NL):
                    par_s[j] = par[:, j * 128:(j + 1) * 128]
                kv_fwd(0, par[:, 0:128], lk)
            region(r2b)

        def pair(i, carry):
            si = lax.rem(ng - 2 + i, ring)
            for c in copies(kvh(2 * i + 1) + kvh(2 * i + 2), si):
                c.wait()
            mlp_conv(2 * i, False)
            kv_fwd(2 * i + 1, par_s[2 * i + 1])
            z = NB + flag_s[1]
            x_s[z, 0:8, :] = jnp.zeros((8, 128), f32)
            hf_s[z, 0:8, :] = jnp.zeros((8, 128), f32)
            mlp_conv(2 * i + 1, True)
            kv_fwd(2 * i + 2, par_s[2 * i + 2])
            return carry

        rl = S - ML

        def out_copies(js, r0, r1):
            return copies([(o_s.at[j, pl.ds(r0, r1 - r0), :], out_hbm.at[pl.ds(r0, r1 - r0), pl.ds(j * 128, 128)])
                           for j in js], sem_out)
        cuts = [0] + [int(rl // 16 * x) * 16 for x in prow] + [rl]
        g_o = [out_copies(range(NL), cuts[i], cuts[i + 1]) for i in range(nco)]
        g_fa = out_copies(range(osp), rl, S)
        g_fm = out_copies(range(osp, NL), rl, rl + rsp)
        g_fb = out_copies(range(osp, NL), rl + rsp, S)

        def pin_after(g, i):
            for c in g:
                c.start()
            z1 = pl.multiple_of(S + flag_s[1], 16)
            z2 = pl.multiple_of(S + flag_s[2], 16)
            o_s[0, pl.ds(z1, 16), :] = jnp.full((16, 128), i, bf16)
            return o_s[0, pl.ds(z2, 16), :].astype(f32)

        def last():
            mlp_conv(NL - 1, False)
            yp_s[NL + flag_s[1], 0:8, :] = jnp.zeros((8, 128), f32)
            p_s[pl.ds(pl.multiple_of(S + flag_s[1], 8), 8), 0:128] = jnp.zeros((8, 128), f32)
            xn = load_xn(rl, ML)
            st = [None]
            hs = []
            gi = 0
            for f in range(13):
                pin = None
                if gi < nco and pins[gi] == f:
                    combine(cuts[gi], cuts[gi + 1], st)
                    pin = pin_after(g_o[gi], gi)
                    gi += 1
                hs.append(mm1(xn, 128 * f, 128 * (f + 1), pin) if f else mm1_first(xn))
            hs.append(mm1_rem(xn))
            h = jnp.concatenate(hs, axis=1).astype(bf16)
            b2 = b2_row() * (1.0 / OSC)
            for j in range(NL):
                cs = slice(j * 128, (j + 1) * 128)
                bj = b2[:, cs]
                if gi < nco and pins[gi] == 14 + j:
                    combine(cuts[gi], cuts[gi + 1], st)
                    bj = jnp.where(false_mask()[0:1, :], pin_after(g_o[gi], gi)[0:1, :], bj)
                    gi += 1
                if j == osp:
                    bj = jnp.where(false_mask()[0:1, :], pin_after(g_fa, nco)[0:1, :], bj)
                for ra, rb in ([(rl, S)] if j < NL - 1 else [(rl, rl + rsp), (rl + rsp, S)]):
                    if ra > rl:
                        bj = jnp.where(false_mask()[0:1, :], pin_after(g_fm, nco + 1)[0:1, :], b2[:, cs])
                    o = (bj + jnp.dot(h[ra - rl:rb - rl, :], w2_s[:, cs], preferred_element_type=f32)) * OSC
                    o = o + load_q(ra, rb - ra, j, j + 1)
                    y = jnp.concatenate([load_y(j, t) for t in range(ra, rb, 8)], axis=0)
                    o_s[j, ra:rb, :] = (o + xn_s[j, ra:rb, :].astype(f32) * y).astype(bf16)
            assert gi == nco
        def it(i, carry):
            pl.when(i == 0)(first)
            pair(i, carry)
            pl.when(i == 1)(last)
            return carry
        lax.fori_loop(0, 2, it, 0)
        for c in g_fb:
            c.start()
        for g in g_o + [g_fa, g_fm, g_fb]:
            for c in g:
                c.wait()

    fw, inv = dft_mats()

    @jax.jit
    def f(q, k, v, sk, h, dd, w1, b1, w2, b2):
        any_ = pl.BlockSpec(memory_space=pl.ANY)
        out = pl.pallas_call(
            kernel,
            in_specs=[any_] * 12,
            out_specs=any_,
            out_shape=jax.ShapeDtypeStruct((S, D), bf16),
            scratch_shapes=[
                pltpu.VMEM((M0, D), bf16),
                pltpu.VMEM((NL, S, 128), bf16),
                pltpu.VMEM((NL, S + KP, 128), bf16),
                pltpu.VMEM((NL, S, 128), bf16),
                pltpu.VMEM((NL, 128, S), bf16),
                pltpu.VMEM((F, D), bf16),
                pltpu.VMEM((F, D), bf16),
                pltpu.VMEM((NL, S, 128), bf16),
                pltpu.VMEM((S + 8, D), f32),
                pltpu.VMEM((NB + 1, 256, 128), f32),
                pltpu.VMEM((NB + 1, 256, 128), f32),
                pltpu.VMEM((NL + 1, S, 128), f32),
                pltpu.VMEM((NL, S + 16, 128), bf16),
                pltpu.VMEM((NL, 8, 128), f32),
                pltpu.VMEM((M0, F), bf16),
                pltpu.VMEM((4, D), bf16), pltpu.VMEM((D,), bf16), pltpu.VMEM((F,), bf16), pltpu.VMEM((D,), bf16),
                pltpu.VMEM((2, 256, 128), bf16), pltpu.VMEM((2, 64, 128), bf16),
                pltpu.VMEM((64, 128), f32),
                pltpu.VMEM((D, 128), bf16),
                pltpu.SMEM((4,), jnp.int32),
                pltpu.SemaphoreType.DMA((ring,)),
            ],
            compiler_params=pltpu.CompilerParams(vmem_limit_bytes=100 * 2**20),
            name=name,
        )(q.reshape(S, D), k.reshape(S, D), v.reshape(S, D), sk.T, h, dd, w1.T, b1, w2, b2, fw, inv)
        return out.reshape(1, S, D)
    return f


_impl = make(name="fused_h3_mlp")


@jax.jit
def pallas_parallel_sum__ssm_conv_h3__dense_activation_gelu__prompt_kernel(
    A_q, A_k, A_v, A_shift_k, A_ssm_k, A_ssm_D, B_x, B_w1, B_b1, B_w2, B_b2,
):
    del B_x
    return _impl(A_q, A_k, A_v, A_shift_k, A_ssm_k, A_ssm_D, B_w1, B_b1, B_w2, B_b2)
```

```python
import numpy as np
import jax
import jax.numpy as jnp
from jax import lax
import jax.experimental.pallas as pl
import jax.experimental.pallas.tpu as pltpu

S, D, F = 2048, 640, 1728
P = 128
NB = S // P
NL = D // 128
KP = 64
FR = F - 64
f32, bf16, u32 = jnp.float32, jnp.bfloat16, jnp.uint32
NT = (((1,), (1,)), ((), ()))

ALPHA = (0.7978845608028654 * 0.044715) ** (1.0 / 3.0)
C1 = 0.7978845608028654 / ALPHA
OSC = 0.5 / ALPHA


def dft_mats():
    ks = np.concatenate([np.arange(0, 128, 2), np.arange(1, 128, 2)])
    n = np.arange(128)
    m = np.arange(64) + 0.5
    fw = np.zeros((2, 256, 128))
    inv = np.zeros((2, 64, 128))
    for p in range(16):
        for s in range(8):
            w = 2 * np.pi * (ks[8 * p + s] + 0.5) / 256
            fw[0, 16 * p + s] = np.cos(w * (n - 63.5))
            fw[0, 16 * p + 8 + s] = -np.sin(w * (n - 63.5))
            fw[1, 16 * p + s] = np.cos(w * n)
            fw[1, 16 * p + 8 + s] = -np.sin(w * n)
            inv[0, :, 8 * p + s] = np.cos(w * m) / (128 * ALPHA)
            inv[1, :, 8 * p + s] = np.sin(w * m) / (128 * ALPHA)
    perm = np.concatenate(
        [16 * t + np.concatenate([np.arange(0, 16, 2), np.arange(1, 16, 2)]) for t in range(8)])
    fw[0] = fw[0][:, perm]
    return fw.astype(np.float32).astype(bf16), inv.astype(np.float32).astype(bf16)


def gelu(g):
    return g * (1.0 + jnp.tanh(g * (C1 + g * g)))


def make(M0=576, M=256, name="v51", kvn=2, qa=256, w1c=(0, 256, 768, F), w2k=1024, lns=960,
         pins=(2, 7, 12, 15), prow=(0.01, 0.28, 0.6), osp=4, lag=4, mg=3, ring=4, rpos=4, rsp=96, lnfree=True):
    ML = S - M0 - NL * M
    assert ML > 0 and ML % 16 == 0 and M0 % 64 == 0 and M % 64 == 0
    n1, nco = len(w1c) - 1, len(pins)

    def kernel(q_hbm, k_hbm, v_hbm, sk_hbm, h_hbm, dd_hbm, w1_hbm, b1_hbm, w2_hbm, b2_hbm, fw_hbm, inv_hbm,
               out_hbm,
               q_s, ql_s, k_s, v_s, h_s, w1_s, w2_s, xn_s, p_s, x_s, hf_s, yp_s, o_s, par_s, hid_s,
               sk_ref, dd_ref, b1_ref, b2_ref, fw_ref, inv_ref, bc_s, w1n_s, flag_s, sem):
        def rows(src, dst, r0, r1):
            return (src.at[pl.ds(r0, r1 - r0)], dst.at[pl.ds(r0, r1 - r0)])

        def qrows(r0, r1):
            return [(q_hbm.at[pl.ds(r0, r1 - r0), pl.ds(j * 128, 128)], ql_s.at[j, pl.ds(r0, r1 - r0), :])
                    for j in range(NL)]

        def load_q(r0, m, j0=0, j1=NL):
            if isinstance(r0, int) and r0 < M0:
                return q_s[r0:r0 + m, j0 * 128:j1 * 128].astype(f32)
            return jnp.concatenate([ql_s[j, pl.ds(r0, m), :].astype(f32) for j in range(j0, j1)], axis=1)

        def kvh(j):
            lane = pl.ds(j * 128, 128) if isinstance(j, int) else pl.ds(pl.multiple_of(j * 128, 128), 128)
            return [(h_hbm.at[lane, :], h_s.at[j]),
                    (k_hbm.at[:, lane], k_s.at[j, pl.ds(KP, S), :]),
                    (v_hbm.at[:, lane], v_s.at[j])]

        def copies(g, si):
            return [pltpu.make_async_copy(src, dst, sem.at[si]) for src, dst in g]

        groups = [[rows(q_hbm, q_s, 0, qa)],
                  [rows(w1_hbm, w1_s, 0, w1c[1]), (b1_hbm, b1_ref)],
                  [rows(q_hbm, q_s, qa, M0)]]
        groups += [[rows(w1_hbm, w1_s, w1c[i], w1c[i + 1])] for i in range(1, n1)]
        groups += [qrows(M0, M0 + lns) + [rows(w2_hbm, w2_s, 0, w2k)],
                   qrows(M0 + lns, S) + [rows(w2_hbm, w2_s, w2k, F), (b2_hbm, b2_ref), (sk_hbm, sk_ref),
                                         (dd_hbm, dd_ref), (fw_hbm, fw_ref), (inv_hbm, inv_ref)] + kvh(0),
                   kvh(1) + kvh(2), kvh(3) + kvh(4)]
        ng = len(groups)
        sem_out = (ng - 3) % ring

        def start(g):
            if g < ng:
                for c in copies(groups[g], g % ring):
                    c.start()

        def wait(g):
            for c in copies(groups[g], g % ring):
                c.wait()

        for g in range(ring):
            start(g)

        flag_s[0] = 100
        flag_s[1] = 0
        flag_s[2] = 0
        for j in range(NL):
            k_s[j, KP - 16:KP, :] = jnp.zeros((16, 128), bf16)
        ku_s = k_s.bitcast(u32)
        vu_s = v_s.bitcast(u32)

        def region(fn):
            pl.when(flag_s[0] == 100)(fn)

        row8 = lax.broadcasted_iota(jnp.int32, (8, 128), 0)

        def false_mask():
            return row8 > flag_s[0]

        def ln(r0, r1, chain, stats=None):
            fm = lax.broadcasted_iota(jnp.int32, (16, 1), 0) > flag_s[0]
            rs = None
            for rr in range(r0, r1, 16):
                x = load_q(rr, 16)
                mu = jnp.sum(x, axis=-1, keepdims=True) * (1.0 / D)
                xc = x - mu
                var = jnp.sum(xc * xc, axis=-1, keepdims=True) * (1.0 / D)
                if chain and rs is not None:
                    var = jnp.where(fm, rs, var)
                rs = lax.rsqrt(var + 1e-5) * ALPHA
                if stats is not None:
                    stats.append((mu, rs))
                xo = xc * rs
                for j in range(NL):
                    xn_s[j, rr:rr + 16, :] = xo[:, j * 128:(j + 1) * 128].astype(bf16)
            return rs

        def load_xn(r0, m):
            return jnp.concatenate([xn_s[j, pl.ds(r0, m), :] for j in range(NL)], axis=1)

        def b1_row():
            return b1_ref[...].astype(f32).reshape(1, F) * ALPHA

        def b2_row():
            return b2_ref[...].astype(f32).reshape(1, D)

        def mm1_rem(xn):
            m = xn.shape[0]
            ht = lax.dot_general(w1_s[FR:F, :], xn, NT, preferred_element_type=f32)
            bc = bc_s[...]
            outs = []
            for c0 in range(0, m, 128):
                c1 = min(c0 + 128, m)
                outs.append(gelu(ht[:, c0:c1] + bc[:, :c1 - c0]).T)
            return jnp.concatenate(outs, axis=0)

        def mm1(xn, f0=0, f1=F, pin=None):
            if f1 == F:
                hr = mm1_rem(xn)
                if f0 == FR:
                    return hr
                return jnp.concatenate([mm1(xn, f0, FR, pin), hr], axis=1)
            b1 = b1_row()[:, f0:f1]
            if pin is not None:
                b1 = jnp.where(false_mask()[0:1, :f1 - f0], pin[0:1, :f1 - f0], b1)
            h = lax.dot_general(xn, w1_s[f0:f1, :], NT, preferred_element_type=f32) + b1
            return gelu(h)

        def mm1_first(xn):
            return gelu(jnp.dot(xn, w1n_s[...], preferred_element_type=f32) + b1_row()[:, 0:128])

        def kv_fwd(j, sk, init=None):
            s = [jnp.broadcast_to(sk[l:l + 1, :], (8, 128)) for l in range(4)]
            dd = sk[4:5, :]
            fm = false_mask()
            lasts = [init] * kvn
            fwx = fw_ref[0]
            fwh = fw_ref[1]
            ev = lambda w: pltpu.bitcast(w << 16, f32)
            od = lambda w: pltpu.bitcast(w & jnp.uint32(0xffff0000), f32)
            kvs = []
            for a in range(NB + lag):
                if a < NB:
                    outs = []
                    for t in range(a * 8, a * 8 + 8):
                        bb = KP // 2 + 8 * t
                        w0 = ku_s[j, bb:bb + 8, :]
                        w1 = ku_s[j, bb - 1:bb + 7, :]
                        w2 = ku_s[j, bb - 2:bb + 6, :]
                        wv = vu_s[j, 8 * t:8 * t + 8, :]
                        e0, o0, e1, o1, o2 = ev(w0), od(w0), ev(w1), od(w1), od(w2)
                        ci = t % kvn
                        if lasts[ci] is not None:
                            e0 = jnp.where(fm, lasts[ci], e0)
                        oe = (e0 * s[0] + o1 * s[1] + e1 * s[2] + o2 * s[3]) * ev(wv)
                        oo = (e0 * s[1] + o0 * s[0] + o1 * s[2] + e1 * s[3]) * od(wv)
                        lasts[ci] = oo
                        outs += [oe, oo]
                    kvs.append(jnp.concatenate(outs, axis=0).astype(bf16))
                    hb = lax.dot_general(fwh, h_s[j, :, a * P:(a + 1) * P], NT, preferred_element_type=f32)
                    if a == 0:
                        hb = jnp.concatenate(
                            [hb[8 * t:8 * t + 8, :] + dd if t % 2 == 0 else hb[8 * t:8 * t + 8, :]
                             for t in range(32)], axis=0)
                    hf_s[a] = hb
                if a >= lag:
                    x_s[a - lag] = jnp.dot(fwx, kvs[a - lag], preferred_element_type=f32)

        def conv_mac(short):
            fm = false_mask()
            last = None
            Y = [[None] * 16 for _ in range(NB)]
            for p in range(16):
                r0, i0 = 16 * p, 16 * p + 8
                prev = None
                for c in range(NB):
                    accr = acci = pend = None
                    for a in range(c + 1):
                        b = c - a
                        xr = x_s[a, r0:r0 + 8, :]
                        xi = x_s[a, i0:i0 + 8, :]
                        hr = hf_s[b, r0:r0 + 8, :]
                        hi = hf_s[b, i0:i0 + 8, :]
                        if accr is None:
                            t1 = xr * hr
                            t2 = xr * hi
                            if last is not None:
                                t1 = jnp.where(fm, last[0], t1)
                                t2 = jnp.where(fm, last[1], t2)
                            accr = t1 - xi * hi
                            acci = t2 + xi * hr
                        elif short:
                            tr = xr * hr - xi * hi
                            ti = xr * hi + xi * hr
                            if pend is not None:
                                tr = tr + pend[0]
                                ti = ti + pend[1]
                                pend = None
                            elif a % mg == 1 and a < c:
                                pend = (tr, ti)
                                continue
                            accr = accr + tr
                            acci = acci + ti
                        else:
                            accr = (accr + xr * hr) - xi * hi
                            acci = (acci + xr * hi) + xi * hr
                    last = (accr, acci)
                    if prev is None:
                        yr, yi = accr, acci
                    else:
                        pr, pi = prev
                        yr, yi = (accr - pi, acci + pr) if p < 8 else (accr + pi, acci - pr)
                    prev = (accr, acci)
                    Y[c][p] = (yr, yi)
            return Y, last[0] + last[1]

        def conv_inv(j, Y):
            ic = inv_ref[0]
            isn = inv_ref[1]
            for c in range(NB):
                yr = jnp.concatenate([y[0] for y in Y[c]], axis=0).astype(bf16)
                yi = jnp.concatenate([y[1] for y in Y[c]], axis=0).astype(bf16)
                e = jnp.dot(ic, yr, preferred_element_type=f32)
                o = jnp.dot(isn, yi, preferred_element_type=f32)
                yp_s[j, c * P + 64:(c + 1) * P, :] = e - o
                lo = e + o
                for i in range(8):
                    yp_s[j, c * P + 8 * (7 - i):c * P + 8 * (8 - i), :] = lo[8 * i:8 * i + 8, :]

        def mlp_conv(i, short):
            r0 = M0 + i * M if isinstance(i, int) else pl.multiple_of(M0 + i * M, 64)
            Y, link = conv_mac(short)
            xn = load_xn(r0, M)
            h0 = mm1_first(xn)
            if short:
                ha = mm1(xn, 128, 128 * rpos)
                hr = mm1_rem(xn)
                h = jnp.concatenate([h0, ha, mm1(xn, 128 * rpos, FR), hr], axis=1)
            else:
                hr = mm1_rem(xn)
                h = jnp.concatenate([h0, mm1(xn, 128, FR), hr], axis=1)
            h = h.astype(bf16)
            b2 = b2_row()
            c4 = D - 128
            o = jnp.dot(h, w2_s[:, :c4], preferred_element_type=f32)
            p_s[pl.ds(r0, M), :c4] = o * OSC + (load_q(r0, M, 0, NL - 1) + b2[:, :c4])
            z = jnp.where(false_mask()[0:1, :], link[0:1, :], b2[:, c4:] * (1.0 / OSC))
            o = z + jnp.dot(h, w2_s[:, c4:], preferred_element_type=f32)
            p_s[pl.ds(r0, M), c4:] = o * OSC + load_q(r0, M, NL - 1, NL)
            conv_inv(i, Y)

        rev8 = 7 - row8

        def load_y(j, t):
            y = yp_s[j, t:t + 8, :]
            if t % P < 64:
                y = jnp.take_along_axis(y, rev8, axis=0)
            return y

        def combine(r0, r1, st):
            fm = false_mask()
            for t in range(r0, r1, 16):
                for j in range(NL):
                    cs = slice(j * 128, (j + 1) * 128)
                    y = jnp.concatenate([load_y(j, t), load_y(j, t + 8)], axis=0)
                    p0 = p_s[t:t + 8, cs]
                    if st[0] is not None:
                        p0 = jnp.where(fm, st[0], p0)
                    pp = jnp.concatenate([p0, p_s[t + 8:t + 16, cs]], axis=0)
                    r = (pp + xn_s[j, t:t + 16, :].astype(f32) * y).astype(bf16)
                    st[0] = r.astype(f32)[0:8, :]
                    o_s[j, t:t + 16, :] = r

        def first():
            wait(0)
            start(ring)
            ln(0, qa, False)
            wait(1)

            def r0a():
                start(1 + ring)
                bc_s[...] = jnp.broadcast_to(b1_row()[:, F - 128:F], (128, 128)).T[64:128, :]
                hid_s[0:qa, 0:w1c[1]] = mm1(load_xn(0, qa), 0, w1c[1]).astype(bf16)
            region(r0a)
            wait(2)

            def r0b():
                start(2 + ring)
                if not lnfree:
                    ln(qa, M0, False)
                    hid_s[qa:M0, 0:w1c[1]] = mm1(load_xn(qa, M0 - qa), 0, w1c[1]).astype(bf16)
                    return
                st = []
                ln(qa, M0, False, st)
                mu = jnp.concatenate([a_ for a_, _ in st], axis=0)
                rs = jnp.concatenate([b_ for _, b_ in st], axis=0)
                lhs = jnp.concatenate([jnp.ones((16, D), bf16), q_s[qa:M0, :]], axis=0)
                z = lax.dot_general(lhs, w1_s[0:w1c[1], :], NT, preferred_element_type=f32)
                g = (z[16:, :] - mu * z[0:1, :]) * rs + b1_row()[:, 0:w1c[1]]
                hid_s[qa:M0, 0:w1c[1]] = gelu(g).astype(bf16)
            region(r0b)
            for i in range(1, n1):
                wait(2 + i)

                def r1(i=i):
                    start(2 + i + ring)
                    if i == 1:
                        for j in range(NL):
                            w1n_s[j * 128:(j + 1) * 128, :] = (
                                w1_s[0:128, j * 128:(j + 1) * 128].astype(f32).T.astype(bf16))
                    hid_s[:, w1c[i]:w1c[i + 1]] = mm1(load_xn(0, M0), w1c[i], w1c[i + 1]).astype(bf16)
                region(r1)
            wait(ng - 4)

            def r2a():
                start(ng - 4 + ring)
                ln(M0, M0 + lns, True)
                p_s[0:M0, :] = jnp.dot(hid_s[:, :w2k], w2_s[:w2k, :], preferred_element_type=f32)
            region(r2a)
            wait(ng - 3)

            def r2b():
                lk = jnp.broadcast_to(ln(M0 + lns, S, True)[0:8, :], (8, 128))
                o = jnp.dot(hid_s[:, w2k:], w2_s[w2k:, :], preferred_element_type=f32) + p_s[0:M0, :]
                p_s[0:M0, :] = o * OSC + (load_q(0, M0) + b2_row())
                par = jnp.concatenate([sk_ref[...].astype(f32), dd_ref[...].astype(f32).reshape(1, D),
                                       jnp.zeros((3, D), f32)], axis=0)
                for j in range(NL):
                    par_s[j] = par[:, j * 128:(j + 1) * 128]
                kv_fwd(0, par[:, 0:128], lk)
            region(r2b)

        def pair(i, carry):
            si = lax.rem(ng - 2 + i, ring)
            for c in copies(kvh(2 * i + 1) + kvh(2 * i + 2), si):
                c.wait()
            mlp_conv(2 * i, False)
            kv_fwd(2 * i + 1, par_s[2 * i + 1])
            z = NB + flag_s[1]
            x_s[z, 0:8, :] = jnp.zeros((8, 128), f32)
            hf_s[z, 0:8, :] = jnp.zeros((8, 128), f32)
            mlp_conv(2 * i + 1, True)
            kv_fwd(2 * i + 2, par_s[2 * i + 2])
            return carry

        rl = S - ML

        def out_copies(js, r0, r1):
            return copies([(o_s.at[j, pl.ds(r0, r1 - r0), :], out_hbm.at[pl.ds(r0, r1 - r0), pl.ds(j * 128, 128)])
                           for j in js], sem_out)
        cuts = [0] + [int(rl // 16 * x) * 16 for x in prow] + [rl]
        g_o = [out_copies(range(NL), cuts[i], cuts[i + 1]) for i in range(nco)]
        g_fa = out_copies(range(osp), rl, S)
        g_fm = out_copies(range(osp, NL), rl, rl + rsp)
        g_fb = out_copies(range(osp, NL), rl + rsp, S)

        def pin_after(g, i):
            for c in g:
                c.start()
            z1 = pl.multiple_of(S + flag_s[1], 16)
            z2 = pl.multiple_of(S + flag_s[2], 16)
            o_s[0, pl.ds(z1, 16), :] = jnp.full((16, 128), i, bf16)
            return o_s[0, pl.ds(z2, 16), :].astype(f32)

        def last():
            mlp_conv(NL - 1, False)
            yp_s[NL + flag_s[1], 0:8, :] = jnp.zeros((8, 128), f32)
            p_s[pl.ds(pl.multiple_of(S + flag_s[1], 8), 8), 0:128] = jnp.zeros((8, 128), f32)
            xn = load_xn(rl, ML)
            st = [None]
            hs = []
            gi = 0
            for f in range(13):
                pin = None
                if gi < nco and pins[gi] == f:
                    combine(cuts[gi], cuts[gi + 1], st)
                    pin = pin_after(g_o[gi], gi)
                    gi += 1
                hs.append(mm1(xn, 128 * f, 128 * (f + 1), pin) if f else mm1_first(xn))
            hs.append(mm1_rem(xn))
            h = jnp.concatenate(hs, axis=1).astype(bf16)
            b2 = b2_row() * (1.0 / OSC)
            for j in range(NL):
                cs = slice(j * 128, (j + 1) * 128)
                bj = b2[:, cs]
                if gi < nco and pins[gi] == 14 + j:
                    combine(cuts[gi], cuts[gi + 1], st)
                    bj = jnp.where(false_mask()[0:1, :], pin_after(g_o[gi], gi)[0:1, :], bj)
                    gi += 1
                if j == osp:
                    bj = jnp.where(false_mask()[0:1, :], pin_after(g_fa, nco)[0:1, :], bj)
                for ra, rb in ([(rl, S)] if j < NL - 1 else [(rl, rl + rsp), (rl + rsp, S)]):
                    if ra > rl:
                        bj = jnp.where(false_mask()[0:1, :], pin_after(g_fm, nco + 1)[0:1, :], b2[:, cs])
                    o = (bj + jnp.dot(h[ra - rl:rb - rl, :], w2_s[:, cs], preferred_element_type=f32)) * OSC
                    o = o + load_q(ra, rb - ra, j, j + 1)
                    y = jnp.concatenate([load_y(j, t) for t in range(ra, rb, 8)], axis=0)
                    o_s[j, ra:rb, :] = (o + xn_s[j, ra:rb, :].astype(f32) * y).astype(bf16)
            assert gi == nco
        def it(i, carry):
            pl.when(i == 0)(first)
            pair(i, carry)
            pl.when(i == 1)(last)
            return carry
        lax.fori_loop(0, 2, it, 0)
        for c in g_fb:
            c.start()
        for g in g_o + [g_fa, g_fm, g_fb]:
            for c in g:
                c.wait()

    fw, inv = dft_mats()

    @jax.jit
    def f(q, k, v, sk, h, dd, w1, b1, w2, b2):
        any_ = pl.BlockSpec(memory_space=pl.ANY)
        out = pl.pallas_call(
            kernel,
            in_specs=[any_] * 12,
            out_specs=any_,
            out_shape=jax.ShapeDtypeStruct((S, D), bf16),
            scratch_shapes=[
                pltpu.VMEM((M0, D), bf16),
                pltpu.VMEM((NL, S, 128), bf16),
                pltpu.VMEM((NL, S + KP, 128), bf16),
                pltpu.VMEM((NL, S, 128), bf16),
                pltpu.VMEM((NL, 128, S), bf16),
                pltpu.VMEM((F, D), bf16),
                pltpu.VMEM((F, D), bf16),
                pltpu.VMEM((NL, S, 128), bf16),
                pltpu.VMEM((S + 8, D), f32),
                pltpu.VMEM((NB + 1, 256, 128), f32),
                pltpu.VMEM((NB + 1, 256, 128), f32),
                pltpu.VMEM((NL + 1, S, 128), f32),
                pltpu.VMEM((NL, S + 16, 128), bf16),
                pltpu.VMEM((NL, 8, 128), f32),
                pltpu.VMEM((M0, F), bf16),
                pltpu.VMEM((4, D), bf16), pltpu.VMEM((D,), bf16), pltpu.VMEM((F,), bf16), pltpu.VMEM((D,), bf16),
                pltpu.VMEM((2, 256, 128), bf16), pltpu.VMEM((2, 64, 128), bf16),
                pltpu.VMEM((64, 128), f32),
                pltpu.VMEM((D, 128), bf16),
                pltpu.SMEM((4,), jnp.int32),
                pltpu.SemaphoreType.DMA((ring,)),
            ],
            compiler_params=pltpu.CompilerParams(vmem_limit_bytes=100 * 2**20),
            name=name,
        )(q.reshape(S, D), k.reshape(S, D), v.reshape(S, D), sk.T, h, dd, w1.T, b1, w2, b2, fw, inv)
        return out.reshape(1, S, D)
    return f


_impl = make(name="fused_h3_mlp")


@jax.jit
def pallas_parallel_sum__ssm_conv_h3__dense_activation_gelu__prompt_kernel(
    A_q, A_k, A_v, A_shift_k, A_ssm_k, A_ssm_D, B_x, B_w1, B_b1, B_w2, B_b2,
):
    del B_x
    return _impl(A_q, A_k, A_v, A_shift_k, A_ssm_k, A_ssm_D, B_w1, B_b1, B_w2, B_b2)
```

```python
import numpy as np
import jax
import jax.numpy as jnp
from jax import lax
import jax.experimental.pallas as pl
import jax.experimental.pallas.tpu as pltpu

S, D, F = 2048, 640, 1728
P = 128
NB = S // P
NL = D // 128
KP = 64
FR = F - 64
f32, bf16, u32 = jnp.float32, jnp.bfloat16, jnp.uint32
NT = (((1,), (1,)), ((), ()))

ALPHA = (0.7978845608028654 * 0.044715) ** (1.0 / 3.0)
C1 = 0.7978845608028654 / ALPHA
OSC = 0.5 / ALPHA


def dft_mats():
    ks = np.concatenate([np.arange(0, 128, 2), np.arange(1, 128, 2)])
    n = np.arange(128)
    m = np.arange(64) + 0.5
    fw = np.zeros((2, 256, 128))
    inv = np.zeros((2, 64, 128))
    for p in range(16):
        for s in range(8):
            w = 2 * np.pi * (ks[8 * p + s] + 0.5) / 256
            fw[0, 16 * p + s] = np.cos(w * (n - 63.5))
            fw[0, 16 * p + 8 + s] = -np.sin(w * (n - 63.5))
            fw[1, 16 * p + s] = np.cos(w * n)
            fw[1, 16 * p + 8 + s] = -np.sin(w * n)
            inv[0, :, 8 * p + s] = np.cos(w * m) / (128 * ALPHA)
            inv[1, :, 8 * p + s] = np.sin(w * m) / (128 * ALPHA)
    perm = np.concatenate(
        [16 * t + np.concatenate([np.arange(0, 16, 2), np.arange(1, 16, 2)]) for t in range(8)])
    fw[0] = fw[0][:, perm]
    return fw.astype(np.float32).astype(bf16), inv.astype(np.float32).astype(bf16)


def gelu(g):
    return g * (1.0 + jnp.tanh(g * (C1 + g * g)))


def make(M0=576, M=256, name="v52", kvn=2, qa=256, w1c=(0, 256, 768, F), w2k=1024, lns=960,
         pins=(2, 7, 12, 15), prow=(0.01, 0.28, 0.6), osp=4, lag=4, mg=3, ring=4, rpos=4, rsp=96):
    ML = S - M0 - NL * M
    assert ML > 0 and ML % 16 == 0 and M0 % 64 == 0 and M % 64 == 0
    n1, nco = len(w1c) - 1, len(pins)

    def kernel(q_hbm, k_hbm, v_hbm, sk_hbm, h_hbm, dd_hbm, w1_hbm, b1_hbm, w2_hbm, b2_hbm, fw_hbm, inv_hbm,
               out_hbm,
               q_s, ql_s, k_s, v_s, h_s, w1_s, w2_s, xn_s, p_s, x_s, hf_s, yp_s, o_s, par_s, hid_s,
               sk_ref, dd_ref, b1_ref, b2_ref, fw_ref, inv_ref, bc_s, w1n_s, flag_s, sem):
        def rows(src, dst, r0, r1):
            return (src.at[pl.ds(r0, r1 - r0)], dst.at[pl.ds(r0, r1 - r0)])

        def qrows(r0, r1):
            return [(q_hbm.at[pl.ds(r0, r1 - r0), pl.ds(j * 128, 128)], ql_s.at[j, pl.ds(r0, r1 - r0), :])
                    for j in range(NL)]

        def load_q(r0, m, j0=0, j1=NL):
            if isinstance(r0, int) and r0 < M0:
                return q_s[r0:r0 + m, j0 * 128:j1 * 128].astype(f32)
            return jnp.concatenate([ql_s[j, pl.ds(r0, m), :].astype(f32) for j in range(j0, j1)], axis=1)

        def kvh(j):
            lane = pl.ds(j * 128, 128) if isinstance(j, int) else pl.ds(pl.multiple_of(j * 128, 128), 128)
            return [(h_hbm.at[lane, :], h_s.at[j]),
                    (k_hbm.at[:, lane], k_s.at[j, pl.ds(KP, S), :]),
                    (v_hbm.at[:, lane], v_s.at[j])]

        def copies(g, si):
            return [pltpu.make_async_copy(src, dst, sem.at[si]) for src, dst in g]

        groups = [[rows(q_hbm, q_s, 0, qa)],
                  [rows(w1_hbm, w1_s, 0, w1c[1]), (b1_hbm, b1_ref)],
                  [rows(q_hbm, q_s, qa, M0)]]
        groups += [[rows(w1_hbm, w1_s, w1c[i], w1c[i + 1])] for i in range(1, n1)]
        groups += [qrows(M0, M0 + lns) + [rows(w2_hbm, w2_s, 0, w2k)],
                   qrows(M0 + lns, S) + [rows(w2_hbm, w2_s, w2k, F), (b2_hbm, b2_ref), (sk_hbm, sk_ref),
                                         (dd_hbm, dd_ref), (fw_hbm, fw_ref), (inv_hbm, inv_ref)] + kvh(0),
                   kvh(1) + kvh(2), kvh(3) + kvh(4)]
        ng = len(groups)
        sem_out = (ng - 3) % ring

        def start(g):
            if g < ng:
                for c in copies(groups[g], g % ring):
                    c.start()

        def wait(g):
            for c in copies(groups[g], g % ring):
                c.wait()

        for g in range(ring):
            start(g)

        flag_s[0] = 100
        flag_s[1] = 0
        flag_s[2] = 0
        for j in range(NL):
            k_s[j, KP - 16:KP, :] = jnp.zeros((16, 128), bf16)
        ku_s = k_s.bitcast(u32)
        vu_s = v_s.bitcast(u32)

        def region(fn):
            pl.when(flag_s[0] == 100)(fn)

        row8 = lax.broadcasted_iota(jnp.int32, (8, 128), 0)

        def false_mask():
            return row8 > flag_s[0]

        def ln(r0, r1, chain, stats=None):
            fm = lax.broadcasted_iota(jnp.int32, (16, 1), 0) > flag_s[0]
            rs = None
            for rr in range(r0, r1, 16):
                x = load_q(rr, 16)
                mu = jnp.sum(x, axis=-1, keepdims=True) * (1.0 / D)
                xc = x - mu
                var = jnp.sum(xc * xc, axis=-1, keepdims=True) * (1.0 / D)
                if chain and rs is not None:
                    var = jnp.where(fm, rs, var)
                rs = lax.rsqrt(var + 1e-5) * ALPHA
                if stats is not None:
                    stats.append((mu, rs))
                xo = xc * rs
                for j in range(NL):
                    xn_s[j, rr:rr + 16, :] = xo[:, j * 128:(j + 1) * 128].astype(bf16)
            return rs

        def load_xn(r0, m):
            return jnp.concatenate([xn_s[j, pl.ds(r0, m), :] for j in range(NL)], axis=1)

        def b1_row():
            return b1_ref[...].astype(f32).reshape(1, F) * ALPHA

        def b2_row():
            return b2_ref[...].astype(f32).reshape(1, D)

        def mm1_rem(xn):
            m = xn.shape[0]
            ht = lax.dot_general(w1_s[FR:F, :], xn, NT, preferred_element_type=f32)
            bc = bc_s[...]
            outs = []
            for c0 in range(0, m, 128):
                c1 = min(c0 + 128, m)
                outs.append(gelu(ht[:, c0:c1] + bc[:, :c1 - c0]).T)
            return jnp.concatenate(outs, axis=0)

        def mm1(xn, f0=0, f1=F, pin=None):
            if f1 == F:
                hr = mm1_rem(xn)
                if f0 == FR:
                    return hr
                return jnp.concatenate([mm1(xn, f0, FR, pin), hr], axis=1)
            b1 = b1_row()[:, f0:f1]
            if pin is not None:
                b1 = jnp.where(false_mask()[0:1, :f1 - f0], pin[0:1, :f1 - f0], b1)
            h = lax.dot_general(xn, w1_s[f0:f1, :], NT, preferred_element_type=f32) + b1
            return gelu(h)

        def mm1_first(xn):
            return gelu(jnp.dot(xn, w1n_s[...], preferred_element_type=f32) + b1_row()[:, 0:128])

        def kv_fwd(j, sk, init=None):
            s = [jnp.broadcast_to(sk[l:l + 1, :], (8, 128)) for l in range(4)]
            dd = sk[4:5, :]
            fm = false_mask()
            lasts = [init] * kvn
            fwx = fw_ref[0]
            fwh = fw_ref[1]
            ev = lambda w: pltpu.bitcast(w << 16, f32)
            od = lambda w: pltpu.bitcast(w & jnp.uint32(0xffff0000), f32)
            kvs = []
            for a in range(NB + lag):
                if a < NB:
                    outs = []
                    for t in range(a * 8, a * 8 + 8):
                        bb = KP // 2 + 8 * t
                        w0 = ku_s[j, bb:bb + 8, :]
                        w1 = ku_s[j, bb - 1:bb + 7, :]
                        w2 = ku_s[j, bb - 2:bb + 6, :]
                        wv = vu_s[j, 8 * t:8 * t + 8, :]
                        e0, o0, e1, o1, o2 = ev(w0), od(w0), ev(w1), od(w1), od(w2)
                        ci = t % kvn
                        if lasts[ci] is not None:
                            e0 = jnp.where(fm, lasts[ci], e0)
                        oe = (e0 * s[0] + o1 * s[1] + e1 * s[2] + o2 * s[3]) * ev(wv)
                        oo = (e0 * s[1] + o0 * s[0] + o1 * s[2] + e1 * s[3]) * od(wv)
                        lasts[ci] = oo
                        outs += [oe, oo]
                    kvs.append(jnp.concatenate(outs, axis=0).astype(bf16))
                    hb = lax.dot_general(fwh, h_s[j, :, a * P:(a + 1) * P], NT, preferred_element_type=f32)
                    if a == 0:
                        hb = jnp.concatenate(
                            [hb[8 * t:8 * t + 8, :] + dd if t % 2 == 0 else hb[8 * t:8 * t + 8, :]
                             for t in range(32)], axis=0)
                    hf_s[a] = hb
                if a >= lag:
                    x_s[a - lag] = jnp.dot(fwx, kvs[a - lag], preferred_element_type=f32)

        def conv_mac(short):
            fm = false_mask()
            last = None
            Y = [[None] * 16 for _ in range(NB)]
            for p in range(16):
                r0, i0 = 16 * p, 16 * p + 8
                prev = None
                for c in range(NB):
                    accr = acci = pend = None
                    for a in range(c + 1):
                        b = c - a
                        xr = x_s[a, r0:r0 + 8, :]
                        xi = x_s[a, i0:i0 + 8, :]
                        hr = hf_s[b, r0:r0 + 8, :]
                        hi = hf_s[b, i0:i0 + 8, :]
                        if accr is None:
                            t1 = xr * hr
                            t2 = xr * hi
                            if last is not None:
                                t1 = jnp.where(fm, last[0], t1)
                                t2 = jnp.where(fm, last[1], t2)
                            accr = t1 - xi * hi
                            acci = t2 + xi * hr
                        elif short:
                            tr = xr * hr - xi * hi
                            ti = xr * hi + xi * hr
                            if pend is not None:
                                tr = tr + pend[0]
                                ti = ti + pend[1]
                                pend = None
                            elif a % mg == 1 and a < c:
                                pend = (tr, ti)
                                continue
                            accr = accr + tr
                            acci = acci + ti
                        else:
                            accr = (accr + xr * hr) - xi * hi
                            acci = (acci + xr * hi) + xi * hr
                    last = (accr, acci)
                    if prev is None:
                        yr, yi = accr, acci
                    else:
                        pr, pi = prev
                        yr, yi = (accr - pi, acci + pr) if p < 8 else (accr + pi, acci - pr)
                    prev = (accr, acci)
                    Y[c][p] = (yr, yi)
            return Y, last[0] + last[1]

        def conv_inv(j, Y):
            ic = inv_ref[0]
            isn = inv_ref[1]
            for c in range(NB):
                yr = jnp.concatenate([y[0] for y in Y[c]], axis=0).astype(bf16)
                yi = jnp.concatenate([y[1] for y in Y[c]], axis=0).astype(bf16)
                e = jnp.dot(ic, yr, preferred_element_type=f32)
                o = jnp.dot(isn, yi, preferred_element_type=f32)
                yp_s[j, c * P + 64:(c + 1) * P, :] = e - o
                lo = e + o
                for i in range(8):
                    yp_s[j, c * P + 8 * (7 - i):c * P + 8 * (8 - i), :] = lo[8 * i:8 * i + 8, :]

        def mlp_conv(i, short):
            r0 = M0 + i * M if isinstance(i, int) else pl.multiple_of(M0 + i * M, 64)
            Y, link = conv_mac(short)
            xn = load_xn(r0, M)
            h0 = mm1_first(xn)
            if short:
                ha = mm1(xn, 128, 128 * rpos)
                hr = mm1_rem(xn)
                h = jnp.concatenate([h0, ha, mm1(xn, 128 * rpos, FR), hr], axis=1)
            else:
                hr = mm1_rem(xn)
                h = jnp.concatenate([h0, mm1(xn, 128, FR), hr], axis=1)
            h = h.astype(bf16)
            b2 = b2_row()
            c4 = D - 128
            o = jnp.dot(h, w2_s[:, :c4], preferred_element_type=f32)
            p_s[pl.ds(r0, M), :c4] = o * OSC + (load_q(r0, M, 0, NL - 1) + b2[:, :c4])
            z = jnp.where(false_mask()[0:1, :], link[0:1, :], b2[:, c4:] * (1.0 / OSC))
            o = z + jnp.dot(h, w2_s[:, c4:], preferred_element_type=f32)
            p_s[pl.ds(r0, M), c4:] = o * OSC + load_q(r0, M, NL - 1, NL)
            conv_inv(i, Y)

        rev8 = 7 - row8

        def load_y(j, t):
            y = yp_s[j, t:t + 8, :]
            if t % P < 64:
                y = jnp.take_along_axis(y, rev8, axis=0)
            return y

        def combine(r0, r1, st):
            fm = false_mask()
            for t in range(r0, r1, 16):
                for j in range(NL):
                    cs = slice(j * 128, (j + 1) * 128)
                    y = jnp.concatenate([load_y(j, t), load_y(j, t + 8)], axis=0)
                    p0 = p_s[t:t + 8, cs]
                    if st[0] is not None:
                        p0 = jnp.where(fm, st[0], p0)
                    pp = jnp.concatenate([p0, p_s[t + 8:t + 16, cs]], axis=0)
                    r = (pp + xn_s[j, t:t + 16, :].astype(f32) * y).astype(bf16)
                    st[0] = r.astype(f32)[0:8, :]
                    o_s[j, t:t + 16, :] = r

        def first():
            wait(0)
            start(ring)
            ln(0, qa, False)
            wait(1)

            def r0a():
                start(1 + ring)
                bc_s[...] = jnp.broadcast_to(b1_row()[:, F - 128:F], (128, 128)).T[64:128, :]
                hid_s[0:qa, 0:w1c[1]] = mm1(load_xn(0, qa), 0, w1c[1]).astype(bf16)
            region(r0a)
            wait(2)

            def r0b():
                start(2 + ring)
                st = []
                ln(qa, M0, False, st)
                mu = jnp.concatenate([a_ for a_, _ in st], axis=0)
                rs = jnp.concatenate([b_ for _, b_ in st], axis=0)
                lhs = jnp.concatenate([jnp.ones((16, D), bf16), q_s[qa:M0, :]], axis=0)
                z = lax.dot_general(lhs, w1_s[0:w1c[1], :], NT, preferred_element_type=f32)
                g = (z[16:, :] - mu * z[0:1, :]) * rs + b1_row()[:, 0:w1c[1]]
                hid_s[qa:M0, 0:w1c[1]] = gelu(g).astype(bf16)
            region(r0b)
            for i in range(1, n1):
                wait(2 + i)

                def r1(i=i):
                    start(2 + i + ring)
                    if i == 1:
                        for j in range(NL):
                            w1n_s[j * 128:(j + 1) * 128, :] = (
                                w1_s[0:128, j * 128:(j + 1) * 128].astype(f32).T.astype(bf16))
                    hid_s[:, w1c[i]:w1c[i + 1]] = mm1(load_xn(0, M0), w1c[i], w1c[i + 1]).astype(bf16)
                region(r1)
            wait(ng - 4)

            def r2a():
                start(ng - 4 + ring)
                ln(M0, M0 + lns, True)
                p_s[0:M0, :] = jnp.dot(hid_s[:, :w2k], w2_s[:w2k, :], preferred_element_type=f32)
            region(r2a)
            wait(ng - 3)

            def r2b():
                lk = jnp.broadcast_to(ln(M0 + lns, S, True)[0:8, :], (8, 128))
                o = jnp.dot(hid_s[:, w2k:], w2_s[w2k:, :], preferred_element_type=f32) + p_s[0:M0, :]
                p_s[0:M0, :] = o * OSC + (load_q(0, M0) + b2_row())
                par = jnp.concatenate([sk_ref[...].astype(f32), dd_ref[...].astype(f32).reshape(1, D),
                                       jnp.zeros((3, D), f32)], axis=0)
                for j in range(NL):
                    par_s[j] = par[:, j * 128:(j + 1) * 128]
                kv_fwd(0, par[:, 0:128], lk)
            region(r2b)

        def pair(i, carry):
            si = lax.rem(ng - 2 + i, ring)
            for c in copies(kvh(2 * i + 1) + kvh(2 * i + 2), si):
                c.wait()
            mlp_conv(2 * i, False)
            kv_fwd(2 * i + 1, par_s[2 * i + 1])
            z = NB + flag_s[1]
            x_s[z, 0:8, :] = jnp.zeros((8, 128), f32)
            hf_s[z, 0:8, :] = jnp.zeros((8, 128), f32)
            mlp_conv(2 * i + 1, True)
            kv_fwd(2 * i + 2, par_s[2 * i + 2])
            return carry

        rl = S - ML

        def out_copies(js, r0, r1):
            return copies([(o_s.at[j, pl.ds(r0, r1 - r0), :], out_hbm.at[pl.ds(r0, r1 - r0), pl.ds(j * 128, 128)])
                           for j in js], sem_out)
        cuts = [0] + [int(rl // 16 * x) * 16 for x in prow] + [rl]
        g_o = [out_copies(range(NL), cuts[i], cuts[i + 1]) for i in range(nco)]
        g_fa = out_copies(range(osp), rl, S)
        g_fm = out_copies(range(osp, NL), rl, rl + rsp)
        g_fb = out_copies(range(osp, NL), rl + rsp, S)

        def pin_after(g, i):
            for c in g:
                c.start()
            z1 = pl.multiple_of(S + flag_s[1], 16)
            z2 = pl.multiple_of(S + flag_s[2], 16)
            o_s[0, pl.ds(z1, 16), :] = jnp.full((16, 128), i, bf16)
            return o_s[0, pl.ds(z2, 16), :].astype(f32)

        def last():
            mlp_conv(NL - 1, False)
            yp_s[NL + flag_s[1], 0:8, :] = jnp.zeros((8, 128), f32)
            p_s[pl.ds(pl.multiple_of(S + flag_s[1], 8), 8), 0:128] = jnp.zeros((8, 128), f32)
            xn = load_xn(rl, ML)
            st = [None]
            hs = []
            gi = 0
            for f in range(13):
                pin = None
                if gi < nco and pins[gi] == f:
                    combine(cuts[gi], cuts[gi + 1], st)
                    pin = pin_after(g_o[gi], gi)
                    gi += 1
                hs.append(mm1(xn, 128 * f, 128 * (f + 1), pin) if f else mm1_first(xn))
            hs.append(mm1_rem(xn))
            h = jnp.concatenate(hs, axis=1).astype(bf16)
            b2 = b2_row() * (1.0 / OSC)
            for j in range(NL):
                cs = slice(j * 128, (j + 1) * 128)
                bj = b2[:, cs]
                if gi < nco and pins[gi] == 14 + j:
                    combine(cuts[gi], cuts[gi + 1], st)
                    bj = jnp.where(false_mask()[0:1, :], pin_after(g_o[gi], gi)[0:1, :], bj)
                    gi += 1
                if j == osp:
                    bj = jnp.where(false_mask()[0:1, :], pin_after(g_fa, nco)[0:1, :], bj)
                for ra, rb in ([(rl, S)] if j < NL - 1 else [(rl, rl + rsp), (rl + rsp, S)]):
                    if ra > rl:
                        bj = jnp.where(false_mask()[0:1, :], pin_after(g_fm, nco + 1)[0:1, :], b2[:, cs])
                    o = (bj + jnp.dot(h[ra - rl:rb - rl, :], w2_s[:, cs], preferred_element_type=f32)) * OSC
                    o = o + load_q(ra, rb - ra, j, j + 1)
                    y = jnp.concatenate([load_y(j, t) for t in range(ra, rb, 8)], axis=0)
                    o_s[j, ra:rb, :] = (o + xn_s[j, ra:rb, :].astype(f32) * y).astype(bf16)
            assert gi == nco
        def it(i, carry):
            pl.when(i == 0)(first)
            pair(i, carry)
            pl.when(i == 1)(last)
            return carry
        lax.fori_loop(0, 2, it, 0)
        for c in g_fb:
            c.start()
        for g in g_o + [g_fa, g_fm, g_fb]:
            for c in g:
                c.wait()

    fw, inv = dft_mats()

    @jax.jit
    def f(q, k, v, sk, h, dd, w1, b1, w2, b2):
        any_ = pl.BlockSpec(memory_space=pl.ANY)
        out = pl.pallas_call(
            kernel,
            in_specs=[any_] * 12,
            out_specs=any_,
            out_shape=jax.ShapeDtypeStruct((S, D), bf16),
            scratch_shapes=[
                pltpu.VMEM((M0, D), bf16),
                pltpu.VMEM((NL, S, 128), bf16),
                pltpu.VMEM((NL, S + KP, 128), bf16),
                pltpu.VMEM((NL, S, 128), bf16),
                pltpu.VMEM((NL, 128, S), bf16),
                pltpu.VMEM((F, D), bf16),
                pltpu.VMEM((F, D), bf16),
                pltpu.VMEM((NL, S, 128), bf16),
                pltpu.VMEM((S + 8, D), f32),
                pltpu.VMEM((NB + 1, 256, 128), f32),
                pltpu.VMEM((NB + 1, 256, 128), f32),
                pltpu.VMEM((NL + 1, S, 128), f32),
                pltpu.VMEM((NL, S + 16, 128), bf16),
                pltpu.VMEM((NL, 8, 128), f32),
                pltpu.VMEM((M0, F), bf16),
                pltpu.VMEM((4, D), bf16), pltpu.VMEM((D,), bf16), pltpu.VMEM((F,), bf16), pltpu.VMEM((D,), bf16),
                pltpu.VMEM((2, 256, 128), bf16), pltpu.VMEM((2, 64, 128), bf16),
                pltpu.VMEM((64, 128), f32),
                pltpu.VMEM((D, 128), bf16),
                pltpu.SMEM((4,), jnp.int32),
                pltpu.SemaphoreType.DMA((ring,)),
            ],
            compiler_params=pltpu.CompilerParams(vmem_limit_bytes=100 * 2**20, shape_invariant_numerics=False),
            name=name,
        )(q.reshape(S, D), k.reshape(S, D), v.reshape(S, D), sk.T, h, dd, w1.T, b1, w2, b2, fw, inv)
        return out.reshape(1, S, D)
    return f


_impl = make(name="fused_h3_mlp")


@jax.jit
def pallas_parallel_sum__ssm_conv_h3__dense_activation_gelu__prompt_kernel(
    A_q, A_k, A_v, A_shift_k, A_ssm_k, A_ssm_D, B_x, B_w1, B_b1, B_w2, B_b2,
):
    del B_x
    return _impl(A_q, A_k, A_v, A_shift_k, A_ssm_k, A_ssm_D, B_w1, B_b1, B_w2, B_b2)
```
